```python
import jax
import jax.numpy as jnp

def _softmax(x, axis=-1):
    return jax.nn.softmax(x, axis=axis)

def _gelu(x):
    return jax.nn.gelu(x, approximate=True)

def _silu(x):
    return jax.nn.silu(x)

def _sigmoid(x):
    return jax.nn.sigmoid(x)

def _layernorm(x, axis=-1, eps=1e-05):
    m = jnp.mean(x, axis=axis, keepdims=True)
    v = jnp.var(x, axis=axis, keepdims=True)
    return (x - m) / jnp.sqrt(v + eps)

def _scatter_add(tgt, idx, src, axis=0):
    return tgt.at[idx].add(src)

def _segment_sum(src, seg, n):
    return jax.ops.segment_sum(src, seg, n)

class _Rng:

    def __init__(self, key):
        self._k = key

    def _next(self):
        self._k, sub = jax.random.split(self._k)
        return sub

    def normal(self, shape):
        return jax.random.normal(self._next(), shape, dtype=jnp.bfloat16)

    def randint(self, lo, hi, shape):
        return jax.random.randint(self._next(), shape, lo, hi, dtype=jnp.int32)

    def uniform(self, shape, lo=0.0, hi=1.0):
        return jax.random.uniform(self._next(), shape, jnp.bfloat16, lo, hi)

    def permutation(self, n):
        return jax.random.permutation(self._next(), n)
kernel_name = 'concat_heads__ssm_conv_h3__memory_aug_infini_attn__prompt'

def setup_inputs():
    _rng = _Rng(jax.random.key(int.from_bytes(__import__("os").urandom(4), "little")))
    _w = lambda a: (lambda t: t.astype(jnp.bfloat16) if jnp.issubdtype(t.dtype, jnp.floating) else t)(jnp.asarray(a))

    def _A_setup():
        B, S, D = (1, 2048, 640)
        ks = 4
        return {'q': _w((lambda *s: _rng.normal(s) * 0.05)(B, S, D)), 'k': _w((lambda *s: _rng.normal(s) * 0.05)(B, S, D)), 'v': _w((lambda *s: _rng.normal(s) * 0.05)(B, S, D)), 'shift_k': _w((lambda *s: _rng.normal(s) * 0.05)(D, ks) * 0.5), 'ssm_k': _w((lambda *s: _rng.normal(s) * 0.05)(D, S) * (1.0 / S ** 0.5)), 'ssm_D': _w((lambda *s: _rng.normal(s) * 0.05)(D))}
    _A_in = _A_setup()

    def _B_setup():
        B, S, D, H = (1, 2048, 640, 32)
        N = 4
        L = max(1, S // N)
        sc = D ** (-0.5)
        return {'x': _w((lambda *s: _rng.normal(s) * 0.05)(B, N * L, D)), 'wq': _w((lambda *s: _rng.normal(s) * 0.05)(D, D) * sc), 'wk': _w((lambda *s: _rng.normal(s) * 0.05)(D, D) * sc), 'wv': _w((lambda *s: _rng.normal(s) * 0.05)(D, D) * sc), 'wo': _w((lambda *s: _rng.normal(s) * 0.05)(D, D) * sc), 'beta': _w((lambda *s: _rng.normal(s) * 0.05)(H))}
    _B_in = _B_setup()
    return {'A_q': _A_in['q'], 'A_k': _A_in['k'], 'A_v': _A_in['v'], 'A_shift_k': _A_in['shift_k'], 'A_ssm_k': _A_in['ssm_k'], 'A_ssm_D': _A_in['ssm_D'], 'B_x': _B_in['x'], 'B_wq': _B_in['wq'], 'B_wk': _B_in['wk'], 'B_wv': _B_in['wv'], 'B_wo': _B_in['wo'], 'B_beta': _B_in['beta']}

def reference(A_q, A_k, A_v, A_shift_k, A_ssm_k, A_ssm_D, B_x, B_wq, B_wk, B_wv, B_wo, B_beta):

    def _A_ref(q, k, v, shift_k, ssm_k, ssm_D):
        B, S, D = q.shape
        ks = shift_k.shape[-1]
        k_pad = jnp.pad(k, ((0, 0), (ks - 1, 0), (0, 0)))
        k_shift = jnp.zeros_like(k)
        for t in range(ks):
            k_shift = k_shift + k_pad[:, t:t + S, :] * shift_k[:, ks - 1 - t][None, None, :]
        kv = k_shift * v
        L = 2 * S
        kv_pad = jnp.pad(kv, ((0, 0), (0, S), (0, 0)))
        kf_pad = jnp.pad(ssm_k, ((0, 0), (0, S)))
        kv_f = (lambda x, axes=(-2, -1): jnp.fft.rfft2(x.astype(jnp.float32), axes=axes))(kv_pad[:, None, :, :], axes=(1, 2))
        kf_f = (lambda x, axes=(-2, -1): jnp.fft.rfft2(x.astype(jnp.float32), axes=axes))(kf_pad[:, None, :], axes=(1, 2))
        kf_f = (lambda x, *d: x.transpose(*d))(kf_f, 1, 2, 0)
        y_f = kv_f * kf_f[None, :, :, :]
        y = (lambda x, s, axes=(-2, -1): jnp.fft.irfft2(x, s=s, axes=axes).astype(jnp.bfloat16))(y_f, (1, L), axes=(1, 2))[:, 0, :S, :]
        y = y + kv * ssm_D[None, None, :]
        return q * y

    def _B_ref(x, wq, wk, wv, wo, beta):
        B, S, D = x.shape
        H = 32
        Dh = D // H
        N = 4
        L = S // N
        q = (lambda x, *d: x.transpose(*d))((x @ wq).reshape(B, S, H, Dh), 0, 2, 1, 3).reshape(B, H, N, L, Dh)
        k = (lambda x, *d: x.transpose(*d))((x @ wk).reshape(B, S, H, Dh), 0, 2, 1, 3).reshape(B, H, N, L, Dh)
        v = (lambda x, *d: x.transpose(*d))((x @ wv).reshape(B, S, H, Dh), 0, 2, 1, 3).reshape(B, H, N, L, Dh)
        phi = lambda t: jnp.where(t > 0, t + 1.0, jnp.exp(t))
        scale = Dh ** (-0.5)
        ar = jnp.arange(L)
        mask = (lambda x, dt: x.astype(dt))(ar[:, None] < ar[None, :], x.dtype) * -1000000000.0
        g = _sigmoid(beta).reshape(1, H, 1, 1)
        M = jnp.einsum('bhd,bhe->bhde', q[:, :, 0, 0, :] * 0.0, q[:, :, 0, 0, :] * 0.0)
        z = q[:, :, 0, 0, :] * 0.0
        outs = []
        for s in range(N):
            qs, ks, vs = (q[:, :, s].copy(), k[:, :, s].copy(), v[:, :, s].copy())
            logits = jnp.einsum('bhqd,bhkd->bhqk', qs, ks) * scale + mask
            p = _softmax(logits, axis=-1)
            a_dot = jnp.einsum('bhqk,bhkd->bhqd', p, vs)
            pq = phi(qs)
            num = jnp.einsum('bhld,bhde->bhle', pq, M)
            den = jnp.einsum('bhld,bhd->bhl', pq, z)[..., None] + 1e-06
            a_mem = num / den
            o = g * a_mem + (1.0 - g) * a_dot
            outs.append(o)
            pk = phi(ks)
            M = M + jnp.einsum('bhld,bhle->bhde', pk, vs)
            z = z + jnp.einsum('bhld->bhd', pk)
        o = (lambda x, *d: x.transpose(*d))(jnp.stack(outs, 2).reshape(B, H, S, Dh), 0, 2, 1, 3).reshape(B, S, D)
        return o @ wo
    a = _A_ref(A_q, A_k, A_v, A_shift_k, A_ssm_k, A_ssm_D)
    b = _B_ref(B_x, B_wq, B_wk, B_wv, B_wo, B_beta)
    return jnp.concatenate([a, b], axis=-1)
```

```python
import math

import numpy as np
import jax
import jax.numpy as jnp
from jax import lax
import jax.experimental.pallas as pl
import jax.experimental.pallas.tpu as pltpu

_S = 2048
_D = 640
_H = 32
_DH = 20
_NSEG = 4
_L = _S // _NSEG
_C = 128
_NC = _S // _C
_NG = _D // _C
_NQ = _H // 4
_KS = 4

_F32 = jnp.float32
_BF16 = jnp.bfloat16
_U32 = jnp.uint32
_LOG2E = math.log2(math.e)
_ONES_BF16_PAIR = 0x3F803F80


def _dft_matrix():
    k = np.concatenate([np.arange(0, _C, 2), np.arange(1, _C, 2)])
    ang = np.pi * np.outer(2 * k + 1, np.arange(_C)) / (2 * _C)
    return np.concatenate([np.cos(ang), -np.sin(ang)], axis=0).astype(np.float32)


def _dot(a, b):
    return jnp.dot(a, b, preferred_element_type=_F32)


def _dot_nt(a, b):
    return lax.dot_general(a, b, (((1,), (1,)), ((), ())), preferred_element_type=_F32)


def _dot_tn(a, b):
    return lax.dot_general(a, b, (((0,), (0,)), ((), ())), preferred_element_type=_F32)


def _as_bf16(words):
    return pltpu.bitcast(words, _BF16)


def _phi(t):
    return jnp.where(t > 0, t + 1.0, jnp.exp(t))


def _causal_conv(u, h):
    out = []
    for a in range(len(u)):
        acc = u[a] * h[0]
        for j in range(1, a + 1):
            acc = acc + u[a - j] * h[j]
        out.append(acc)
    return out


def _kernel(q_hbm, k_hbm, v_hbm, shift_hbm, h_hbm, d_hbm, x_hbm,
            wq_hbm, wk_hbm, wv_hbm, wo_hbm, beta_hbm, f_hbm, ft_hbm, out_hbm,
            qa_buf, ka_buf, va_buf, h_buf, x_buf, wq_buf, wk_buf, wv_buf, wo_buf,
            shift_buf, d_buf, beta_buf, f_buf, ft_buf,
            par_scr, gate_scr, kpad_scr, kv_scr, u_scr, hs_scr, y_scr, outa_buf,
            wt_scr, qs_scr, pq_scr, vt_scr, kn_scr, pk_scr, kwin_scr, pkwin_scr,
            ot_scr, outb_buf,
            sem_a, sem_b, sem_c, sem_oa, sem_ob):

    def col(j):
        return pl.ds(pl.multiple_of(j * _C, _C), _C)

    def group_copies(j):
        cp = pltpu.make_async_copy
        return [
            cp(k_hbm.at[:, col(j)], ka_buf.at[j], sem_a.at[0, j]),
            cp(v_hbm.at[:, col(j)], va_buf.at[j], sem_a.at[1, j]),
            cp(h_hbm.at[col(j), :], h_buf.at[j], sem_a.at[2, j]),
            cp(wq_hbm.at[:, col(j)], wq_buf.at[j], sem_a.at[3, j]),
            cp(wk_hbm.at[:, col(j)], wk_buf.at[j], sem_a.at[4, j]),
            cp(wv_hbm.at[:, col(j)], wv_buf.at[j], sem_a.at[5, j]),
            cp(q_hbm.at[:, col(j)], qa_buf.at[j], sem_a.at[6, j]),
        ]

    def outa_copy(j):
        return pltpu.make_async_copy(outa_buf.at[j], out_hbm.at[:, col(j)], sem_oa.at[j])

    def outb_copy(p):
        return pltpu.make_async_copy(
            outb_buf.at[p], out_hbm.at[pl.ds(p * _L, _L), pl.ds(_D, _D)], sem_ob.at[p])

    small = [
        pltpu.make_async_copy(shift_hbm, shift_buf, sem_c.at[0]),
        pltpu.make_async_copy(d_hbm, d_buf, sem_c.at[1]),
        pltpu.make_async_copy(beta_hbm, beta_buf, sem_c.at[2]),
        pltpu.make_async_copy(f_hbm, f_buf, sem_c.at[3]),
        pltpu.make_async_copy(ft_hbm, ft_buf, sem_c.at[4]),
    ]
    x_copies = [
        pltpu.make_async_copy(x_hbm.at[:, pl.ds(g * _C, _C)], x_buf.at[g], sem_b.at[g])
        for g in range(_NG)
    ]
    wo_copy = pltpu.make_async_copy(wo_hbm, wo_buf, sem_c.at[5])

    for c in small:
        c.start()
    for c in group_copies(0):
        c.start()
    for c in x_copies:
        c.start()
    for c in small:
        c.wait()

    shift = shift_buf[...].astype(_F32)
    dvec = d_buf[...].astype(_F32).reshape(1, _D)
    for g in range(_NG):
        sl = slice(g * _C, (g + 1) * _C)
        for t in range(_KS):
            par_scr[g, t] = jnp.broadcast_to(shift[t:t + 1, sl], (8, _C))
        par_scr[g, _KS] = jnp.broadcast_to(dvec[:, sl], (8, _C))
    beta = beta_buf[...].astype(_F32).reshape(1, _H)
    gate = 1.0 / (1.0 + jnp.exp(-beta))
    for hd in range(_H):
        gate_scr[hd] = jnp.broadcast_to(gate[:, hd:hd + 1], (8, _C))
    kpad_scr[0:8, :] = jnp.zeros((8, _C), _F32)

    for c in x_copies:
        c.wait()

    x_w = x_buf.bitcast(_U32)
    f_w = f_buf.bitcast(_U32)
    ka_w = ka_buf.bitcast(_U32)
    va_w = va_buf.bitcast(_U32)
    qa_w = qa_buf.bitcast(_U32)
    kv_w = kv_scr.bitcast(_U32)
    wt_w = wt_scr.bitcast(_U32)
    wk_w = wk_buf.bitcast(_U32)
    q_scale = _DH ** -0.5 * _LOG2E

    def x_rows(lo, n):
        return jnp.concatenate(
            [_as_bf16(x_w[g, lo // 2:(lo + n) // 2, :]) for g in range(_NG)], axis=1)

    def phase1(j, carry):
        @pl.when(j + 1 < _NG)
        def _():
            for c in group_copies(j + 1):
                c.start()

        @pl.when(j == _NG - 1)
        def _():
            wo_copy.start()

        for c in group_copies(j):
            c.wait()

        for w_buf, base in ((wq_buf, 0), (wv_buf, _C)):
            wt = w_buf[j].T
            for g in range(_NG):
                wt_scr[g, base:base + _C, :] = wt[:, g * _C:(g + 1) * _C]

        taps = [par_scr[j, t] for t in range(_KS)]
        skip = par_scr[j, _KS]
        fmat = _as_bf16(f_w[...])

        def tile(v):
            return jnp.tile(v, (_C // 8, 1))

        for a in range(_NC):
            rows = slice(a * _C // 2, (a + 1) * _C // 2)
            kpad_scr[8 + a * _C:8 + (a + 1) * _C, :] = _as_bf16(ka_w[j, rows, :]).astype(_F32)
        for a in range(_NC):
            rows = slice(a * _C // 2, (a + 1) * _C // 2)
            ks = kpad_scr[8 + a * _C:8 + (a + 1) * _C, :] * tile(taps[0])
            for t in range(1, _KS):
                ks = ks + kpad_scr[8 + a * _C - t:8 + (a + 1) * _C - t, :] * tile(taps[t])
            kv = (ks * _as_bf16(va_w[j, rows, :]).astype(_F32)).astype(_BF16)
            kv_scr[a * _C:(a + 1) * _C, :] = kv
            u_scr[a] = _dot(fmat, kv)
            hs_scr[a] = _dot_nt(fmat, h_buf[j, :, a * _C:(a + 1) * _C])

        def cross_chunk(r):
            re, im = slice(8 * r, 8 * r + 8), slice(_C + 8 * r, _C + 8 * r + 8)
            hr = [hs_scr[a, re, :] for a in range(_NC)]
            hi = [hs_scr[a, im, :] for a in range(_NC)]
            if r < _C // 16:
                c = [hr[0]] + [hr[a] - hi[a - 1] for a in range(1, _NC)]
                d = [hi[0]] + [hi[a] + hr[a - 1] for a in range(1, _NC)]
            else:
                c = [hr[0]] + [hr[a] + hi[a - 1] for a in range(1, _NC)]
                d = [hi[0]] + [hi[a] - hr[a - 1] for a in range(1, _NC)]
            ur = [u_scr[a, re, :] for a in range(_NC)]
            ui = [u_scr[a, im, :] for a in range(_NC)]
            k1 = _causal_conv([ur[a] + ui[a] for a in range(_NC)], c)
            k2 = _causal_conv(ur, [d[a] - c[a] for a in range(_NC)])
            for a in range(_NC):
                y_scr[a, im, :] = k1[a] + k2[a]
            k3 = _causal_conv(ui, [c[a] + d[a] for a in range(_NC)])
            for a in range(_NC):
                y_scr[a, re, :] = k1[a] - k3[a]

        def project(p, n):
            xs = x_rows(p * n, n)
            wt = jnp.concatenate([_as_bf16(wt_w[g]) for g in range(_NG)], axis=1)
            qv = _dot_nt(wt, xs)
            wk = jnp.concatenate(
                [_as_bf16(wk_w[j, g * 64:(g + 1) * 64, :]) for g in range(_NG)], axis=0)
            kn = _dot(xs, wk)
            row = pl.ds(pl.multiple_of(j * _C, _C), _C)
            for t in range(n // _C):
                tt = p * (n // _C) + t
                qt = qv[0:_C, t * _C:(t + 1) * _C]
                qs_scr[tt, row, :] = (qt * q_scale).astype(_BF16)
                if tt >= _L // _C:
                    pq_scr[tt - _L // _C, row, :] = _phi(qt).astype(_BF16)
                vt_scr[tt, row, :] = qv[_C:2 * _C, t * _C:(t + 1) * _C].astype(_BF16)
            kn_scr[j, p * n:(p + 1) * n, :] = kn.astype(_BF16)
            if p * n < _S - _L:
                pk_scr[j, p * n:(p + 1) * n, :] = _phi(kn).astype(_BF16)

        piece = 256
        n_piece = _S // piece
        for p in range(n_piece):
            project(p, piece)
            for r in range(p * 16 // n_piece, (p + 1) * 16 // n_piece):
                cross_chunk(r)

        ftm = ft_buf[...]
        for a in range(_NC):
            rows = slice(a * _C // 2, (a + 1) * _C // 2)
            y = _dot(ftm, y_scr[a].astype(_BF16)) * (1.0 / _C)
            y = y + _as_bf16(kv_w[rows, :]).astype(_F32) * tile(skip)
            outa_buf[j, a * _C:(a + 1) * _C, :] = (
                _as_bf16(qa_w[j, rows, :]).astype(_F32) * y).astype(_BF16)
        outa_copy(j).start()
        return carry

    lax.fori_loop(0, _NG, phase1, 0)

    qs_w = qs_scr.bitcast(_U32)
    pq_w = pq_scr.bitcast(_U32)
    vt_w = vt_scr.bitcast(_U32)
    kn_w = kn_scr.bitcast(_U32)
    pk_w = pk_scr.bitcast(_U32)
    kwin_w = kwin_scr.bitcast(_U32)
    pkwin_w = pkwin_scr.bitcast(_U32)
    tiles = _L // _C

    def phase2(m, carry):
        first = m * (4 * _DH)
        off = lax.rem(first, _C)
        g0 = lax.div(first, _C)
        g1 = jnp.minimum(g0 + 1, _NG - 1)
        shift_l = lax.rem(_C - off, _C)

        def window(src, dst, n_rows):
            lane = lax.broadcasted_iota(jnp.int32, (n_rows // 2, _C), 1)
            w = jnp.where(lane >= off, src[g0], src[g1])
            dst[...] = pltpu.roll(w, shift_l, 1)

        window(kn_w, kwin_w, _S)
        window(pk_w, pkwin_w, _S - _L)

        wrow = pl.ds(pl.multiple_of(m * 40, 8), 40)
        row16 = lax.broadcasted_iota(jnp.int32, (16, _C), 0)
        in_head = [(row16 >= 2 * hh) & (row16 < 2 * hh + 10) for hh in range(4)]
        key_id = lax.broadcasted_iota(jnp.int32, (_C, _C), 0)
        qry_id = lax.broadcasted_iota(jnp.int32, (_C, _C), 1)
        causal = key_id <= qry_id
        row8 = lax.broadcasted_iota(jnp.int32, (8, _C), 0)
        low_half = row8 < 4
        gates = [gate_scr[m * 4 + hh] for hh in range(4)]
        ones_w = jnp.full((8, _C), _ONES_BF16_PAIR, _U32)

        mrow = lax.broadcasted_iota(jnp.int32, (96, _C), 0)
        mlane = lax.broadcasted_iota(jnp.int32, (96, _C), 1)
        mmask = jnp.zeros((96, _C), jnp.bool_)
        for hh in range(4):
            lanes = (mlane >= _DH * hh) & (mlane < _DH * (hh + 1))
            rows = ((mrow >= _DH * hh) & (mrow < _DH * (hh + 1))) | (mrow == 80 + hh)
            mmask = mmask | (lanes & rows)

        def spread(f):
            return jnp.concatenate(
                [f[0], f[0], jnp.where(low_half, f[0], f[1]), f[1], f[1],
                 f[2], f[2], jnp.where(low_half, f[2], f[3]), f[3], f[3]], axis=0)

        mem = None
        for s in range(_NSEG):
            vq = [vt_w[tiles * s + t, wrow, :] for t in range(tiles)]
            vext = [
                [_as_bf16(jnp.where(in_head[hh], vq[t][8 * hh:8 * hh + 16],
                                    jnp.uint32(_ONES_BF16_PAIR))) for t in range(tiles)]
                for hh in range(4)]
            mem_b = None if mem is None else mem.astype(_BF16)
            for i in range(tiles):
                tt = tiles * s + i
                qq = qs_w[tt, wrow, :]
                accs, norm = [], []
                for hh in range(4):
                    qh = jnp.where(in_head[hh], qq[8 * hh:8 * hh + 16], jnp.uint32(0))
                    parts = []
                    if hh > 0:
                        parts.append(jnp.zeros((8 * hh, _C), _U32))
                    parts += [qh, jnp.zeros((48 - 8 * hh, _C), _U32)]
                    qm = _as_bf16(jnp.concatenate(parts, axis=0))
                    keys = _as_bf16(kwin_w[s * _L // 2:(s * _L + (i + 1) * _C) // 2, :])
                    sc = _dot(keys, qm)
                    diag = jnp.where(causal, sc[i * _C:], -jnp.inf)
                    sc = diag if i == 0 else jnp.concatenate([sc[:i * _C], diag], axis=0)
                    mx = jnp.max(sc, axis=0, keepdims=True)
                    p = jnp.exp2(sc - mx).astype(_BF16)
                    vh = jnp.concatenate(vext[hh][:i + 1], axis=1)
                    acc = _dot(vh, p)
                    accs.append(acc)
                    denom = acc[24:32] if hh < 2 else acc[0:8]
                    norm.append((1.0 - gates[hh]) / denom)
                o = jnp.concatenate(
                    [accs[0][0:16], jnp.where(low_half, accs[0][16:24], accs[1][0:8]),
                     accs[1][8:24], accs[2][8:24],
                     jnp.where(low_half, accs[2][24:32], accs[3][8:16]), accs[3][16:32]],
                    axis=0) * spread(norm)
                if mem_b is not None:
                    pq = _as_bf16(jnp.concatenate(
                        [pq_w[tt - tiles, wrow, :], jnp.zeros((24, _C), _U32)], axis=0))
                    got = _dot(mem_b, pq)
                    fac = [gates[hh] / (jnp.broadcast_to(got[80 + hh:81 + hh], (8, _C)) + 1e-6)
                           for hh in range(4)]
                    o = o + got[0:80] * spread(fac)
                ot_scr[tt, pl.ds(pl.multiple_of(first, 16), 80), :] = o.astype(_BF16)
            if s < _NSEG - 1:
                vall = jnp.concatenate(
                    [_as_bf16(jnp.concatenate([vq[t], ones_w], axis=0)) for t in range(tiles)],
                    axis=1)
                pk = _as_bf16(pkwin_w[s * _L // 2:(s + 1) * _L // 2, :])
                upd = jnp.where(mmask, _dot(vall, pk), 0.0)
                mem = upd if mem is None else mem + upd
        return carry

    lax.fori_loop(0, _NQ, phase2, 0)

    wo_copy.wait()
    for p in range(_NSEG):
        ot = jnp.concatenate([ot_scr[tiles * p + t] for t in range(tiles)], axis=1)
        outb_buf[p] = _dot_tn(ot, wo_buf[...]).astype(_BF16)
        outb_copy(p).start()
    for j in range(_NG):
        outa_copy(j).wait()
    for p in range(_NSEG):
        outb_copy(p).wait()


@jax.jit
def pallas_concat_heads__ssm_conv_h3__memory_aug_infini_attn__prompt_kernel(
    A_q: jax.Array,
    A_k: jax.Array,
    A_v: jax.Array,
    A_shift_k: jax.Array,
    A_ssm_k: jax.Array,
    A_ssm_D: jax.Array,
    B_x: jax.Array,
    B_wq: jax.Array,
    B_wk: jax.Array,
    B_wv: jax.Array,
    B_wo: jax.Array,
    B_beta: jax.Array,
):
    assert A_q.shape == (1, _S, _D) and B_x.shape == (1, _S, _D)
    assert A_shift_k.shape == (_D, _KS) and B_beta.shape == (_H,)
    fmat = _dft_matrix()
    f_fwd = fmat.astype(_BF16)
    f_inv = np.ascontiguousarray(fmat.T).astype(_BF16)

    vmem = pltpu.VMEM
    dma = pltpu.SemaphoreType.DMA
    scratch = [
        vmem((_NG, _S, _C), _BF16),
        vmem((_NG, _S, _C), _BF16),
        vmem((_NG, _S, _C), _BF16),
        vmem((_NG, _C, _S), _BF16),
        vmem((_NG, _S, _C), _BF16),
        vmem((_NG, _D, _C), _BF16),
        vmem((_NG, _D, _C), _BF16),
        vmem((_NG, _D, _C), _BF16),
        vmem((_D, _D), _BF16),
        vmem((_KS, _D), _BF16),
        vmem((_D,), _BF16),
        vmem((_H,), _BF16),
        vmem((2 * _C, _C), _BF16),
        vmem((_C, 2 * _C), _BF16),
        vmem((_NG, _KS + 1, 8, _C), _F32),
        vmem((_H, 8, _C), _F32),
        vmem((_S + 8, _C), _F32),
        vmem((_S, _C), _BF16),
        vmem((_NC, 2 * _C, _C), _F32),
        vmem((_NC, 2 * _C, _C), _F32),
        vmem((_NC, 2 * _C, _C), _F32),
        vmem((_NG, _S, _C), _BF16),
        vmem((_NG, 2 * _C, _C), _BF16),
        vmem((_NC, _D, _C), _BF16),
        vmem((_NC - _L // _C, _D, _C), _BF16),
        vmem((_NC, _D, _C), _BF16),
        vmem((_NG, _S, _C), _BF16),
        vmem((_NG, _S - _L, _C), _BF16),
        vmem((_S, _C), _BF16),
        vmem((_S - _L, _C), _BF16),
        vmem((_NC, _D, _C), _BF16),
        vmem((_NSEG, _L, _D), _BF16),
        dma((7, _NG)), dma((_NG,)), dma((6,)), dma((_NG,)), dma((_NSEG,)),
    ]
    out = pl.pallas_call(
        _kernel,
        out_shape=jax.ShapeDtypeStruct((_S, 2 * _D), _BF16),
        in_specs=[pl.BlockSpec(memory_space=pl.ANY)] * 14,
        out_specs=pl.BlockSpec(memory_space=pl.ANY),
        scratch_shapes=scratch,
        compiler_params=pltpu.CompilerParams(vmem_limit_bytes=100 * 1024 * 1024),
        name="h3_infini",
    )(A_q.reshape(_S, _D), A_k.reshape(_S, _D), A_v.reshape(_S, _D), A_shift_k.T,
      A_ssm_k, A_ssm_D, B_x.reshape(_S, _D), B_wq, B_wk, B_wv, B_wo, B_beta,
      f_fwd, f_inv)
    return out.reshape(1, _S, 2 * _D)
```

```python
import math

import numpy as np
import jax
import jax.numpy as jnp
from jax import lax
import jax.experimental.pallas as pl
import jax.experimental.pallas.tpu as pltpu

_S = 2048
_D = 640
_H = 32
_DH = 20
_NSEG = 4
_L = _S // _NSEG
_C = 128
_NC = _S // _C
_NG = _D // _C
_NQ = _H // 4
_KS = 4
_LAG = 5

_F32 = jnp.float32
_BF16 = jnp.bfloat16
_U32 = jnp.uint32
_LOG2E = math.log2(math.e)
_ONES_BF16_PAIR = 0x3F803F80


def _dft_matrix():
    k = np.concatenate([np.arange(0, _C, 2), np.arange(1, _C, 2)])
    ang = np.pi * np.outer(2 * k + 1, np.arange(_C)) / (2 * _C)
    return np.concatenate([np.cos(ang), -np.sin(ang)], axis=0).astype(np.float32)


def _dot(a, b):
    return jnp.dot(a, b, preferred_element_type=_F32)


def _dot_nt(a, b):
    return lax.dot_general(a, b, (((1,), (1,)), ((), ())), preferred_element_type=_F32)


def _dot_tn(a, b):
    return lax.dot_general(a, b, (((0,), (0,)), ((), ())), preferred_element_type=_F32)


def _as_bf16(words):
    return pltpu.bitcast(words, _BF16)


def _phi(t):
    return jnp.where(t > 0, t + 1.0, jnp.exp(t))


def _causal_conv(u, h):
    out = []
    for a in range(len(u)):
        acc = u[a] * h[0]
        for j in range(1, a + 1):
            acc = acc + u[a - j] * h[j]
        out.append(acc)
    return out


def _kernel(q_hbm, k_hbm, v_hbm, shift_hbm, h_hbm, d_hbm, x_hbm,
            wq_hbm, wk_hbm, wv_hbm, wo_hbm, beta_hbm, f_hbm, ft_hbm, out_hbm,
            qa_buf, ka_buf, va_buf, h_buf, x_buf, wq_buf, wk_buf, wv_buf, wo_buf,
            shift_buf, d_buf, beta_buf, f_buf, ft_buf,
            par_scr, gate_scr, kpad_scr, kv_scr, u_scr, hs_scr, y_scr, outa_buf,
            wt_scr, qs_scr, pq_scr, vt_scr, kn_scr, pk_scr, kwin_scr, pkwin_scr,
            s_scr, amem_scr, ot_scr, outb_buf,
            sem_a, sem_b, sem_c, sem_oa, sem_ob):

    def col(j):
        return pl.ds(pl.multiple_of(j * _C, _C), _C)

    def group_copies(j):
        cp = pltpu.make_async_copy
        return [
            cp(k_hbm.at[:, col(j)], ka_buf.at[j], sem_a.at[0, j]),
            cp(v_hbm.at[:, col(j)], va_buf.at[j], sem_a.at[1, j]),
            cp(h_hbm.at[col(j), :], h_buf.at[j], sem_a.at[2, j]),
            cp(wq_hbm.at[:, col(j)], wq_buf.at[j], sem_a.at[3, j]),
            cp(wk_hbm.at[:, col(j)], wk_buf.at[j], sem_a.at[4, j]),
            cp(wv_hbm.at[:, col(j)], wv_buf.at[j], sem_a.at[5, j]),
            cp(q_hbm.at[:, col(j)], qa_buf.at[j], sem_a.at[6, j]),
        ]

    def outa_copy(j):
        return pltpu.make_async_copy(outa_buf.at[j], out_hbm.at[:, col(j)], sem_oa.at[j])

    def outb_copy(p):
        return pltpu.make_async_copy(
            outb_buf.at[p], out_hbm.at[pl.ds(p * _L, _L), pl.ds(_D, _D)], sem_ob.at[p])

    small = [
        pltpu.make_async_copy(shift_hbm, shift_buf, sem_c.at[0]),
        pltpu.make_async_copy(d_hbm, d_buf, sem_c.at[1]),
        pltpu.make_async_copy(beta_hbm, beta_buf, sem_c.at[2]),
        pltpu.make_async_copy(f_hbm, f_buf, sem_c.at[3]),
        pltpu.make_async_copy(ft_hbm, ft_buf, sem_c.at[4]),
    ]
    x_copies = [
        pltpu.make_async_copy(x_hbm.at[:, pl.ds(g * _C, _C)], x_buf.at[g], sem_b.at[g])
        for g in range(_NG)
    ]
    wo_copy = pltpu.make_async_copy(wo_hbm, wo_buf, sem_c.at[5])

    for c in small:
        c.start()
    for c in group_copies(0):
        c.start()
    for c in x_copies:
        c.start()
    for c in small:
        c.wait()

    shift = shift_buf[...].astype(_F32)
    dvec = d_buf[...].astype(_F32).reshape(1, _D)
    for g in range(_NG):
        sl = slice(g * _C, (g + 1) * _C)
        for t in range(_KS):
            par_scr[g, t] = jnp.broadcast_to(shift[t:t + 1, sl], (8, _C))
        par_scr[g, _KS] = jnp.broadcast_to(dvec[:, sl], (8, _C))
    beta = beta_buf[...].astype(_F32).reshape(1, _H)
    gate = 1.0 / (1.0 + jnp.exp(-beta))
    for hd in range(_H):
        gate_scr[hd] = jnp.broadcast_to(gate[:, hd:hd + 1], (8, _C))
    kpad_scr[0:8, :] = jnp.zeros((8, _C), _F32)

    for c in x_copies:
        c.wait()

    x_w = x_buf.bitcast(_U32)
    f_w = f_buf.bitcast(_U32)
    ka_w = ka_buf.bitcast(_U32)
    va_w = va_buf.bitcast(_U32)
    qa_w = qa_buf.bitcast(_U32)
    kv_w = kv_scr.bitcast(_U32)
    wt_w = wt_scr.bitcast(_U32)
    wk_w = wk_buf.bitcast(_U32)
    q_scale = _DH ** -0.5 * _LOG2E

    def x_rows(lo, n):
        return jnp.concatenate(
            [_as_bf16(x_w[g, lo // 2:(lo + n) // 2, :]) for g in range(_NG)], axis=1)

    def phase1(j, carry):
        @pl.when(j + 1 < _NG)
        def _():
            for c in group_copies(j + 1):
                c.start()

        @pl.when(j == _NG - 1)
        def _():
            wo_copy.start()

        for c in group_copies(j):
            c.wait()

        for w_buf, base in ((wq_buf, 0), (wv_buf, _C)):
            wt = w_buf[j].T
            for g in range(_NG):
                wt_scr[g, base:base + _C, :] = wt[:, g * _C:(g + 1) * _C]

        taps = [par_scr[j, t] for t in range(_KS)]
        skip = par_scr[j, _KS]
        fmat = _as_bf16(f_w[...])

        def tile(v):
            return jnp.tile(v, (_C // 8, 1))

        for a in range(_NC):
            rows = slice(a * _C // 2, (a + 1) * _C // 2)
            kpad_scr[8 + a * _C:8 + (a + 1) * _C, :] = _as_bf16(ka_w[j, rows, :]).astype(_F32)
        for a in range(_NC):
            rows = slice(a * _C // 2, (a + 1) * _C // 2)
            ks = kpad_scr[8 + a * _C:8 + (a + 1) * _C, :] * tile(taps[0])
            for t in range(1, _KS):
                ks = ks + kpad_scr[8 + a * _C - t:8 + (a + 1) * _C - t, :] * tile(taps[t])
            kv = (ks * _as_bf16(va_w[j, rows, :]).astype(_F32)).astype(_BF16)
            kv_scr[a * _C:(a + 1) * _C, :] = kv
            u_scr[a] = _dot(fmat, kv)
            hs_scr[a] = _dot_nt(fmat, h_buf[j, :, a * _C:(a + 1) * _C])

        def cross_chunk(r):
            re, im = slice(8 * r, 8 * r + 8), slice(_C + 8 * r, _C + 8 * r + 8)
            hr = [hs_scr[a, re, :] for a in range(_NC)]
            hi = [hs_scr[a, im, :] for a in range(_NC)]
            if r < _C // 16:
                c = [hr[0]] + [hr[a] - hi[a - 1] for a in range(1, _NC)]
                d = [hi[0]] + [hi[a] + hr[a - 1] for a in range(1, _NC)]
            else:
                c = [hr[0]] + [hr[a] + hi[a - 1] for a in range(1, _NC)]
                d = [hi[0]] + [hi[a] - hr[a - 1] for a in range(1, _NC)]
            ur = [u_scr[a, re, :] for a in range(_NC)]
            ui = [u_scr[a, im, :] for a in range(_NC)]
            k1 = _causal_conv([ur[a] + ui[a] for a in range(_NC)], c)
            k2 = _causal_conv(ur, [d[a] - c[a] for a in range(_NC)])
            for a in range(_NC):
                y_scr[a, im, :] = k1[a] + k2[a]
            k3 = _causal_conv(ui, [c[a] + d[a] for a in range(_NC)])
            for a in range(_NC):
                y_scr[a, re, :] = k1[a] - k3[a]

        def project(p, n):
            xs = x_rows(p * n, n)
            wt = jnp.concatenate([_as_bf16(wt_w[g]) for g in range(_NG)], axis=1)
            qv = _dot_nt(wt, xs)
            wk = jnp.concatenate(
                [_as_bf16(wk_w[j, g * 64:(g + 1) * 64, :]) for g in range(_NG)], axis=0)
            kn = _dot(xs, wk)
            row = pl.ds(pl.multiple_of(j * _C, _C), _C)
            for t in range(n // _C):
                tt = p * (n // _C) + t
                qt = qv[0:_C, t * _C:(t + 1) * _C]
                qs_scr[tt, row, :] = (qt * q_scale).astype(_BF16)
                if tt >= _L // _C:
                    pq_scr[tt - _L // _C, row, :] = _phi(qt).astype(_BF16)
                vt_scr[tt, row, :] = qv[_C:2 * _C, t * _C:(t + 1) * _C].astype(_BF16)
            kn_scr[j, p * n:(p + 1) * n, :] = kn.astype(_BF16)
            if p * n < _S - _L:
                pk_scr[j, p * n:(p + 1) * n, :] = _phi(kn).astype(_BF16)

        piece = 256
        n_piece = _S // piece
        for p in range(n_piece):
            project(p, piece)
            for r in range(p * 16 // n_piece, (p + 1) * 16 // n_piece):
                cross_chunk(r)

        ftm = ft_buf[...]
        for a in range(_NC):
            rows = slice(a * _C // 2, (a + 1) * _C // 2)
            y = _dot(ftm, y_scr[a].astype(_BF16)) * (1.0 / _C)
            y = y + _as_bf16(kv_w[rows, :]).astype(_F32) * tile(skip)
            outa_buf[j, a * _C:(a + 1) * _C, :] = (
                _as_bf16(qa_w[j, rows, :]).astype(_F32) * y).astype(_BF16)
        outa_copy(j).start()
        return carry

    lax.fori_loop(0, _NG, phase1, 0)

    qs_w = qs_scr.bitcast(_U32)
    pq_w = pq_scr.bitcast(_U32)
    vt_w = vt_scr.bitcast(_U32)
    kn_w = kn_scr.bitcast(_U32)
    pk_w = pk_scr.bitcast(_U32)
    kwin_w = kwin_scr.bitcast(_U32)
    pkwin_w = pkwin_scr.bitcast(_U32)
    tiles = _L // _C

    def phase2(m, carry):
        first = m * (4 * _DH)
        off = lax.rem(first, _C)
        g0 = lax.div(first, _C)
        g1 = jnp.minimum(g0 + 1, _NG - 1)
        shift_l = lax.rem(_C - off, _C)

        def window(src, dst, n_rows):
            lane = lax.broadcasted_iota(jnp.int32, (n_rows // 2, _C), 1)
            w = jnp.where(lane >= off, src[g0], src[g1])
            dst[...] = pltpu.roll(w, shift_l, 1)

        window(kn_w, kwin_w, _S)
        window(pk_w, pkwin_w, _S - _L)

        wrow = pl.ds(pl.multiple_of(m * 40, 8), 40)
        row16 = lax.broadcasted_iota(jnp.int32, (16, _C), 0)
        in_head = [(row16 >= 2 * hh) & (row16 < 2 * hh + 10) for hh in range(4)]
        key_id = lax.broadcasted_iota(jnp.int32, (_C, _C), 0)
        qry_id = lax.broadcasted_iota(jnp.int32, (_C, _C), 1)
        causal = key_id <= qry_id
        row8 = lax.broadcasted_iota(jnp.int32, (8, _C), 0)
        low_half = row8 < 4
        gates = [gate_scr[m * 4 + hh] for hh in range(4)]
        ones_w = jnp.full((8, _C), _ONES_BF16_PAIR, _U32)

        mrow = lax.broadcasted_iota(jnp.int32, (96, _C), 0)
        mlane = lax.broadcasted_iota(jnp.int32, (96, _C), 1)
        mmask = jnp.zeros((96, _C), jnp.bool_)
        for hh in range(4):
            lanes = (mlane >= _DH * hh) & (mlane < _DH * (hh + 1))
            rows = ((mrow >= _DH * hh) & (mrow < _DH * (hh + 1))) | (mrow == 80 + hh)
            mmask = mmask | (lanes & rows)

        def spread(f):
            return jnp.concatenate(
                [f[0], f[0], jnp.where(low_half, f[0], f[1]), f[1], f[1],
                 f[2], f[2], jnp.where(low_half, f[2], f[3]), f[3], f[3]], axis=0)

        def v_words(s, t):
            return vt_w[tiles * s + t, wrow, :]

        def memory_update(s, mem):
            vall = jnp.concatenate(
                [_as_bf16(jnp.concatenate([v_words(s, t), ones_w], axis=0))
                 for t in range(tiles)], axis=1)
            pk = _as_bf16(pkwin_w[s * _L // 2:(s + 1) * _L // 2, :])
            upd = jnp.where(mmask, _dot(vall, pk), 0.0)
            return upd if mem is None else mem + upd

        def memory_read(s, mem):
            pq = jnp.concatenate(
                [_as_bf16(jnp.concatenate(
                    [pq_w[tiles * (s - 1) + i, wrow, :], jnp.zeros((24, _C), _U32)], axis=0))
                 for i in range(tiles)], axis=1)
            got = _dot(mem.astype(_BF16), pq)
            for i in range(tiles):
                gi = got[:, i * _C:(i + 1) * _C]
                fac = [gates[hh] / (jnp.broadcast_to(gi[80 + hh:81 + hh], (8, _C)) + 1e-6)
                       for hh in range(4)]
                amem_scr[s % 2, i] = gi[0:80] * spread(fac)

        def masked_queries(s, i):
            qq = qs_w[tiles * s + i, wrow, :]
            cols = []
            for hh in range(4):
                qh = jnp.where(in_head[hh], qq[8 * hh:8 * hh + 16], jnp.uint32(0))
                parts = [jnp.zeros((8 * hh, _C), _U32)] if hh > 0 else []
                parts += [qh, jnp.zeros((48 - 8 * hh, _C), _U32)]
                cols.append(_as_bf16(jnp.concatenate(parts, axis=0)))
            return jnp.concatenate(cols, axis=1)

        units = [(s, i, t) for s in range(_NSEG) for i in range(tiles) for t in range(i + 1)]
        run_max, row_max, accs = None, {}, None
        mem = None
        for n in range(len(units) + _LAG):
            if n < len(units):
                s, i, t = units[n]
                if i == 0 and s > 0:
                    mem = memory_update(s - 1, mem)
                if i == 1 and s > 0:
                    memory_read(s, mem)
                lo = (s * _L + t * _C) // 2
                sc = _dot(_as_bf16(kwin_w[lo:lo + _C // 2, :]), masked_queries(s, i))
                cur = []
                for hh in range(4):
                    sh = sc[:, hh * _C:(hh + 1) * _C]
                    if t == i:
                        sh = jnp.where(causal, sh, -jnp.inf)
                    s_scr[n % (_LAG + 1), hh] = sh
                    part = jnp.max(sh.reshape(_C // 8, 8, _C), axis=0)
                    cur.append(part if t == 0 else jnp.maximum(run_max[hh], part))
                run_max = cur
                if t == i:
                    row_max[(s, i)] = [
                        jnp.broadcast_to(jnp.max(c, axis=0, keepdims=True), (8, _C)) for c in cur]
            if n >= _LAG:
                s, i, t = units[n - _LAG]
                vq = v_words(s, t)
                cur = []
                for hh in range(4):
                    mx = jnp.tile(row_max[(s, i)][hh], (_C // 8, 1))
                    p = jnp.exp2(s_scr[(n - _LAG) % (_LAG + 1), hh] - mx).astype(_BF16)
                    vh = _as_bf16(jnp.where(in_head[hh], vq[8 * hh:8 * hh + 16],
                                            jnp.uint32(_ONES_BF16_PAIR)))
                    pv = _dot(vh, p)
                    cur.append(pv if t == 0 else accs[hh] + pv)
                accs = cur
                if t == i:
                    norm = [(1.0 - gates[hh]) / (accs[hh][24:32] if hh < 2 else accs[hh][0:8])
                            for hh in range(4)]
                    o = jnp.concatenate(
                        [accs[0][0:16], jnp.where(low_half, accs[0][16:24], accs[1][0:8]),
                         accs[1][8:24], accs[2][8:24],
                         jnp.where(low_half, accs[2][24:32], accs[3][8:16]), accs[3][16:32]],
                        axis=0) * spread(norm)
                    if s > 0:
                        o = o + amem_scr[s % 2, i]
                    ot_scr[tiles * s + i, pl.ds(pl.multiple_of(first, 16), 80), :] = (
                        o.astype(_BF16))
        return carry

    lax.fori_loop(0, _NQ, phase2, 0)

    wo_copy.wait()
    for p in range(_NSEG):
        ot = jnp.concatenate([ot_scr[tiles * p + t] for t in range(tiles)], axis=1)
        outb_buf[p] = _dot_tn(ot, wo_buf[...]).astype(_BF16)
        outb_copy(p).start()
    for j in range(_NG):
        outa_copy(j).wait()
    for p in range(_NSEG):
        outb_copy(p).wait()


@jax.jit
def pallas_concat_heads__ssm_conv_h3__memory_aug_infini_attn__prompt_kernel(
    A_q: jax.Array,
    A_k: jax.Array,
    A_v: jax.Array,
    A_shift_k: jax.Array,
    A_ssm_k: jax.Array,
    A_ssm_D: jax.Array,
    B_x: jax.Array,
    B_wq: jax.Array,
    B_wk: jax.Array,
    B_wv: jax.Array,
    B_wo: jax.Array,
    B_beta: jax.Array,
):
    assert A_q.shape == (1, _S, _D) and B_x.shape == (1, _S, _D)
    assert A_shift_k.shape == (_D, _KS) and B_beta.shape == (_H,)
    fmat = _dft_matrix()
    f_fwd = fmat.astype(_BF16)
    f_inv = np.ascontiguousarray(fmat.T).astype(_BF16)

    vmem = pltpu.VMEM
    dma = pltpu.SemaphoreType.DMA
    scratch = [
        vmem((_NG, _S, _C), _BF16),
        vmem((_NG, _S, _C), _BF16),
        vmem((_NG, _S, _C), _BF16),
        vmem((_NG, _C, _S), _BF16),
        vmem((_NG, _S, _C), _BF16),
        vmem((_NG, _D, _C), _BF16),
        vmem((_NG, _D, _C), _BF16),
        vmem((_NG, _D, _C), _BF16),
        vmem((_D, _D), _BF16),
        vmem((_KS, _D), _BF16),
        vmem((_D,), _BF16),
        vmem((_H,), _BF16),
        vmem((2 * _C, _C), _BF16),
        vmem((_C, 2 * _C), _BF16),
        vmem((_NG, _KS + 1, 8, _C), _F32),
        vmem((_H, 8, _C), _F32),
        vmem((_S + 8, _C), _F32),
        vmem((_S, _C), _BF16),
        vmem((_NC, 2 * _C, _C), _F32),
        vmem((_NC, 2 * _C, _C), _F32),
        vmem((_NC, 2 * _C, _C), _F32),
        vmem((_NG, _S, _C), _BF16),
        vmem((_NG, 2 * _C, _C), _BF16),
        vmem((_NC, _D, _C), _BF16),
        vmem((_NC - _L // _C, _D, _C), _BF16),
        vmem((_NC, _D, _C), _BF16),
        vmem((_NG, _S, _C), _BF16),
        vmem((_NG, _S - _L, _C), _BF16),
        vmem((_S, _C), _BF16),
        vmem((_S - _L, _C), _BF16),
        vmem((_LAG + 1, 4, _C, _C), _F32),
        vmem((2, 4, 80, _C), _F32),
        vmem((_NC, _D, _C), _BF16),
        vmem((_NSEG, _L, _D), _BF16),
        dma((7, _NG)), dma((_NG,)), dma((6,)), dma((_NG,)), dma((_NSEG,)),
    ]
    out = pl.pallas_call(
        _kernel,
        out_shape=jax.ShapeDtypeStruct((_S, 2 * _D), _BF16),
        in_specs=[pl.BlockSpec(memory_space=pl.ANY)] * 14,
        out_specs=pl.BlockSpec(memory_space=pl.ANY),
        scratch_shapes=scratch,
        compiler_params=pltpu.CompilerParams(vmem_limit_bytes=100 * 1024 * 1024),
        name="h3_infini",
    )(A_q.reshape(_S, _D), A_k.reshape(_S, _D), A_v.reshape(_S, _D), A_shift_k.T,
      A_ssm_k, A_ssm_D, B_x.reshape(_S, _D), B_wq, B_wk, B_wv, B_wo, B_beta,
      f_fwd, f_inv)
    return out.reshape(1, _S, 2 * _D)
```

```python
import math

import numpy as np
import jax
import jax.numpy as jnp
from jax import lax
import jax.experimental.pallas as pl
import jax.experimental.pallas.tpu as pltpu

_S = 2048
_D = 640
_H = 32
_DH = 20
_NSEG = 4
_L = _S // _NSEG
_C = 128
_NC = _S // _C
_NG = _D // _C
_NQ = _H // 4
_KS = 4
_LAG = 2

_F32 = jnp.float32
_BF16 = jnp.bfloat16
_U32 = jnp.uint32
_LOG2E = math.log2(math.e)
_ONES_BF16_PAIR = 0x3F803F80


def _dft_matrix():
    k = np.concatenate([np.arange(0, _C, 2), np.arange(1, _C, 2)])
    ang = np.pi * np.outer(2 * k + 1, np.arange(_C)) / (2 * _C)
    return np.concatenate([np.cos(ang), -np.sin(ang)], axis=0).astype(np.float32)


def _dot(a, b):
    return jnp.dot(a, b, preferred_element_type=_F32)


def _dot_nt(a, b):
    return lax.dot_general(a, b, (((1,), (1,)), ((), ())), preferred_element_type=_F32)


def _dot_tn(a, b):
    return lax.dot_general(a, b, (((0,), (0,)), ((), ())), preferred_element_type=_F32)


def _as_bf16(words):
    return pltpu.bitcast(words, _BF16)


def _phi(t):
    return jnp.where(t > 0, t + 1.0, jnp.exp(t))


def _causal_conv(u, h):
    out = []
    for a in range(len(u)):
        acc = u[a] * h[0]
        for j in range(1, a + 1):
            acc = acc + u[a - j] * h[j]
        out.append(acc)
    return out


def _kernel(q_hbm, k_hbm, v_hbm, shift_hbm, h_hbm, d_hbm, x_hbm,
            wq_hbm, wk_hbm, wv_hbm, wo_hbm, beta_hbm, f_hbm, ft_hbm, out_hbm,
            qa_buf, ka_buf, va_buf, h_buf, x_buf, wq_buf, wk_buf, wv_buf, wo_buf,
            shift_buf, d_buf, beta_buf, f_buf, ft_buf,
            par_scr, gate_scr, kpad_scr, kv_scr, u_scr, hs_scr, y_scr, outa_buf,
            wt_scr, qs_scr, pq_scr, vt_scr, kn_scr, pk_scr, kwin_scr, pkwin_scr,
            s_scr, amem_scr, ot_scr, outb_buf,
            sem_a, sem_b, sem_c, sem_oa, sem_ob):

    def col(j):
        return pl.ds(pl.multiple_of(j * _C, _C), _C)

    def group_copies(j):
        cp = pltpu.make_async_copy
        return [
            cp(k_hbm.at[:, col(j)], ka_buf.at[j], sem_a.at[0, j]),
            cp(v_hbm.at[:, col(j)], va_buf.at[j], sem_a.at[1, j]),
            cp(h_hbm.at[col(j), :], h_buf.at[j], sem_a.at[2, j]),
            cp(wq_hbm.at[:, col(j)], wq_buf.at[j], sem_a.at[3, j]),
            cp(wk_hbm.at[:, col(j)], wk_buf.at[j], sem_a.at[4, j]),
            cp(wv_hbm.at[:, col(j)], wv_buf.at[j], sem_a.at[5, j]),
            cp(q_hbm.at[:, col(j)], qa_buf.at[j], sem_a.at[6, j]),
        ]

    def outa_copy(j):
        return pltpu.make_async_copy(outa_buf.at[j], out_hbm.at[:, col(j)], sem_oa.at[j])

    def outb_copy(p):
        return pltpu.make_async_copy(
            outb_buf.at[p], out_hbm.at[pl.ds(p * _L, _L), pl.ds(_D, _D)], sem_ob.at[p])

    small = [
        pltpu.make_async_copy(shift_hbm, shift_buf, sem_c.at[0]),
        pltpu.make_async_copy(d_hbm, d_buf, sem_c.at[1]),
        pltpu.make_async_copy(beta_hbm, beta_buf, sem_c.at[2]),
        pltpu.make_async_copy(f_hbm, f_buf, sem_c.at[3]),
        pltpu.make_async_copy(ft_hbm, ft_buf, sem_c.at[4]),
    ]
    x_copies = [
        pltpu.make_async_copy(x_hbm.at[:, pl.ds(g * _C, _C)], x_buf.at[g], sem_b.at[g])
        for g in range(_NG)
    ]
    wo_copy = pltpu.make_async_copy(wo_hbm, wo_buf, sem_c.at[5])

    for c in small:
        c.start()
    for c in group_copies(0):
        c.start()
    for c in x_copies:
        c.start()
    for c in small:
        c.wait()

    shift = shift_buf[...].astype(_F32)
    dvec = d_buf[...].astype(_F32).reshape(1, _D)
    for g in range(_NG):
        sl = slice(g * _C, (g + 1) * _C)
        for t in range(_KS):
            par_scr[g, t] = jnp.broadcast_to(shift[t:t + 1, sl], (8, _C))
        par_scr[g, _KS] = jnp.broadcast_to(dvec[:, sl], (8, _C))
    beta = beta_buf[...].astype(_F32).reshape(1, _H)
    gate = 1.0 / (1.0 + jnp.exp(-beta))
    for hd in range(_H):
        gate_scr[hd] = jnp.broadcast_to(gate[:, hd:hd + 1], (8, _C))
    kpad_scr[0:8, :] = jnp.zeros((8, _C), _F32)

    for c in x_copies:
        c.wait()

    x_w = x_buf.bitcast(_U32)
    f_w = f_buf.bitcast(_U32)
    ka_w = ka_buf.bitcast(_U32)
    va_w = va_buf.bitcast(_U32)
    qa_w = qa_buf.bitcast(_U32)
    kv_w = kv_scr.bitcast(_U32)
    wt_w = wt_scr.bitcast(_U32)
    wk_w = wk_buf.bitcast(_U32)
    q_scale = _DH ** -0.5 * _LOG2E

    def x_rows(lo, n):
        return jnp.concatenate(
            [_as_bf16(x_w[g, lo // 2:(lo + n) // 2, :]) for g in range(_NG)], axis=1)

    def phase1(j, carry):
        @pl.when(j + 1 < _NG)
        def _():
            for c in group_copies(j + 1):
                c.start()

        @pl.when(j == _NG - 1)
        def _():
            wo_copy.start()

        for c in group_copies(j):
            c.wait()

        for w_buf, base in ((wq_buf, 0), (wv_buf, _C)):
            wt = w_buf[j].T
            for g in range(_NG):
                wt_scr[g, base:base + _C, :] = wt[:, g * _C:(g + 1) * _C]

        taps = [par_scr[j, t] for t in range(_KS)]
        skip = par_scr[j, _KS]
        fmat = _as_bf16(f_w[...])

        def tile(v):
            return jnp.tile(v, (_C // 8, 1))

        for a in range(_NC):
            rows = slice(a * _C // 2, (a + 1) * _C // 2)
            kpad_scr[8 + a * _C:8 + (a + 1) * _C, :] = _as_bf16(ka_w[j, rows, :]).astype(_F32)
        for a in range(_NC):
            rows = slice(a * _C // 2, (a + 1) * _C // 2)
            ks = kpad_scr[8 + a * _C:8 + (a + 1) * _C, :] * tile(taps[0])
            for t in range(1, _KS):
                ks = ks + kpad_scr[8 + a * _C - t:8 + (a + 1) * _C - t, :] * tile(taps[t])
            kv = (ks * _as_bf16(va_w[j, rows, :]).astype(_F32)).astype(_BF16)
            kv_scr[a * _C:(a + 1) * _C, :] = kv
            u_scr[a] = _dot(fmat, kv)
            hs_scr[a] = _dot_nt(fmat, h_buf[j, :, a * _C:(a + 1) * _C])

        def cross_chunk(r):
            re, im = slice(8 * r, 8 * r + 8), slice(_C + 8 * r, _C + 8 * r + 8)
            hr = [hs_scr[a, re, :] for a in range(_NC)]
            hi = [hs_scr[a, im, :] for a in range(_NC)]
            if r < _C // 16:
                c = [hr[0]] + [hr[a] - hi[a - 1] for a in range(1, _NC)]
                d = [hi[0]] + [hi[a] + hr[a - 1] for a in range(1, _NC)]
            else:
                c = [hr[0]] + [hr[a] + hi[a - 1] for a in range(1, _NC)]
                d = [hi[0]] + [hi[a] - hr[a - 1] for a in range(1, _NC)]
            ur = [u_scr[a, re, :] for a in range(_NC)]
            ui = [u_scr[a, im, :] for a in range(_NC)]
            k1 = _causal_conv([ur[a] + ui[a] for a in range(_NC)], c)
            k2 = _causal_conv(ur, [d[a] - c[a] for a in range(_NC)])
            for a in range(_NC):
                y_scr[a, im, :] = k1[a] + k2[a]
            k3 = _causal_conv(ui, [c[a] + d[a] for a in range(_NC)])
            for a in range(_NC):
                y_scr[a, re, :] = k1[a] - k3[a]

        def project(p, n):
            xs = x_rows(p * n, n)
            wt = jnp.concatenate([_as_bf16(wt_w[g]) for g in range(_NG)], axis=1)
            qv = _dot_nt(wt, xs)
            wk = jnp.concatenate(
                [_as_bf16(wk_w[j, g * 64:(g + 1) * 64, :]) for g in range(_NG)], axis=0)
            kn = _dot(xs, wk)
            row = pl.ds(pl.multiple_of(j * _C, _C), _C)
            for t in range(n // _C):
                tt = p * (n // _C) + t
                qt = qv[0:_C, t * _C:(t + 1) * _C]
                qs_scr[tt, row, :] = (qt * q_scale).astype(_BF16)
                if tt >= _L // _C:
                    pq_scr[tt - _L // _C, row, :] = _phi(qt).astype(_BF16)
                vt_scr[tt, row, :] = qv[_C:2 * _C, t * _C:(t + 1) * _C].astype(_BF16)
            kn_scr[j, p * n:(p + 1) * n, :] = kn.astype(_BF16)
            if p * n < _S - _L:
                pk_scr[j, p * n:(p + 1) * n, :] = _phi(kn).astype(_BF16)

        piece = 256
        n_piece = _S // piece
        for p in range(n_piece):
            project(p, piece)
            for r in range(p * 16 // n_piece, (p + 1) * 16 // n_piece):
                cross_chunk(r)

        ftm = ft_buf[...]
        for a in range(_NC):
            rows = slice(a * _C // 2, (a + 1) * _C // 2)
            y = _dot(ftm, y_scr[a].astype(_BF16)) * (1.0 / _C)
            y = y + _as_bf16(kv_w[rows, :]).astype(_F32) * tile(skip)
            outa_buf[j, a * _C:(a + 1) * _C, :] = (
                _as_bf16(qa_w[j, rows, :]).astype(_F32) * y).astype(_BF16)
        outa_copy(j).start()
        return carry

    lax.fori_loop(0, _NG, phase1, 0)

    qs_w = qs_scr.bitcast(_U32)
    pq_w = pq_scr.bitcast(_U32)
    vt_w = vt_scr.bitcast(_U32)
    kn_w = kn_scr.bitcast(_U32)
    pk_w = pk_scr.bitcast(_U32)
    kwin_w = kwin_scr.bitcast(_U32)
    pkwin_w = pkwin_scr.bitcast(_U32)
    tiles = _L // _C

    def phase2(m, carry):
        first = m * (4 * _DH)
        off = lax.rem(first, _C)
        g0 = lax.div(first, _C)
        g1 = jnp.minimum(g0 + 1, _NG - 1)
        shift_l = lax.rem(_C - off, _C)

        def window(src, dst, n_rows):
            lane = lax.broadcasted_iota(jnp.int32, (n_rows // 2, _C), 1)
            w = jnp.where(lane >= off, src[g0], src[g1])
            dst[...] = pltpu.roll(w, shift_l, 1)

        window(kn_w, kwin_w, _S)
        window(pk_w, pkwin_w, _S - _L)

        wrow = pl.ds(pl.multiple_of(m * 40, 8), 40)
        row16 = lax.broadcasted_iota(jnp.int32, (16, _C), 0)
        in_head = [(row16 >= 2 * hh) & (row16 < 2 * hh + 10) for hh in range(4)]
        key_id = lax.broadcasted_iota(jnp.int32, (_C, _C), 0)
        qry_id = lax.broadcasted_iota(jnp.int32, (_C, _C), 1)
        causal = key_id <= qry_id
        row8 = lax.broadcasted_iota(jnp.int32, (8, _C), 0)
        low_half = row8 < 4
        gates = [gate_scr[m * 4 + hh] for hh in range(4)]
        ones_w = jnp.full((8, _C), _ONES_BF16_PAIR, _U32)

        mrow = lax.broadcasted_iota(jnp.int32, (96, _C), 0)
        mlane = lax.broadcasted_iota(jnp.int32, (96, _C), 1)
        mmask = jnp.zeros((96, _C), jnp.bool_)
        for hh in range(4):
            lanes = (mlane >= _DH * hh) & (mlane < _DH * (hh + 1))
            rows = ((mrow >= _DH * hh) & (mrow < _DH * (hh + 1))) | (mrow == 80 + hh)
            mmask = mmask | (lanes & rows)

        def spread(f):
            return jnp.concatenate(
                [f[0], f[0], jnp.where(low_half, f[0], f[1]), f[1], f[1],
                 f[2], f[2], jnp.where(low_half, f[2], f[3]), f[3], f[3]], axis=0)

        def v_words(s, t):
            return vt_w[tiles * s + t, wrow, :]

        def memory_update(s, mem):
            vall = jnp.concatenate(
                [_as_bf16(jnp.concatenate([v_words(s, t), ones_w], axis=0))
                 for t in range(tiles)], axis=1)
            pk = _as_bf16(pkwin_w[s * _L // 2:(s + 1) * _L // 2, :])
            upd = jnp.where(mmask, _dot(vall, pk), 0.0)
            return upd if mem is None else mem + upd

        def memory_read(s, mem):
            pq = jnp.concatenate(
                [_as_bf16(jnp.concatenate(
                    [pq_w[tiles * (s - 1) + i, wrow, :], jnp.zeros((24, _C), _U32)], axis=0))
                 for i in range(tiles)], axis=1)
            got = _dot(mem.astype(_BF16), pq)
            for i in range(tiles):
                gi = got[:, i * _C:(i + 1) * _C]
                fac = [gates[hh] / (jnp.broadcast_to(gi[80 + hh:81 + hh], (8, _C)) + 1e-6)
                       for hh in range(4)]
                amem_scr[s % 2, i] = gi[0:80] * spread(fac)

        def masked_queries(s, i):
            qq = qs_w[tiles * s + i, wrow, :]
            cols = []
            for hh in range(4):
                qh = jnp.where(in_head[hh], qq[8 * hh:8 * hh + 16], jnp.uint32(0))
                parts = [jnp.zeros((8 * hh, _C), _U32)] if hh > 0 else []
                parts += [qh, jnp.zeros((48 - 8 * hh, _C), _U32)]
                cols.append(_as_bf16(jnp.concatenate(parts, axis=0)))
            return jnp.concatenate(cols, axis=1)

        units = [(s, i, t) for s in range(_NSEG) for i in range(tiles) for t in range(i + 1)]
        run_max, accs = {}, None
        mem = None
        for n in range(len(units) + _LAG):
            if n < len(units):
                s, i, t = units[n]
                if i == 0 and s > 0:
                    mem = memory_update(s - 1, mem)
                if i == 1 and s > 0:
                    memory_read(s, mem)
                lo = (s * _L + t * _C) // 2
                sc = _dot(_as_bf16(kwin_w[lo:lo + _C // 2, :]), masked_queries(s, i))
                cur = []
                for hh in range(4):
                    sh = sc[:, hh * _C:(hh + 1) * _C]
                    if t == i:
                        sh = jnp.where(causal, sh, -jnp.inf)
                    s_scr[n % (_LAG + 1), hh] = sh
                    part = jnp.max(sh, axis=0, keepdims=True)
                    cur.append(part if t == 0 else jnp.maximum(run_max[n - 1][hh], part))
                run_max[n] = cur
            if n >= _LAG:
                u = n - _LAG
                s, i, t = units[u]
                vq = v_words(s, t)
                cur = []
                for hh in range(4):
                    mx = run_max[u][hh]
                    p = jnp.exp2(s_scr[u % (_LAG + 1), hh] - mx).astype(_BF16)
                    vh = _as_bf16(jnp.where(in_head[hh], vq[8 * hh:8 * hh + 16],
                                            jnp.uint32(_ONES_BF16_PAIR)))
                    pv = _dot(vh, p)
                    if t > 0:
                        pv = pv + accs[hh] * jnp.exp2(run_max[u - 1][hh] - mx)
                    cur.append(pv)
                accs = cur
                if t == i:
                    norm = [(1.0 - gates[hh]) / (accs[hh][24:32] if hh < 2 else accs[hh][0:8])
                            for hh in range(4)]
                    o = jnp.concatenate(
                        [accs[0][0:16], jnp.where(low_half, accs[0][16:24], accs[1][0:8]),
                         accs[1][8:24], accs[2][8:24],
                         jnp.where(low_half, accs[2][24:32], accs[3][8:16]), accs[3][16:32]],
                        axis=0) * spread(norm)
                    if s > 0:
                        o = o + amem_scr[s % 2, i]
                    ot_scr[tiles * s + i, pl.ds(pl.multiple_of(first, 16), 80), :] = (
                        o.astype(_BF16))
        return carry

    lax.fori_loop(0, _NQ, phase2, 0)

    wo_copy.wait()
    for p in range(_NSEG):
        ot = jnp.concatenate([ot_scr[tiles * p + t] for t in range(tiles)], axis=1)
        outb_buf[p] = _dot_tn(ot, wo_buf[...]).astype(_BF16)
        outb_copy(p).start()
    for j in range(_NG):
        outa_copy(j).wait()
    for p in range(_NSEG):
        outb_copy(p).wait()


@jax.jit
def pallas_concat_heads__ssm_conv_h3__memory_aug_infini_attn__prompt_kernel(
    A_q: jax.Array,
    A_k: jax.Array,
    A_v: jax.Array,
    A_shift_k: jax.Array,
    A_ssm_k: jax.Array,
    A_ssm_D: jax.Array,
    B_x: jax.Array,
    B_wq: jax.Array,
    B_wk: jax.Array,
    B_wv: jax.Array,
    B_wo: jax.Array,
    B_beta: jax.Array,
):
    assert A_q.shape == (1, _S, _D) and B_x.shape == (1, _S, _D)
    assert A_shift_k.shape == (_D, _KS) and B_beta.shape == (_H,)
    fmat = _dft_matrix()
    f_fwd = fmat.astype(_BF16)
    f_inv = np.ascontiguousarray(fmat.T).astype(_BF16)

    vmem = pltpu.VMEM
    dma = pltpu.SemaphoreType.DMA
    scratch = [
        vmem((_NG, _S, _C), _BF16),
        vmem((_NG, _S, _C), _BF16),
        vmem((_NG, _S, _C), _BF16),
        vmem((_NG, _C, _S), _BF16),
        vmem((_NG, _S, _C), _BF16),
        vmem((_NG, _D, _C), _BF16),
        vmem((_NG, _D, _C), _BF16),
        vmem((_NG, _D, _C), _BF16),
        vmem((_D, _D), _BF16),
        vmem((_KS, _D), _BF16),
        vmem((_D,), _BF16),
        vmem((_H,), _BF16),
        vmem((2 * _C, _C), _BF16),
        vmem((_C, 2 * _C), _BF16),
        vmem((_NG, _KS + 1, 8, _C), _F32),
        vmem((_H, 8, _C), _F32),
        vmem((_S + 8, _C), _F32),
        vmem((_S, _C), _BF16),
        vmem((_NC, 2 * _C, _C), _F32),
        vmem((_NC, 2 * _C, _C), _F32),
        vmem((_NC, 2 * _C, _C), _F32),
        vmem((_NG, _S, _C), _BF16),
        vmem((_NG, 2 * _C, _C), _BF16),
        vmem((_NC, _D, _C), _BF16),
        vmem((_NC - _L // _C, _D, _C), _BF16),
        vmem((_NC, _D, _C), _BF16),
        vmem((_NG, _S, _C), _BF16),
        vmem((_NG, _S - _L, _C), _BF16),
        vmem((_S, _C), _BF16),
        vmem((_S - _L, _C), _BF16),
        vmem((_LAG + 1, 4, _C, _C), _F32),
        vmem((2, 4, 80, _C), _F32),
        vmem((_NC, _D, _C), _BF16),
        vmem((_NSEG, _L, _D), _BF16),
        dma((7, _NG)), dma((_NG,)), dma((6,)), dma((_NG,)), dma((_NSEG,)),
    ]
    out = pl.pallas_call(
        _kernel,
        out_shape=jax.ShapeDtypeStruct((_S, 2 * _D), _BF16),
        in_specs=[pl.BlockSpec(memory_space=pl.ANY)] * 14,
        out_specs=pl.BlockSpec(memory_space=pl.ANY),
        scratch_shapes=scratch,
        compiler_params=pltpu.CompilerParams(vmem_limit_bytes=100 * 1024 * 1024),
        name="h3_infini",
    )(A_q.reshape(_S, _D), A_k.reshape(_S, _D), A_v.reshape(_S, _D), A_shift_k.T,
      A_ssm_k, A_ssm_D, B_x.reshape(_S, _D), B_wq, B_wk, B_wv, B_wo, B_beta,
      f_fwd, f_inv)
    return out.reshape(1, _S, 2 * _D)
```

```python
import functools
import math

import numpy as np
import jax
import jax.numpy as jnp
from jax import lax
import jax.experimental.pallas as pl
import jax.experimental.pallas.tpu as pltpu

_S = 2048
_D = 640
_H = 32
_DH = 20
_NSEG = 4
_L = _S // _NSEG
_C = 128
_NC = _S // _C
_NG = _D // _C
_NQ = _H // 4
_KS = 4
_PIECE = 256
_X_SPLIT = (0, 256, 512, 1024, 2048)
_LAG = 2

_F32 = jnp.float32
_BF16 = jnp.bfloat16
_U32 = jnp.uint32
_LOG2E = math.log2(math.e)
_ONES_BF16_PAIR = 0x3F803F80


def _dft_matrix():
    k = np.concatenate([np.arange(0, _C, 2), np.arange(1, _C, 2)])
    ang = np.pi * np.outer(2 * k + 1, np.arange(_C)) / (2 * _C)
    return np.concatenate([np.cos(ang), -np.sin(ang)], axis=0).astype(np.float32)


def _dot(a, b):
    return jnp.dot(a, b, preferred_element_type=_F32)


def _dot_nt(a, b):
    return lax.dot_general(a, b, (((1,), (1,)), ((), ())), preferred_element_type=_F32)


def _dot_tn(a, b):
    return lax.dot_general(a, b, (((0,), (0,)), ((), ())), preferred_element_type=_F32)


def _as_bf16(words):
    return pltpu.bitcast(words, _BF16)


def _phi(t):
    return jnp.where(t > 0, t + 1.0, jnp.exp(t))


def _kernel(q_hbm, k_hbm, v_hbm, shift_hbm, h_hbm, d_hbm, x_hbm,
            wq_hbm, wk_hbm, wv_hbm, wo_hbm, beta_hbm, f_hbm, ft_hbm, out_hbm,
            qa_buf, ka_buf, va_buf, h_buf, x_buf, wq_buf, wk_buf, wv_buf, wo_buf,
            shift_buf, d_buf, beta_buf, f_buf, ft_buf,
            par_scr, gate_scr, kpad_scr, kv_scr, outa_buf,
            wt_scr, z_scr, zero_smem, qs_scr, pq_scr, vt_scr, kn_scr, pk_scr, kwin_scr, pkwin_scr,
            s_scr, amem_scr, ot_scr, outb_buf,
            sem_a, sem_w, sem_x, sem_c, sem_oa, sem_ob):

    cp = pltpu.make_async_copy

    def col(j):
        return pl.ds(j * _C if isinstance(j, int) else pl.multiple_of(j * _C, _C), _C)

    def conv_copies(j):
        return [cp(k_hbm.at[:, col(j)], ka_buf.at[j], sem_a.at[0, j]),
                cp(v_hbm.at[:, col(j)], va_buf.at[j], sem_a.at[1, j]),
                cp(h_hbm.at[col(j), :], h_buf.at[j], sem_a.at[2, j])]

    def gate_copy(j):
        return cp(q_hbm.at[:, col(j)], qa_buf.at[j], sem_a.at[3, j])

    def weight_copies(j):
        return [cp(wk_hbm.at[:, col(j)], wk_buf.at[j], sem_w.at[0, j]),
                cp(wq_hbm.at[:, col(j)], wq_buf.at[j], sem_w.at[1, j]),
                cp(wv_hbm.at[:, col(j)], wv_buf.at[j], sem_w.at[2, j])]

    def x_copies(p):
        rows = pl.ds(_X_SPLIT[p], _X_SPLIT[p + 1] - _X_SPLIT[p])
        return [cp(x_hbm.at[rows, col(g)], x_buf.at[g, rows], sem_x.at[p]) for g in range(_NG)]

    def outa_copy(j):
        return cp(outa_buf.at[j], out_hbm.at[:, col(j)], sem_oa.at[j])

    def outb_copy(p):
        return cp(outb_buf.at[p], out_hbm.at[pl.ds(p * _L, _L), pl.ds(_D, _D)], sem_ob.at[p])

    small = [cp(shift_hbm, shift_buf, sem_c.at[0]), cp(d_hbm, d_buf, sem_c.at[1]),
             cp(beta_hbm, beta_buf, sem_c.at[2]), cp(f_hbm, f_buf, sem_c.at[3]),
             cp(ft_hbm, ft_buf, sem_c.at[4])]
    wo_copy = cp(wo_hbm, wo_buf, sem_c.at[5])

    def start(copies):
        for c in copies:
            c.start()

    def wait(copies):
        for c in copies:
            c.wait()

    x_w = x_buf.bitcast(_U32)
    f_w = f_buf.bitcast(_U32)
    ka_w = ka_buf.bitcast(_U32)
    va_w = va_buf.bitcast(_U32)
    qa_w = qa_buf.bitcast(_U32)
    wk_w = wk_buf.bitcast(_U32)
    q_scale = _DH ** -0.5 * _LOG2E
    wt_w = wt_scr.bitcast(_U32)
    kv_w = kv_scr.bitcast(_U32)

    def tile(v):
        return jnp.tile(v, (_C // 8, 1))

    def words(a):
        return slice(a * _C // 2, (a + 1) * _C // 2)

    def transpose_weights(j):
        for w_buf, base in ((wq_buf, 0), (wv_buf, _C)):
            wt = w_buf[j].T
            for g in range(_NG):
                wt_scr[j, g, base:base + _C, :] = wt[:, g * _C:(g + 1) * _C]

    def project(j, lo, n):
        xs = jnp.concatenate(
            [_as_bf16(x_w[g, lo // 2:(lo + n) // 2, :]) for g in range(_NG)], axis=1)
        wk = jnp.concatenate([_as_bf16(wk_w[j, words(g), :]) for g in range(_NG)], axis=0)
        kn = _dot(xs, wk)
        kn_scr[j, lo:lo + n, :] = kn.astype(_BF16)
        if lo < _S - _L:
            pk_scr[j, lo:lo + n, :] = _phi(kn).astype(_BF16)
        wt = jnp.concatenate([_as_bf16(wt_w[j, g]) for g in range(_NG)], axis=1)
        qv = _dot_nt(wt, xs)
        for t in range(n // _C):
            tt = lo // _C + t
            qt = qv[0:_C, t * _C:(t + 1) * _C]
            qs_scr[tt, col(j), :] = (qt * q_scale).astype(_BF16)
            if tt >= _L // _C:
                pq_scr[tt - _L // _C, col(j), :] = _phi(qt).astype(_BF16)
            vt_scr[tt, col(j), :] = qv[_C:2 * _C, t * _C:(t + 1) * _C].astype(_BF16)

    def spectrum(j, a):
        fmat = _as_bf16(f_w[...])
        z_scr[1, a] = _dot_nt(fmat, h_buf[j, :, a * _C:(a + 1) * _C])
        lo = 8 + a * _C
        kpad_scr[lo:lo + _C, :] = _as_bf16(ka_w[j, words(a), :]).astype(_F32)
        ks = kpad_scr[lo:lo + _C, :] * tile(par_scr[j, 0])
        for t in range(1, _KS):
            ks = ks + kpad_scr[lo - t:lo + _C - t, :] * tile(par_scr[j, t])
        kv = (ks * _as_bf16(va_w[j, words(a), :]).astype(_F32)).astype(_BF16)
        kv_scr[a * _C:(a + 1) * _C, :] = kv
        z_scr[0, a] = _dot(fmat, kv)

    def cross_chunks():
        z_st, z_ld = zero_smem[0], zero_smem[1]
        nb = 4
        for r in range(_NC):
            re, im = slice(8 * r, 8 * r + 8), slice(_C + 8 * r, _C + 8 * r + 8)

            def triple(which, a):
                x, y = z_scr[z_ld + which, a, re, :], z_scr[z_ld + which, a, im, :]
                return x, y, x + y

            prev = None
            for lo in range(0, _NC, nb):
                u, acc = {}, {}
                for t in range(lo + nb):
                    h = triple(1, t)
                    for a in range(max(lo, t), lo + nb):
                        if a - t not in u:
                            u[a - t] = triple(0, a - t)
                        prod = [x * y for x, y in zip(u[a - t], h)]
                        acc[a] = prod if t == 0 else [x + y for x, y in zip(acc[a], prod)]
                outs = []
                for a in range(lo, lo + nb):
                    k1, k2, k3 = acc[a]
                    yr, yi = cur = (k1 - k2, k3 - k1 - k2)
                    if prev is not None:
                        yr, yi = ((yr - prev[1], yi + prev[0]) if r < _C // 16
                                  else (yr + prev[1], yi - prev[0]))
                    prev = cur
                    outs.append((a, yr, yi))
                for a, yr, yi in outs:
                    z_scr[z_st + 2, a, re, :] = yr
                    z_scr[z_st + 2, a, im, :] = yi

    def finish(j, a):
        y = _dot(ft_buf[...], z_scr[zero_smem[1] + 2, a].astype(_BF16)) * (1.0 / _C)
        y = y + _as_bf16(kv_w[words(a), :]).astype(_F32) * tile(par_scr[j, _KS])
        outa_buf[j, a * _C:(a + 1) * _C, :] = (
            _as_bf16(qa_w[j, words(a), :]).astype(_F32) * y).astype(_BF16)

    def convolve(j, fillers, lead):
        for n, job in enumerate(fillers[:-1]):
            if n == lead:
                for a in range(_NC):
                    spectrum(j, a)
            job()
        cross_chunks()
        for a in range(_NC):
            finish(j, a)
        outa_copy(j).start()
        fillers[-1]()

    start(weight_copies(0))
    start(x_copies(0))
    start(small)
    start(x_copies(1))
    wait(small)
    shift = shift_buf[...].astype(_F32)
    dvec = d_buf[...].astype(_F32).reshape(1, _D)
    for g in range(_NG):
        sl = slice(g * _C, (g + 1) * _C)
        for t in range(_KS):
            par_scr[g, t] = jnp.broadcast_to(shift[t:t + 1, sl], (8, _C))
        par_scr[g, _KS] = jnp.broadcast_to(dvec[:, sl], (8, _C))
    beta = beta_buf[...].astype(_F32).reshape(1, _H)
    gate = 1.0 / (1.0 + jnp.exp(-beta))
    for hd in range(_H):
        gate_scr[hd] = jnp.broadcast_to(gate[:, hd:hd + 1], (8, _C))
    kpad_scr[0:8, :] = jnp.zeros((8, _C), _F32)
    zero_smem[0] = 0
    zero_smem[1] = 0
    wait(weight_copies(0))
    transpose_weights(0)

    n_load = len(_X_SPLIT) - 1
    for p in range(n_load):
        if p + 2 < n_load:
            start(x_copies(p + 2))
        if p == n_load - 2:
            start(weight_copies(1) + conv_copies(0))
        if p == n_load - 1:
            start([gate_copy(0)] + weight_copies(2))
        wait(x_copies(p))
        if p == n_load - 1:
            wait(weight_copies(1))
            transpose_weights(1)
        for lo in range(_X_SPLIT[p], _X_SPLIT[p + 1], _PIECE):
            project(0, lo, _PIECE)

    def phase1(j, carry):
        start(conv_copies(j + 1) + [gate_copy(j + 1)])

        @pl.when(j + 2 < _NG)
        def _():
            wait(weight_copies(j + 2))

        @pl.when(j + 3 < _NG)
        def _():
            start(weight_copies(j + 3))

        @pl.when(j == _NG - 2)
        def _():
            wo_copy.start()

        wait(conv_copies(j) + [gate_copy(j)])
        jobs = [functools.partial(project, j + 1, lo, _PIECE) for lo in range(0, _S, _PIECE)]
        convolve(j, jobs + [lambda: transpose_weights(jnp.minimum(j + 2, _NG - 1))], 1)
        return carry

    lax.fori_loop(0, _NG - 1, phase1, 0)

    qs_w = qs_scr.bitcast(_U32)
    pq_w = pq_scr.bitcast(_U32)
    vt_w = vt_scr.bitcast(_U32)
    kn_w = kn_scr.bitcast(_U32)
    pk_w = pk_scr.bitcast(_U32)
    kwin_w = kwin_scr.bitcast(_U32)
    pkwin_w = pkwin_scr.bitcast(_U32)
    tiles = _L // _C

    def phase2(m, carry):
        first = m * (4 * _DH)
        off = lax.rem(first, _C)
        g0 = lax.div(first, _C)
        g1 = jnp.minimum(g0 + 1, _NG - 1)
        shift_l = lax.rem(_C - off, _C)

        def window(src, dst, n_rows):
            lane = lax.broadcasted_iota(jnp.int32, (n_rows // 2, _C), 1)
            w = jnp.where(lane >= off, src[g0], src[g1])
            dst[...] = pltpu.roll(w, shift_l, 1)

        window(kn_w, kwin_w, _S)
        window(pk_w, pkwin_w, _S - _L)

        wrow = pl.ds(pl.multiple_of(m * 40, 8), 40)
        row16 = lax.broadcasted_iota(jnp.int32, (16, _C), 0)
        in_head = [(row16 >= 2 * hh) & (row16 < 2 * hh + 10) for hh in range(4)]
        key_id = lax.broadcasted_iota(jnp.int32, (_C, _C), 0)
        qry_id = lax.broadcasted_iota(jnp.int32, (_C, _C), 1)
        causal = key_id <= qry_id
        row8 = lax.broadcasted_iota(jnp.int32, (8, _C), 0)
        low_half = row8 < 4
        gates = [gate_scr[m * 4 + hh] for hh in range(4)]
        ones_w = jnp.full((8, _C), _ONES_BF16_PAIR, _U32)

        mrow = lax.broadcasted_iota(jnp.int32, (96, _C), 0)
        mlane = lax.broadcasted_iota(jnp.int32, (96, _C), 1)
        mmask = jnp.zeros((96, _C), jnp.bool_)
        for hh in range(4):
            lanes = (mlane >= _DH * hh) & (mlane < _DH * (hh + 1))
            rows = ((mrow >= _DH * hh) & (mrow < _DH * (hh + 1))) | (mrow == 80 + hh)
            mmask = mmask | (lanes & rows)

        def spread(f):
            return jnp.concatenate(
                [f[0], f[0], jnp.where(low_half, f[0], f[1]), f[1], f[1],
                 f[2], f[2], jnp.where(low_half, f[2], f[3]), f[3], f[3]], axis=0)

        def v_words(s, t):
            return vt_w[tiles * s + t, wrow, :]

        def memory_update(s, mem):
            vall = jnp.concatenate(
                [_as_bf16(jnp.concatenate([v_words(s, t), ones_w], axis=0))
                 for t in range(tiles)], axis=1)
            pk = _as_bf16(pkwin_w[s * _L // 2:(s + 1) * _L // 2, :])
            upd = jnp.where(mmask, _dot(vall, pk), 0.0)
            return upd if mem is None else mem + upd

        def memory_read(s, mem):
            pq = jnp.concatenate(
                [_as_bf16(jnp.concatenate(
                    [pq_w[tiles * (s - 1) + i, wrow, :], jnp.zeros((24, _C), _U32)], axis=0))
                 for i in range(tiles)], axis=1)
            got = _dot(mem.astype(_BF16), pq)
            for i in range(tiles):
                gi = got[:, i * _C:(i + 1) * _C]
                fac = [gates[hh] / (jnp.broadcast_to(gi[80 + hh:81 + hh], (8, _C)) + 1e-6)
                       for hh in range(4)]
                amem_scr[s % 2, i] = gi[0:80] * spread(fac)

        def masked_queries(s, i):
            qq = qs_w[tiles * s + i, wrow, :]
            cols = []
            for hh in range(4):
                qh = jnp.where(in_head[hh], qq[8 * hh:8 * hh + 16], jnp.uint32(0))
                parts = [jnp.zeros((8 * hh, _C), _U32)] if hh > 0 else []
                parts += [qh, jnp.zeros((48 - 8 * hh, _C), _U32)]
                cols.append(_as_bf16(jnp.concatenate(parts, axis=0)))
            return jnp.concatenate(cols, axis=1)

        units = [(s, i, t) for s in range(_NSEG) for i in range(tiles) for t in range(i + 1)]
        run_max, accs = {}, None
        mem = None
        for n in range(len(units) + _LAG):
            if n < len(units):
                s, i, t = units[n]
                if i == 0 and s > 0:
                    mem = memory_update(s - 1, mem)
                if i == 1 and s > 0:
                    memory_read(s, mem)
                lo = (s * _L + t * _C) // 2
                sc = _dot(_as_bf16(kwin_w[lo:lo + _C // 2, :]), masked_queries(s, i))
                cur = []
                for hh in range(4):
                    sh = sc[:, hh * _C:(hh + 1) * _C]
                    if t == i:
                        sh = jnp.where(causal, sh, -jnp.inf)
                    s_scr[n % (_LAG + 1), hh] = sh
                    part = jnp.max(sh, axis=0, keepdims=True)
                    cur.append(part if t == 0 else jnp.maximum(run_max[n - 1][hh], part))
                run_max[n] = cur
            if n >= _LAG:
                u = n - _LAG
                s, i, t = units[u]
                vq = v_words(s, t)
                cur = []
                for hh in range(4):
                    mx = run_max[u][hh]
                    p = jnp.exp2(s_scr[u % (_LAG + 1), hh] - mx).astype(_BF16)
                    vh = _as_bf16(jnp.where(in_head[hh], vq[8 * hh:8 * hh + 16],
                                            jnp.uint32(_ONES_BF16_PAIR)))
                    pv = _dot(vh, p)
                    if t > 0:
                        pv = pv + accs[hh] * jnp.exp2(run_max[u - 1][hh] - mx)
                    cur.append(pv)
                accs = cur
                if t == i:
                    norm = [(1.0 - gates[hh]) / (accs[hh][24:32] if hh < 2 else accs[hh][0:8])
                            for hh in range(4)]
                    o = jnp.concatenate(
                        [accs[0][0:16], jnp.where(low_half, accs[0][16:24], accs[1][0:8]),
                         accs[1][8:24], accs[2][8:24],
                         jnp.where(low_half, accs[2][24:32], accs[3][8:16]), accs[3][16:32]],
                        axis=0) * spread(norm)
                    if s > 0:
                        o = o + amem_scr[s % 2, i]
                    ot_scr[tiles * s + i, pl.ds(pl.multiple_of(first, 16), 80), :] = (
                        o.astype(_BF16))
        return carry

    lax.fori_loop(0, _NQ, phase2, 0)

    def output_projection(p):
        ot = jnp.concatenate([ot_scr[tiles * p + t] for t in range(tiles)], axis=1)
        outb_buf[p] = _dot_tn(ot, wo_buf[...]).astype(_BF16)

    def last_piece():
        start([outb_copy(p) for p in range(_NSEG - 1)])
        output_projection(_NSEG - 1)
        outb_copy(_NSEG - 1).start()

    wait([wo_copy, gate_copy(_NG - 1)] + conv_copies(_NG - 1))
    convolve(_NG - 1, [functools.partial(output_projection, p) for p in range(_NSEG - 1)]
             + [last_piece], 0)
    wait([outa_copy(j) for j in range(_NG)] + [outb_copy(p) for p in range(_NSEG)])


@jax.jit
def pallas_concat_heads__ssm_conv_h3__memory_aug_infini_attn__prompt_kernel(
    A_q: jax.Array,
    A_k: jax.Array,
    A_v: jax.Array,
    A_shift_k: jax.Array,
    A_ssm_k: jax.Array,
    A_ssm_D: jax.Array,
    B_x: jax.Array,
    B_wq: jax.Array,
    B_wk: jax.Array,
    B_wv: jax.Array,
    B_wo: jax.Array,
    B_beta: jax.Array,
):
    assert A_q.shape == (1, _S, _D) and B_x.shape == (1, _S, _D)
    assert A_shift_k.shape == (_D, _KS) and B_beta.shape == (_H,)
    fmat = _dft_matrix()
    f_fwd = fmat.astype(_BF16)
    f_inv = np.ascontiguousarray(fmat.T).astype(_BF16)

    vmem = pltpu.VMEM
    dma = pltpu.SemaphoreType.DMA
    scratch = [
        vmem((_NG, _S, _C), _BF16),
        vmem((_NG, _S, _C), _BF16),
        vmem((_NG, _S, _C), _BF16),
        vmem((_NG, _C, _S), _BF16),
        vmem((_NG, _S, _C), _BF16),
        vmem((_NG, _D, _C), _BF16),
        vmem((_NG, _D, _C), _BF16),
        vmem((_NG, _D, _C), _BF16),
        vmem((_D, _D), _BF16),
        vmem((_KS, _D), _BF16),
        vmem((_D,), _BF16),
        vmem((_H,), _BF16),
        vmem((2 * _C, _C), _BF16),
        vmem((_C, 2 * _C), _BF16),
        vmem((_NG, _KS + 1, 8, _C), _F32),
        vmem((_H, 8, _C), _F32),
        vmem((_S + 8, _C), _F32),
        vmem((_S, _C), _BF16),
        vmem((_NG, _S, _C), _BF16),
        vmem((_NG, _NG, 2 * _C, _C), _BF16),
        vmem((3, _NC, 2 * _C, _C), _F32),
        pltpu.SMEM((2,), jnp.int32),
        vmem((_NC, _D, _C), _BF16),
        vmem((_NC - _L // _C, _D, _C), _BF16),
        vmem((_NC, _D, _C), _BF16),
        vmem((_NG, _S, _C), _BF16),
        vmem((_NG, _S - _L, _C), _BF16),
        vmem((_S, _C), _BF16),
        vmem((_S - _L, _C), _BF16),
        vmem((_LAG + 1, 4, _C, _C), _F32),
        vmem((2, 4, 80, _C), _F32),
        vmem((_NC, _D, _C), _BF16),
        vmem((_NSEG, _L, _D), _BF16),
        dma((4, _NG)), dma((3, _NG)), dma((len(_X_SPLIT) - 1,)), dma((6,)), dma((_NG,)),
        dma((_NSEG,)),
    ]
    out = pl.pallas_call(
        _kernel,
        out_shape=jax.ShapeDtypeStruct((_S, 2 * _D), _BF16),
        in_specs=[pl.BlockSpec(memory_space=pl.ANY)] * 14,
        out_specs=pl.BlockSpec(memory_space=pl.ANY),
        scratch_shapes=scratch,
        compiler_params=pltpu.CompilerParams(vmem_limit_bytes=100 * 1024 * 1024),
        name="h3_infini",
    )(A_q.reshape(_S, _D), A_k.reshape(_S, _D), A_v.reshape(_S, _D), A_shift_k.T,
      A_ssm_k, A_ssm_D, B_x.reshape(_S, _D), B_wq, B_wk, B_wv, B_wo, B_beta,
      f_fwd, f_inv)
    return out.reshape(1, _S, 2 * _D)
```

```python
import functools
import math

import numpy as np
import jax
import jax.numpy as jnp
from jax import lax
import jax.experimental.pallas as pl
import jax.experimental.pallas.tpu as pltpu

_S = 2048
_D = 640
_H = 32
_DH = 20
_NSEG = 4
_L = _S // _NSEG
_C = 128
_NC = _S // _C
_NG = _D // _C
_NQ = _H // 4
_KS = 4
_PIECE = 256
_X_SPLIT = (0, 256, 512, 1024, 2048)
_OUT_SPLIT = (0, 512, 1024, 1536, 1792, 2048)
_OUT_OVERLAP = 2
_LAG = 2

_F32 = jnp.float32
_BF16 = jnp.bfloat16
_U32 = jnp.uint32
_LOG2E = math.log2(math.e)
_ONES_BF16_PAIR = 0x3F803F80


def _dft_matrix():
    k = np.concatenate([np.arange(0, _C, 2), np.arange(1, _C, 2)])
    ang = np.pi * np.outer(2 * k + 1, np.arange(_C)) / (2 * _C)
    return np.concatenate([np.cos(ang), -np.sin(ang)], axis=0).astype(np.float32)


def _dot(a, b):
    return jnp.dot(a, b, preferred_element_type=_F32)


def _dot_nt(a, b):
    return lax.dot_general(a, b, (((1,), (1,)), ((), ())), preferred_element_type=_F32)


def _dot_tn(a, b):
    return lax.dot_general(a, b, (((0,), (0,)), ((), ())), preferred_element_type=_F32)


def _as_bf16(words):
    return pltpu.bitcast(words, _BF16)


def _phi(t):
    return jnp.where(t > 0, t + 1.0, jnp.exp(t))


def _kernel(q_hbm, k_hbm, v_hbm, shift_hbm, h_hbm, d_hbm, x_hbm,
            wq_hbm, wk_hbm, wv_hbm, wo_hbm, beta_hbm, f_hbm, ft_hbm, zero_hbm,
            out_hbm,
            qa_buf, ka_buf, va_buf, h_buf, x_buf, wq_buf, wk_buf, wv_buf, wo_buf,
            shift_buf, d_buf, beta_buf, f_buf, ft_buf,
            par_scr, gate_scr, kpad_scr, kv_scr, outa_buf,
            wt_scr, z_scr, zero_smem, qs_scr, pq_scr, vt_scr, kn_scr, pk_scr, kwin_scr, pkwin_scr,
            s_scr, amem_scr, ot_scr, outb_buf,
            sem_a, sem_w, sem_x, sem_c, sem_oa, sem_ob):

    cp = pltpu.make_async_copy

    def col(j):
        return pl.ds(j * _C if isinstance(j, int) else pl.multiple_of(j * _C, _C), _C)

    def conv_copies(j):
        return [cp(k_hbm.at[:, col(j)], ka_buf.at[j], sem_a.at[0, j]),
                cp(v_hbm.at[:, col(j)], va_buf.at[j], sem_a.at[1, j]),
                cp(h_hbm.at[col(j), :], h_buf.at[j], sem_a.at[2, j])]

    def gate_copy(j):
        return cp(q_hbm.at[:, col(j)], qa_buf.at[j], sem_a.at[3, j])

    def weight_copies(j):
        return [cp(wk_hbm.at[:, col(j)], wk_buf.at[j], sem_w.at[0, j]),
                cp(wq_hbm.at[:, col(j)], wq_buf.at[j], sem_w.at[1, j]),
                cp(wv_hbm.at[:, col(j)], wv_buf.at[j], sem_w.at[2, j])]

    def x_copies(p):
        rows = pl.ds(_X_SPLIT[p], _X_SPLIT[p + 1] - _X_SPLIT[p])
        return [cp(x_hbm.at[rows, col(g)], x_buf.at[g, rows], sem_x.at[p]) for g in range(_NG)]

    def outa_copy(j):
        return cp(outa_buf.at[j], out_hbm.at[:, col(j)], sem_oa.at[j])

    def outb_copy(p):
        rows = pl.ds(_OUT_SPLIT[p], _OUT_SPLIT[p + 1] - _OUT_SPLIT[p])
        return cp(outb_buf.at[rows], out_hbm.at[rows, pl.ds(_D, _D)], sem_ob.at[p])

    small = [cp(shift_hbm, shift_buf, sem_c.at[0]), cp(d_hbm, d_buf, sem_c.at[1]),
             cp(beta_hbm, beta_buf, sem_c.at[2]), cp(f_hbm, f_buf, sem_c.at[3]),
             cp(ft_hbm, ft_buf, sem_c.at[4]), cp(zero_hbm, zero_smem, sem_c.at[5])]
    wo_copy = cp(wo_hbm, wo_buf, sem_c.at[6])

    def start(copies):
        for c in copies:
            c.start()

    def wait(copies):
        for c in copies:
            c.wait()

    x_w = x_buf.bitcast(_U32)
    f_w = f_buf.bitcast(_U32)
    ka_w = ka_buf.bitcast(_U32)
    va_w = va_buf.bitcast(_U32)
    qa_w = qa_buf.bitcast(_U32)
    wk_w = wk_buf.bitcast(_U32)
    q_scale = _DH ** -0.5 * _LOG2E
    wt_w = wt_scr.bitcast(_U32)
    kv_w = kv_scr.bitcast(_U32)

    def tile(v):
        return jnp.tile(v, (_C // 8, 1))

    def words(a):
        return slice(a * _C // 2, (a + 1) * _C // 2)

    def transpose_weights(j):
        for w_buf, base in ((wq_buf, 0), (wv_buf, _C)):
            wt = w_buf[j].T
            for g in range(_NG):
                wt_scr[j, g, base:base + _C, :] = wt[:, g * _C:(g + 1) * _C]

    def project(j, lo, n):
        xs = jnp.concatenate(
            [_as_bf16(x_w[g, lo // 2:(lo + n) // 2, :]) for g in range(_NG)], axis=1)
        wk = jnp.concatenate([_as_bf16(wk_w[j, words(g), :]) for g in range(_NG)], axis=0)
        kn = _dot(xs, wk)
        kn_scr[j, lo:lo + n, :] = kn.astype(_BF16)
        if lo < _S - _L:
            pk_scr[j, lo:lo + n, :] = _phi(kn).astype(_BF16)
        wt = jnp.concatenate([_as_bf16(wt_w[j, g]) for g in range(_NG)], axis=1)
        qv = _dot_nt(wt, xs)
        for t in range(n // _C):
            tt = lo // _C + t
            qt = qv[0:_C, t * _C:(t + 1) * _C]
            qs_scr[tt, col(j), :] = (qt * q_scale).astype(_BF16)
            if tt >= _L // _C:
                pq_scr[tt - _L // _C, col(j), :] = _phi(qt).astype(_BF16)
            vt_scr[tt, col(j), :] = qv[_C:2 * _C, t * _C:(t + 1) * _C].astype(_BF16)

    def spectrum(j, a):
        fmat = _as_bf16(f_w[...])
        z_scr[1, a] = _dot_nt(fmat, h_buf[j, :, a * _C:(a + 1) * _C])
        lo = 8 + a * _C
        kpad_scr[lo:lo + _C, :] = _as_bf16(ka_w[j, words(a), :]).astype(_F32)
        ks = kpad_scr[lo:lo + _C, :] * tile(par_scr[j, 0])
        for t in range(1, _KS):
            ks = ks + kpad_scr[lo - t:lo + _C - t, :] * tile(par_scr[j, t])
        kv = (ks * _as_bf16(va_w[j, words(a), :]).astype(_F32)).astype(_BF16)
        kv_scr[a * _C:(a + 1) * _C, :] = kv
        z_scr[0, a] = _dot(fmat, kv)

    def cross_chunks():
        z_st, z_ld = zero_smem[0], zero_smem[1]
        nb = 4
        for r in range(_NC):
            re, im = slice(8 * r, 8 * r + 8), slice(_C + 8 * r, _C + 8 * r + 8)

            def triple(which, a):
                x, y = z_scr[z_ld + which, a, re, :], z_scr[z_ld + which, a, im, :]
                return x, y, x + y

            prev = None
            for lo in range(0, _NC, nb):
                u, acc = {}, {}
                for t in range(lo + nb):
                    h = triple(1, t)
                    for a in range(max(lo, t), lo + nb):
                        if a - t not in u:
                            u[a - t] = triple(0, a - t)
                        prod = [x * y for x, y in zip(u[a - t], h)]
                        acc[a] = prod if t == 0 else [x + y for x, y in zip(acc[a], prod)]
                outs = []
                for a in range(lo, lo + nb):
                    k1, k2, k3 = acc[a]
                    yr, yi = cur = (k1 - k2, k3 - k1 - k2)
                    if prev is not None:
                        yr, yi = ((yr - prev[1], yi + prev[0]) if r < _C // 16
                                  else (yr + prev[1], yi - prev[0]))
                    prev = cur
                    outs.append((a, yr, yi))
                for a, yr, yi in outs:
                    z_scr[z_st + 2, a, re, :] = yr
                    z_scr[z_st + 2, a, im, :] = yi

    def finish(j, a):
        y = _dot(ft_buf[...], z_scr[zero_smem[1] + 2, a].astype(_BF16)) * (1.0 / _C)
        y = y + _as_bf16(kv_w[words(a), :]).astype(_F32) * tile(par_scr[j, _KS])
        outa_buf[j, a * _C:(a + 1) * _C, :] = (
            _as_bf16(qa_w[j, words(a), :]).astype(_F32) * y).astype(_BF16)

    def convolve(j, fillers, lead):
        for n, job in enumerate(fillers):
            if n == lead:
                for a in range(_NC):
                    spectrum(j, a)
            job()
        cross_chunks()
        for a in range(_NC):
            finish(j, a)
        outa_copy(j).start()

    def group_copies(j):
        return conv_copies(j) + [gate_copy(j)] + (weight_copies(j + 1) if j + 1 < _NG else [])

    start(small + weight_copies(0) + x_copies(0))
    wait(small)
    start(x_copies(1) + x_copies(2))
    later = {1: x_copies(3), 2: group_copies(0)[2:3] + weight_copies(1),
             3: group_copies(0)[:2] + [gate_copy(0)]}
    wait(weight_copies(0))
    for p in range(len(_X_SPLIT) - 1):
        start(later.get(p, []))
        wait(x_copies(p))
        if p == 0:
            transpose_weights(0)
        if p == 1:
            shift = shift_buf[...].astype(_F32)
            dvec = d_buf[...].astype(_F32).reshape(1, _D)
            for g in range(_NG):
                sl = slice(g * _C, (g + 1) * _C)
                for t in range(_KS):
                    par_scr[g, t] = jnp.broadcast_to(shift[t:t + 1, sl], (8, _C))
                par_scr[g, _KS] = jnp.broadcast_to(dvec[:, sl], (8, _C))
            beta = beta_buf[...].astype(_F32).reshape(1, _H)
            gate = 1.0 / (1.0 + jnp.exp(-beta))
            for hd in range(_H):
                gate_scr[hd] = jnp.broadcast_to(gate[:, hd:hd + 1], (8, _C))
            kpad_scr[0:8, :] = jnp.zeros((8, _C), _F32)
        for lo in range(_X_SPLIT[p], _X_SPLIT[p + 1], _PIECE):
            project(0, lo, _PIECE)

    for j in range(_NG - 1):
        start(group_copies(j + 1) + ([wo_copy] if j == 0 else []))
        wait(group_copies(j))
        transpose_weights(j + 1)
        jobs = [functools.partial(project, j + 1, lo, _PIECE) for lo in range(0, _S, _PIECE)]
        convolve(j, jobs, 1)

    qs_w = qs_scr.bitcast(_U32)
    pq_w = pq_scr.bitcast(_U32)
    vt_w = vt_scr.bitcast(_U32)
    kn_w = kn_scr.bitcast(_U32)
    pk_w = pk_scr.bitcast(_U32)
    kwin_w = kwin_scr.bitcast(_U32)
    pkwin_w = pkwin_scr.bitcast(_U32)
    tiles = _L // _C

    row16 = lax.broadcasted_iota(jnp.int32, (16, _C), 0)
    row8 = lax.broadcasted_iota(jnp.int32, (8, _C), 0)

    def in_head(hh):
        return (row16 >= 2 * hh) & (row16 < 2 * hh + 10)

    def spread(f):
        return jnp.concatenate(
            [f[0], f[0], jnp.where(row8 < 4, f[0], f[1]), f[1], f[1],
             f[2], f[2], jnp.where(row8 < 4, f[2], f[3]), f[3], f[3]], axis=0)

    class Quad:
        def __init__(self, m, slot):
            self.m, self.slot = m, slot
            self.wrow = pl.ds(m * 40, 40)
            self.mem = None
            first = m * (4 * _DH)
            off, g0 = first % _C, first // _C
            g1 = min(g0 + 1, _NG - 1)
            for src, dst, n_rows in ((kn_w, kwin_w, _S), (pk_w, pkwin_w, _S - _L)):
                lane = lax.broadcasted_iota(jnp.int32, (n_rows // 2, _C), 1)
                if off == 0:
                    dst[slot] = src[g0]
                else:
                    dst[slot] = pltpu.roll(jnp.where(lane >= off, src[g0], src[g1]), _C - off, 1)

        def gate(self, hh):
            return gate_scr[self.m * 4 + hh]

        def v_words(self, s, t):
            return vt_w[tiles * s + t, self.wrow, :]

        def memory_update(self, s):
            ones = jnp.full((8, _C), _ONES_BF16_PAIR, _U32)
            v_ext = jnp.concatenate(
                [_as_bf16(jnp.concatenate([self.v_words(s, t), ones], axis=0))
                 for t in range(tiles)], axis=1)
            pk = _as_bf16(pkwin_w[self.slot, s * _L // 2:(s + 1) * _L // 2, :])
            row = lax.broadcasted_iota(jnp.int32, (96, _C), 0)
            lane = lax.broadcasted_iota(jnp.int32, (96, _C), 1)
            keep = jnp.zeros((96, _C), jnp.bool_)
            for hh in range(4):
                rows = ((row >= _DH * hh) & (row < _DH * (hh + 1))) | (row == 80 + hh)
                keep = keep | (rows & (lane >= _DH * hh) & (lane < _DH * (hh + 1)))
            upd = jnp.where(keep, _dot(v_ext, pk), 0.0)
            self.mem = upd if self.mem is None else self.mem + upd

        def memory_read(self, s):
            pq = jnp.concatenate(
                [_as_bf16(jnp.concatenate(
                    [pq_w[tiles * (s - 1) + i, self.wrow, :], jnp.zeros((24, _C), _U32)],
                    axis=0)) for i in range(tiles)], axis=1)
            got = _dot(self.mem.astype(_BF16), pq)
            for i in range(tiles):
                gi = got[:, i * _C:(i + 1) * _C]
                fac = [self.gate(hh) / (jnp.broadcast_to(gi[80 + hh:81 + hh], (8, _C)) + 1e-6)
                       for hh in range(4)]
                amem_scr[s % 2, i] = gi[0:80] * spread(fac)

        def logits(self, s, i, t):
            qq = qs_w[tiles * s + i, self.wrow, :]
            cols = []
            for hh in range(4):
                qh = jnp.where(in_head(hh), qq[8 * hh:8 * hh + 16], jnp.uint32(0))
                parts = [jnp.zeros((8 * hh, _C), _U32)] if hh > 0 else []
                parts += [qh, jnp.zeros((48 - 8 * hh, _C), _U32)]
                cols.append(_as_bf16(jnp.concatenate(parts, axis=0)))
            lo = (s * _L + t * _C) // 2
            keys = _as_bf16(kwin_w[self.slot, lo:lo + _C // 2, :])
            return _dot(keys, jnp.concatenate(cols, axis=1))

        def store(self, s, i, accs):
            norm = [(1.0 - self.gate(hh)) / (accs[hh][24:32] if hh < 2 else accs[hh][0:8])
                    for hh in range(4)]
            o = jnp.concatenate(
                [accs[0][0:16], jnp.where(row8 < 4, accs[0][16:24], accs[1][0:8]),
                 accs[1][8:24], accs[2][8:24],
                 jnp.where(row8 < 4, accs[2][24:32], accs[3][8:16]), accs[3][16:32]],
                axis=0) * spread(norm)
            if s > 0:
                o = o + amem_scr[s % 2, i]
            rows = pl.ds(self.m * (4 * _DH), 4 * _DH)
            ot_scr[tiles * s + i, rows, :] = o.astype(_BF16)

    def attention():
        quads = [Quad(m, m) for m in range(_NQ)]
        units = [(quad, s, i, t) for quad in quads for s in range(_NSEG)
                 for i in range(tiles) for t in range(i + 1)]
        causal = (lax.broadcasted_iota(jnp.int32, (_C, _C), 0)
                  <= lax.broadcasted_iota(jnp.int32, (_C, _C), 1))
        run_max, accs = {}, None
        for n in range(len(units) + _LAG):
            if n < len(units):
                quad, s, i, t = units[n]
                if s > 0 and (i, t) == (0, 0):
                    quad.memory_update(s - 1)
                if s > 0 and (i, t) == (1, 1):
                    quad.memory_read(s)
                sc = quad.logits(s, i, t)
                cur = []
                for hh in range(4):
                    sh = sc[:, hh * _C:(hh + 1) * _C]
                    if t == i:
                        sh = jnp.where(causal, sh, -jnp.inf)
                    s_scr[n % (_LAG + 1), hh] = sh
                    part = jnp.max(sh, axis=0, keepdims=True)
                    cur.append(part if t == 0 else jnp.maximum(run_max[n - 1][hh], part))
                run_max[n] = cur
            if n >= _LAG:
                u = n - _LAG
                quad, s, i, t = units[u]
                vq = quad.v_words(s, t)
                cur = []
                for hh in range(4):
                    mx = run_max[u][hh]
                    p = jnp.exp2(s_scr[u % (_LAG + 1), hh] - mx).astype(_BF16)
                    vh = _as_bf16(jnp.where(in_head(hh), vq[8 * hh:8 * hh + 16],
                                            jnp.uint32(_ONES_BF16_PAIR)))
                    pv = _dot(vh, p)
                    if t > 0:
                        pv = pv + accs[hh] * jnp.exp2(run_max[u - 1][hh] - mx)
                    cur.append(pv)
                accs = cur
                if t == i:
                    quad.store(s, i, accs)

    wo_copy.wait()
    attention()

    def output_projection(p):
        lo, hi = _OUT_SPLIT[p] // _C, _OUT_SPLIT[p + 1] // _C
        ot = jnp.concatenate([ot_scr[t] for t in range(lo, hi)], axis=1)
        outb_buf[lo * _C:hi * _C, :] = _dot_tn(ot, wo_buf[...]).astype(_BF16)
        outb_copy(p).start()

    n_out = len(_OUT_SPLIT) - 1
    wait(group_copies(_NG - 1))
    convolve(_NG - 1, [functools.partial(output_projection, p) for p in range(_OUT_OVERLAP)], 0)
    for p in range(_OUT_OVERLAP, n_out):
        output_projection(p)
    wait([outa_copy(j) for j in range(_NG)] + [outb_copy(p) for p in range(n_out)])


@jax.jit
def pallas_concat_heads__ssm_conv_h3__memory_aug_infini_attn__prompt_kernel(
    A_q: jax.Array,
    A_k: jax.Array,
    A_v: jax.Array,
    A_shift_k: jax.Array,
    A_ssm_k: jax.Array,
    A_ssm_D: jax.Array,
    B_x: jax.Array,
    B_wq: jax.Array,
    B_wk: jax.Array,
    B_wv: jax.Array,
    B_wo: jax.Array,
    B_beta: jax.Array,
):
    assert A_q.shape == (1, _S, _D) and B_x.shape == (1, _S, _D)
    assert A_shift_k.shape == (_D, _KS) and B_beta.shape == (_H,)
    fmat = _dft_matrix()
    f_fwd = fmat.astype(_BF16)
    f_inv = np.ascontiguousarray(fmat.T).astype(_BF16)

    vmem = pltpu.VMEM
    dma = pltpu.SemaphoreType.DMA
    scratch = [
        vmem((_NG, _S, _C), _BF16),
        vmem((_NG, _S, _C), _BF16),
        vmem((_NG, _S, _C), _BF16),
        vmem((_NG, _C, _S), _BF16),
        vmem((_NG, _S, _C), _BF16),
        vmem((_NG, _D, _C), _BF16),
        vmem((_NG, _D, _C), _BF16),
        vmem((_NG, _D, _C), _BF16),
        vmem((_D, _D), _BF16),
        vmem((_KS, _D), _BF16),
        vmem((_D,), _BF16),
        vmem((_H,), _BF16),
        vmem((2 * _C, _C), _BF16),
        vmem((_C, 2 * _C), _BF16),
        vmem((_NG, _KS + 1, 8, _C), _F32),
        vmem((_H, 8, _C), _F32),
        vmem((_S + 8, _C), _F32),
        vmem((_S, _C), _BF16),
        vmem((_NG, _S, _C), _BF16),
        vmem((_NG, _NG, 2 * _C, _C), _BF16),
        vmem((3, _NC, 2 * _C, _C), _F32),
        pltpu.SMEM((_C,), jnp.int32),
        vmem((_NC, _D, _C), _BF16),
        vmem((_NC - _L // _C, _D, _C), _BF16),
        vmem((_NC, _D, _C), _BF16),
        vmem((_NG, _S, _C), _BF16),
        vmem((_NG, _S - _L, _C), _BF16),
        vmem((_NQ, _S, _C), _BF16),
        vmem((_NQ, _S - _L, _C), _BF16),
        vmem((_LAG + 1, 4, _C, _C), _F32),
        vmem((2, 4, 80, _C), _F32),
        vmem((_NC, _D, _C), _BF16),
        vmem((_S, _D), _BF16),
        dma((4, _NG)), dma((3, _NG)), dma((len(_X_SPLIT) - 1,)), dma((7,)), dma((_NG,)),
        dma((len(_OUT_SPLIT) - 1,)),
    ]
    out = pl.pallas_call(
        _kernel,
        out_shape=jax.ShapeDtypeStruct((_S, 2 * _D), _BF16),
        in_specs=[pl.BlockSpec(memory_space=pl.ANY)] * 15,
        out_specs=pl.BlockSpec(memory_space=pl.ANY),
        scratch_shapes=scratch,
        compiler_params=pltpu.CompilerParams(vmem_limit_bytes=100 * 1024 * 1024),
        name="h3_infini",
    )(A_q.reshape(_S, _D), A_k.reshape(_S, _D), A_v.reshape(_S, _D), A_shift_k.T,
      A_ssm_k, A_ssm_D, B_x.reshape(_S, _D), B_wq, B_wk, B_wv, B_wo, B_beta,
      f_fwd, f_inv, np.zeros((_C,), np.int32))
    return out.reshape(1, _S, 2 * _D)
```

```python
import functools
import math

import numpy as np
import jax
import jax.numpy as jnp
from jax import lax
import jax.experimental.pallas as pl
import jax.experimental.pallas.tpu as pltpu

_S = 2048
_D = 640
_H = 32
_DH = 20
_NSEG = 4
_L = _S // _NSEG
_C = 128
_NC = _S // _C
_NG = _D // _C
_NQ = _H // 4
_KS = 4
_PIECE = 256
_X_SPLIT = (0, 256, 512, 1024, 2048)
_OUT_SPLIT = (0, 512, 1024, 1536, 1792, 2048)
_OUT_OVERLAP = 2
_LAG = 2

_F32 = jnp.float32
_BF16 = jnp.bfloat16
_U32 = jnp.uint32
_LOG2E = math.log2(math.e)
_ONES_BF16_PAIR = 0x3F803F80


def _dft_matrix():
    k = np.concatenate([np.arange(0, _C, 2), np.arange(1, _C, 2)])
    ang = np.pi * np.outer(2 * k + 1, np.arange(_C)) / (2 * _C)
    return np.concatenate([np.cos(ang), -np.sin(ang)], axis=0).astype(np.float32)


def _dot(a, b):
    return jnp.dot(a, b, preferred_element_type=_F32)


def _dot_nt(a, b):
    return lax.dot_general(a, b, (((1,), (1,)), ((), ())), preferred_element_type=_F32)


def _dot_tn(a, b):
    return lax.dot_general(a, b, (((0,), (0,)), ((), ())), preferred_element_type=_F32)


def _as_bf16(words):
    return pltpu.bitcast(words, _BF16)


def _phi(t):
    return jnp.where(t > 0, t + 1.0, jnp.exp(t))


def _kernel(q_hbm, k_hbm, v_hbm, shift_hbm, h_hbm, d_hbm, x_hbm,
            wq_hbm, wk_hbm, wv_hbm, wo_hbm, beta_hbm, f_hbm, ft_hbm, out_hbm,
            qa_buf, ka_buf, va_buf, h_buf, x_buf, wq_buf, wk_buf, wv_buf, wo_buf,
            shift_buf, d_buf, beta_buf, f_buf, ft_buf,
            par_scr, gate_scr, kpad_scr, kv_scr, outa_buf,
            wt_scr, z_scr, zero_smem, qs_scr, pq_scr, vt_scr, kn_scr, pk_scr, kwin_scr, pkwin_scr,
            s_scr, amem_scr, ot_scr, outb_buf,
            sem_a, sem_w, sem_x, sem_c, sem_oa, sem_ob):

    cp = pltpu.make_async_copy

    def col(j):
        return pl.ds(j * _C if isinstance(j, int) else pl.multiple_of(j * _C, _C), _C)

    def conv_copies(j):
        return [cp(k_hbm.at[:, col(j)], ka_buf.at[j], sem_a.at[0, j]),
                cp(v_hbm.at[:, col(j)], va_buf.at[j], sem_a.at[1, j]),
                cp(h_hbm.at[col(j), :], h_buf.at[j], sem_a.at[2, j])]

    def gate_copy(j):
        return cp(q_hbm.at[:, col(j)], qa_buf.at[j], sem_a.at[3, j])

    def weight_copies(j):
        return [cp(wk_hbm.at[:, col(j)], wk_buf.at[j], sem_w.at[0, j]),
                cp(wq_hbm.at[:, col(j)], wq_buf.at[j], sem_w.at[1, j]),
                cp(wv_hbm.at[:, col(j)], wv_buf.at[j], sem_w.at[2, j])]

    def x_copies(p):
        rows = pl.ds(_X_SPLIT[p], _X_SPLIT[p + 1] - _X_SPLIT[p])
        return [cp(x_hbm.at[rows, col(g)], x_buf.at[g, rows], sem_x.at[p]) for g in range(_NG)]

    def outa_copy(j):
        return cp(outa_buf.at[j], out_hbm.at[:, col(j)], sem_oa.at[j])

    def outb_copy(p):
        rows = pl.ds(_OUT_SPLIT[p], _OUT_SPLIT[p + 1] - _OUT_SPLIT[p])
        return cp(outb_buf.at[rows], out_hbm.at[rows, pl.ds(_D, _D)], sem_ob.at[p])

    small = [cp(shift_hbm, shift_buf, sem_c.at[0]), cp(d_hbm, d_buf, sem_c.at[1]),
             cp(beta_hbm, beta_buf, sem_c.at[2])]
    dft_copies = [cp(f_hbm, f_buf, sem_c.at[3]), cp(ft_hbm, ft_buf, sem_c.at[4])]
    wo_copy = cp(wo_hbm, wo_buf, sem_c.at[5])

    def start(copies):
        for c in copies:
            c.start()

    def wait(copies):
        for c in copies:
            c.wait()

    x_w = x_buf.bitcast(_U32)
    f_w = f_buf.bitcast(_U32)
    ka_w = ka_buf.bitcast(_U32)
    va_w = va_buf.bitcast(_U32)
    qa_w = qa_buf.bitcast(_U32)
    wk_w = wk_buf.bitcast(_U32)
    q_scale = _DH ** -0.5 * _LOG2E
    wt_w = wt_scr.bitcast(_U32)
    kv_w = kv_scr.bitcast(_U32)

    def tile(v):
        return jnp.tile(v, (_C // 8, 1))

    def words(a):
        return slice(a * _C // 2, (a + 1) * _C // 2)

    def transpose_weights(j):
        for w_buf, base in ((wq_buf, 0), (wv_buf, _C)):
            wt = w_buf[j].T
            for g in range(_NG):
                wt_scr[j, g, base:base + _C, :] = wt[:, g * _C:(g + 1) * _C]

    def project(j, lo, n):
        xs = jnp.concatenate(
            [_as_bf16(x_w[g, lo // 2:(lo + n) // 2, :]) for g in range(_NG)], axis=1)
        wk = jnp.concatenate([_as_bf16(wk_w[j, words(g), :]) for g in range(_NG)], axis=0)
        kn = _dot(xs, wk)
        kn_scr[j, lo:lo + n, :] = kn.astype(_BF16)
        if lo < _S - _L:
            pk_scr[j, lo:lo + n, :] = _phi(kn).astype(_BF16)
        wt = jnp.concatenate([_as_bf16(wt_w[j, g]) for g in range(_NG)], axis=1)
        qv = _dot_nt(wt, xs)
        for t in range(n // _C):
            tt = lo // _C + t
            qt = qv[0:_C, t * _C:(t + 1) * _C]
            qs_scr[tt, col(j), :] = (qt * q_scale).astype(_BF16)
            if tt >= _L // _C:
                pq_scr[tt - _L // _C, col(j), :] = _phi(qt).astype(_BF16)
            vt_scr[tt, col(j), :] = qv[_C:2 * _C, t * _C:(t + 1) * _C].astype(_BF16)

    def spectrum(j, a):
        fmat = _as_bf16(f_w[...])
        z_scr[1, a] = _dot_nt(fmat, h_buf[j, :, a * _C:(a + 1) * _C])
        lo = 8 + a * _C
        kpad_scr[lo:lo + _C, :] = _as_bf16(ka_w[j, words(a), :]).astype(_F32)
        ks = kpad_scr[lo:lo + _C, :] * tile(par_scr[j, 0])
        for t in range(1, _KS):
            ks = ks + kpad_scr[lo - t:lo + _C - t, :] * tile(par_scr[j, t])
        kv = (ks * _as_bf16(va_w[j, words(a), :]).astype(_F32)).astype(_BF16)
        kv_scr[a * _C:(a + 1) * _C, :] = kv
        z_scr[0, a] = _dot(fmat, kv)

    def cross_chunks():
        z_st, z_ld = zero_smem[0], zero_smem[1]
        nb = 4
        for r in range(_NC):
            re, im = slice(8 * r, 8 * r + 8), slice(_C + 8 * r, _C + 8 * r + 8)

            def triple(which, a):
                x, y = z_scr[z_ld + which, a, re, :], z_scr[z_ld + which, a, im, :]
                return x, y, x + y

            prev = None
            for lo in range(0, _NC, nb):
                u, acc = {}, {}
                for t in range(lo + nb):
                    h = triple(1, t)
                    for a in range(max(lo, t), lo + nb):
                        if a - t not in u:
                            u[a - t] = triple(0, a - t)
                        prod = [x * y for x, y in zip(u[a - t], h)]
                        acc[a] = prod if t == 0 else [x + y for x, y in zip(acc[a], prod)]
                outs = []
                for a in range(lo, lo + nb):
                    k1, k2, k3 = acc[a]
                    yr, yi = cur = (k1 - k2, k3 - k1 - k2)
                    if prev is not None:
                        yr, yi = ((yr - prev[1], yi + prev[0]) if r < _C // 16
                                  else (yr + prev[1], yi - prev[0]))
                    prev = cur
                    outs.append((a, yr, yi))
                for a, yr, yi in outs:
                    z_scr[z_st + 2, a, re, :] = yr
                    z_scr[z_st + 2, a, im, :] = yi

    def finish(j, a):
        y = _dot(ft_buf[...], z_scr[zero_smem[1] + 2, a].astype(_BF16)) * (1.0 / _C)
        y = y + _as_bf16(kv_w[words(a), :]).astype(_F32) * tile(par_scr[j, _KS])
        outa_buf[j, a * _C:(a + 1) * _C, :] = (
            _as_bf16(qa_w[j, words(a), :]).astype(_F32) * y).astype(_BF16)

    def convolve(j, fillers, lead):
        for n, job in enumerate(fillers):
            if n == lead:
                for a in range(_NC):
                    spectrum(j, a)
            job()
        cross_chunks()
        for a in range(_NC):
            finish(j, a)
        outa_copy(j).start()

    qs_w = qs_scr.bitcast(_U32)
    pq_w = pq_scr.bitcast(_U32)
    vt_w = vt_scr.bitcast(_U32)
    kn_w = kn_scr.bitcast(_U32)
    pk_w = pk_scr.bitcast(_U32)
    kwin_w = kwin_scr.bitcast(_U32)
    pkwin_w = pkwin_scr.bitcast(_U32)
    tiles = _L // _C

    row16 = lax.broadcasted_iota(jnp.int32, (16, _C), 0)
    row8 = lax.broadcasted_iota(jnp.int32, (8, _C), 0)

    def in_head(hh):
        return (row16 >= 2 * hh) & (row16 < 2 * hh + 10)

    def spread(f):
        return jnp.concatenate(
            [f[0], f[0], jnp.where(row8 < 4, f[0], f[1]), f[1], f[1],
             f[2], f[2], jnp.where(row8 < 4, f[2], f[3]), f[3], f[3]], axis=0)

    class Quad:
        def __init__(self, m, slot):
            self.m, self.slot = m, slot
            self.wrow = pl.ds(m * 40, 40)
            self.mem = None
            first = m * (4 * _DH)
            off, g0 = first % _C, first // _C
            g1 = min(g0 + 1, _NG - 1)
            for src, dst, n_rows in ((kn_w, kwin_w, _S), (pk_w, pkwin_w, _S - _L)):
                lane = lax.broadcasted_iota(jnp.int32, (n_rows // 2, _C), 1)
                if off == 0:
                    dst[slot] = src[g0]
                else:
                    dst[slot] = pltpu.roll(jnp.where(lane >= off, src[g0], src[g1]), _C - off, 1)

        def gate(self, hh):
            return gate_scr[self.m * 4 + hh]

        def v_words(self, s, t):
            return vt_w[tiles * s + t, self.wrow, :]

        def memory_update(self, s):
            ones = jnp.full((8, _C), _ONES_BF16_PAIR, _U32)
            v_ext = jnp.concatenate(
                [_as_bf16(jnp.concatenate([self.v_words(s, t), ones], axis=0))
                 for t in range(tiles)], axis=1)
            pk = _as_bf16(pkwin_w[self.slot, s * _L // 2:(s + 1) * _L // 2, :])
            row = lax.broadcasted_iota(jnp.int32, (96, _C), 0)
            lane = lax.broadcasted_iota(jnp.int32, (96, _C), 1)
            keep = jnp.zeros((96, _C), jnp.bool_)
            for hh in range(4):
                rows = ((row >= _DH * hh) & (row < _DH * (hh + 1))) | (row == 80 + hh)
                keep = keep | (rows & (lane >= _DH * hh) & (lane < _DH * (hh + 1)))
            upd = jnp.where(keep, _dot(v_ext, pk), 0.0)
            self.mem = upd if self.mem is None else self.mem + upd

        def memory_read(self, s):
            pq = jnp.concatenate(
                [_as_bf16(jnp.concatenate(
                    [pq_w[tiles * (s - 1) + i, self.wrow, :], jnp.zeros((24, _C), _U32)],
                    axis=0)) for i in range(tiles)], axis=1)
            got = _dot(self.mem.astype(_BF16), pq)
            for i in range(tiles):
                gi = got[:, i * _C:(i + 1) * _C]
                fac = [self.gate(hh) / (jnp.broadcast_to(gi[80 + hh:81 + hh], (8, _C)) + 1e-6)
                       for hh in range(4)]
                amem_scr[s % 2, i] = gi[0:80] * spread(fac)

        def logits(self, s, i, t):
            qq = qs_w[tiles * s + i, self.wrow, :]
            cols = []
            for hh in range(4):
                qh = jnp.where(in_head(hh), qq[8 * hh:8 * hh + 16], jnp.uint32(0))
                parts = [jnp.zeros((8 * hh, _C), _U32)] if hh > 0 else []
                parts += [qh, jnp.zeros((48 - 8 * hh, _C), _U32)]
                cols.append(_as_bf16(jnp.concatenate(parts, axis=0)))
            lo = (s * _L + t * _C) // 2
            keys = _as_bf16(kwin_w[self.slot, lo:lo + _C // 2, :])
            return _dot(keys, jnp.concatenate(cols, axis=1))

        def store(self, s, i, accs):
            norm = [(1.0 - self.gate(hh)) / (accs[hh][24:32] if hh < 2 else accs[hh][0:8])
                    for hh in range(4)]
            o = jnp.concatenate(
                [accs[0][0:16], jnp.where(row8 < 4, accs[0][16:24], accs[1][0:8]),
                 accs[1][8:24], accs[2][8:24],
                 jnp.where(row8 < 4, accs[2][24:32], accs[3][8:16]), accs[3][16:32]],
                axis=0) * spread(norm)
            if s > 0:
                o = o + amem_scr[s % 2, i]
            rows = pl.ds(self.m * (4 * _DH), 4 * _DH)
            ot_scr[tiles * s + i, rows, :] = o.astype(_BF16)

    def attention(which):
        quads = [Quad(m, m) for m in which]
        units = [(quad, s, i, t) for quad in quads for s in range(_NSEG)
                 for i in range(tiles) for t in range(i + 1)]
        causal = (lax.broadcasted_iota(jnp.int32, (_C, _C), 0)
                  <= lax.broadcasted_iota(jnp.int32, (_C, _C), 1))
        run_max, accs = {}, None
        for n in range(len(units) + _LAG):
            if n < len(units):
                quad, s, i, t = units[n]
                if s > 0 and (i, t) == (0, 0):
                    quad.memory_update(s - 1)
                if s > 0 and (i, t) == (1, 1):
                    quad.memory_read(s)
                sc = quad.logits(s, i, t)
                cur = []
                for hh in range(4):
                    sh = sc[:, hh * _C:(hh + 1) * _C]
                    if t == i:
                        sh = jnp.where(causal, sh, -jnp.inf)
                    s_scr[n % (_LAG + 1), hh] = sh
                    part = jnp.max(sh, axis=0, keepdims=True)
                    cur.append(part if t == 0 else jnp.maximum(run_max[n - 1][hh], part))
                run_max[n] = cur
            if n >= _LAG:
                u = n - _LAG
                quad, s, i, t = units[u]
                vq = quad.v_words(s, t)
                cur = []
                for hh in range(4):
                    mx = run_max[u][hh]
                    p = jnp.exp2(s_scr[u % (_LAG + 1), hh] - mx).astype(_BF16)
                    vh = _as_bf16(jnp.where(in_head(hh), vq[8 * hh:8 * hh + 16],
                                            jnp.uint32(_ONES_BF16_PAIR)))
                    pv = _dot(vh, p)
                    if t > 0:
                        pv = pv + accs[hh] * jnp.exp2(run_max[u - 1][hh] - mx)
                    cur.append(pv)
                accs = cur
                if t == i:
                    quad.store(s, i, accs)

    start(small + weight_copies(0) + x_copies(0))
    wait(small)
    start(x_copies(1) + x_copies(2))
    wait(weight_copies(0))
    for p in range(len(_X_SPLIT) - 1):
        if p == 1:
            start(x_copies(3))
        if p == 3:
            start(dft_copies + weight_copies(1))
        wait(x_copies(p))
        if p == 0:
            transpose_weights(0)
        if p == 1:
            shift = shift_buf[...].astype(_F32)
            dvec = d_buf[...].astype(_F32).reshape(1, _D)
            for g in range(_NG):
                sl = slice(g * _C, (g + 1) * _C)
                for t in range(_KS):
                    par_scr[g, t] = jnp.broadcast_to(shift[t:t + 1, sl], (8, _C))
                par_scr[g, _KS] = jnp.broadcast_to(dvec[:, sl], (8, _C))
            beta = beta_buf[...].astype(_F32).reshape(1, _H)
            gate = 1.0 / (1.0 + jnp.exp(-beta))
            for hd in range(_H):
                gate_scr[hd] = jnp.broadcast_to(gate[:, hd:hd + 1], (8, _C))
            kpad_scr[0:8, :] = jnp.zeros((8, _C), _F32)
            zero_smem[0] = 0
            zero_smem[1] = 0
        for lo in range(_X_SPLIT[p], _X_SPLIT[p + 1], _PIECE):
            project(0, lo, _PIECE)
    start(conv_copies(0) + [gate_copy(0)])
    wait(weight_copies(1))
    attention(range(1))
    wait(dft_copies)

    def phase1(j, carry):
        @pl.when(j > 0)
        def _():
            wait(weight_copies(j + 1))

        wait(conv_copies(j)[:2] + [gate_copy(j)])
        start(conv_copies(j + 1) + [gate_copy(j + 1)])

        @pl.when(j + 2 < _NG)
        def _():
            start(weight_copies(j + 2))

        @pl.when(j == _NG - 2)
        def _():
            wo_copy.start()

        wait(conv_copies(j)[2:])
        transpose_weights(j + 1)
        jobs = [functools.partial(project, j + 1, lo, _PIECE) for lo in range(0, _S, _PIECE)]
        convolve(j, jobs, 1)
        return carry

    lax.fori_loop(0, _NG - 1, phase1, 0)

    wait([wo_copy])
    attention(range(1, _NQ))

    def output_projection(p):
        lo, hi = _OUT_SPLIT[p] // _C, _OUT_SPLIT[p + 1] // _C
        ot = jnp.concatenate([ot_scr[t] for t in range(lo, hi)], axis=1)
        outb_buf[lo * _C:hi * _C, :] = _dot_tn(ot, wo_buf[...]).astype(_BF16)
        outb_copy(p).start()

    n_out = len(_OUT_SPLIT) - 1
    wait(conv_copies(_NG - 1) + [gate_copy(_NG - 1)])
    convolve(_NG - 1, [functools.partial(output_projection, p) for p in range(_OUT_OVERLAP)], 0)
    for p in range(_OUT_OVERLAP, n_out):
        output_projection(p)
    wait([outa_copy(j) for j in range(_NG)] + [outb_copy(p) for p in range(n_out)])


@jax.jit
def pallas_concat_heads__ssm_conv_h3__memory_aug_infini_attn__prompt_kernel(
    A_q: jax.Array,
    A_k: jax.Array,
    A_v: jax.Array,
    A_shift_k: jax.Array,
    A_ssm_k: jax.Array,
    A_ssm_D: jax.Array,
    B_x: jax.Array,
    B_wq: jax.Array,
    B_wk: jax.Array,
    B_wv: jax.Array,
    B_wo: jax.Array,
    B_beta: jax.Array,
):
    assert A_q.shape == (1, _S, _D) and B_x.shape == (1, _S, _D)
    assert A_shift_k.shape == (_D, _KS) and B_beta.shape == (_H,)
    fmat = _dft_matrix()
    f_fwd = fmat.astype(_BF16)
    f_inv = np.ascontiguousarray(fmat.T).astype(_BF16)

    vmem = pltpu.VMEM
    dma = pltpu.SemaphoreType.DMA
    scratch = [
        vmem((_NG, _S, _C), _BF16),
        vmem((_NG, _S, _C), _BF16),
        vmem((_NG, _S, _C), _BF16),
        vmem((_NG, _C, _S), _BF16),
        vmem((_NG, _S, _C), _BF16),
        vmem((_NG, _D, _C), _BF16),
        vmem((_NG, _D, _C), _BF16),
        vmem((_NG, _D, _C), _BF16),
        vmem((_D, _D), _BF16),
        vmem((_KS, _D), _BF16),
        vmem((_D,), _BF16),
        vmem((_H,), _BF16),
        vmem((2 * _C, _C), _BF16),
        vmem((_C, 2 * _C), _BF16),
        vmem((_NG, _KS + 1, 8, _C), _F32),
        vmem((_H, 8, _C), _F32),
        vmem((_S + 8, _C), _F32),
        vmem((_S, _C), _BF16),
        vmem((_NG, _S, _C), _BF16),
        vmem((_NG, _NG, 2 * _C, _C), _BF16),
        vmem((3, _NC, 2 * _C, _C), _F32),
        pltpu.SMEM((2,), jnp.int32),
        vmem((_NC, _D, _C), _BF16),
        vmem((_NC - _L // _C, _D, _C), _BF16),
        vmem((_NC, _D, _C), _BF16),
        vmem((_NG, _S, _C), _BF16),
        vmem((_NG, _S - _L, _C), _BF16),
        vmem((_NQ, _S, _C), _BF16),
        vmem((_NQ, _S - _L, _C), _BF16),
        vmem((_LAG + 1, 4, _C, _C), _F32),
        vmem((2, 4, 80, _C), _F32),
        vmem((_NC, _D, _C), _BF16),
        vmem((_S, _D), _BF16),
        dma((4, _NG)), dma((3, _NG)), dma((len(_X_SPLIT) - 1,)), dma((6,)), dma((_NG,)),
        dma((len(_OUT_SPLIT) - 1,)),
    ]
    out = pl.pallas_call(
        _kernel,
        out_shape=jax.ShapeDtypeStruct((_S, 2 * _D), _BF16),
        in_specs=[pl.BlockSpec(memory_space=pl.ANY)] * 14,
        out_specs=pl.BlockSpec(memory_space=pl.ANY),
        scratch_shapes=scratch,
        compiler_params=pltpu.CompilerParams(vmem_limit_bytes=100 * 1024 * 1024),
        name="h3_infini",
    )(A_q.reshape(_S, _D), A_k.reshape(_S, _D), A_v.reshape(_S, _D), A_shift_k.T,
      A_ssm_k, A_ssm_D, B_x.reshape(_S, _D), B_wq, B_wk, B_wv, B_wo, B_beta,
      f_fwd, f_inv)
    return out.reshape(1, _S, 2 * _D)
```

```python
import functools
import math

import numpy as np
import jax
import jax.numpy as jnp
from jax import lax
import jax.experimental.pallas as pl
import jax.experimental.pallas.tpu as pltpu

_S = 2048
_D = 640
_H = 32
_DH = 20
_NSEG = 4
_L = _S // _NSEG
_C = 128
_NC = _S // _C
_NG = _D // _C
_NQ = _H // 4
_KS = 4
_PIECE = 256
_X_SPLIT = (0, 256, 512, 1024, 2048)
_OUT_SPLIT = (0, 512, 1024, 1536, 1792, 2048)
_OUT_OVERLAP = 2
_PAD = 16
_LAG = 2

_F32 = jnp.float32
_BF16 = jnp.bfloat16
_U32 = jnp.uint32
_LOG2E = math.log2(math.e)
_ONES_BF16_PAIR = 0x3F803F80


def _dft_matrices():
    even = np.arange(0, _C, 2)
    k = np.concatenate([even, _C - 1 - even])
    ang = np.pi * np.outer(2 * k + 1, np.arange(_C)) / (2 * _C)
    fwd = np.concatenate([np.cos(ang), -np.sin(ang)], axis=0)
    half = np.concatenate([np.cos(ang[:_C // 2]), -np.sin(ang[:_C // 2])], axis=0).T / _C
    inv = np.concatenate([half[0::2], half[1::2]], axis=0)
    return fwd.astype(np.float32), inv.astype(np.float32)


def _dot(a, b):
    return jnp.dot(a, b, preferred_element_type=_F32)


def _dot_nt(a, b):
    return lax.dot_general(a, b, (((1,), (1,)), ((), ())), preferred_element_type=_F32)


def _dot_tn(a, b):
    return lax.dot_general(a, b, (((0,), (0,)), ((), ())), preferred_element_type=_F32)


def _as_bf16(words):
    return pltpu.bitcast(words, _BF16)


def _row_pairs(words):
    return tuple(pltpu.unpack_elementwise(words, index=i, packed_dtype=_BF16, unpacked_dtype=_F32)
                 for i in range(2))


def _pack_rows(even, odd):
    return pltpu.pack_elementwise([even, odd], packed_dtype=_BF16)


def _phi(t):
    return jnp.where(t > 0, t + 1.0, jnp.exp(t))


def _kernel(q_hbm, k_hbm, v_hbm, shift_hbm, h_hbm, d_hbm, x_hbm,
            wq_hbm, wk_hbm, wv_hbm, wo_hbm, beta_hbm, f_hbm, ft_hbm, out_hbm,
            qa_buf, ka_buf, va_buf, h_buf, x_buf, wq_buf, wk_buf, wv_buf, wo_buf,
            shift_buf, d_buf, beta_buf, f_buf, ft_buf,
            par_scr, gate_scr, kv_scr, outa_buf,
            wt_scr, z_scr, zero_smem, qs_scr, pq_scr, vt_scr, kn_scr, pk_scr,
            ot_scr, outb_buf,
            sem_a, sem_w, sem_x, sem_c, sem_oa, sem_ob):

    cp = pltpu.make_async_copy

    def col(j):
        return pl.ds(j * _C if isinstance(j, int) else pl.multiple_of(j * _C, _C), _C)

    def conv_copies(j):
        return [cp(k_hbm.at[:, col(j)], ka_buf.at[j, pl.ds(_PAD, _S)], sem_a.at[0, j]),
                cp(v_hbm.at[:, col(j)], va_buf.at[j], sem_a.at[1, j]),
                cp(h_hbm.at[col(j), :], h_buf.at[j], sem_a.at[2, j])]

    def gate_copy(j):
        return cp(q_hbm.at[:, col(j)], qa_buf.at[j], sem_a.at[3, j])

    def weight_copies(j):
        return [cp(wk_hbm.at[:, col(j)], wk_buf.at[j], sem_w.at[0, j]),
                cp(wq_hbm.at[:, col(j)], wq_buf.at[j], sem_w.at[1, j]),
                cp(wv_hbm.at[:, col(j)], wv_buf.at[j], sem_w.at[2, j])]

    def x_copies(p):
        rows = pl.ds(_X_SPLIT[p], _X_SPLIT[p + 1] - _X_SPLIT[p])
        return [cp(x_hbm.at[rows, col(g)], x_buf.at[g, rows], sem_x.at[p]) for g in range(_NG)]

    def outa_copy(j):
        return cp(outa_buf.at[j], out_hbm.at[:, col(j)], sem_oa.at[j])

    def outb_copy(p):
        rows = pl.ds(_OUT_SPLIT[p], _OUT_SPLIT[p + 1] - _OUT_SPLIT[p])
        return cp(outb_buf.at[rows], out_hbm.at[rows, pl.ds(_D, _D)], sem_ob.at[p])

    small = [cp(shift_hbm, shift_buf, sem_c.at[0]), cp(d_hbm, d_buf, sem_c.at[1]),
             cp(beta_hbm, beta_buf, sem_c.at[2])]
    dft_copies = [cp(f_hbm, f_buf, sem_c.at[3]), cp(ft_hbm, ft_buf, sem_c.at[4])]
    wo_copy = cp(wo_hbm, wo_buf, sem_c.at[5])

    def start(copies):
        for c in copies:
            c.start()

    def wait(copies):
        for c in copies:
            c.wait()

    x_w = x_buf.bitcast(_U32)
    f_w = f_buf.bitcast(_U32)
    ka_w = ka_buf.bitcast(_U32)
    va_w = va_buf.bitcast(_U32)
    qa_w = qa_buf.bitcast(_U32)
    wk_w = wk_buf.bitcast(_U32)
    q_scale = _DH ** -0.5 * _LOG2E
    wt_w = wt_scr.bitcast(_U32)
    ft_w = ft_buf.bitcast(_U32)
    outa_w = outa_buf.bitcast(_U32)

    def tile(v):
        return jnp.tile(v, (_C // 16, 1))

    def words(a):
        return slice(a * _C // 2, (a + 1) * _C // 2)

    def transpose_weights(j):
        for w_buf, base in ((wq_buf, 0), (wv_buf, _C)):
            wt = w_buf[j].T
            for g in range(_NG):
                wt_scr[j, g, base:base + _C, :] = wt[:, g * _C:(g + 1) * _C]

    def project(j, lo, n):
        xs = jnp.concatenate(
            [_as_bf16(x_w[g, lo // 2:(lo + n) // 2, :]) for g in range(_NG)], axis=1)
        wk = jnp.concatenate([_as_bf16(wk_w[j, words(g), :]) for g in range(_NG)], axis=0)
        kn = _dot(xs, wk)
        kn_scr[j, lo:lo + n, :] = kn.astype(_BF16)
        if lo < _S - _L:
            pk_scr[j, lo:lo + n, :] = _phi(kn).astype(_BF16)
        wt = jnp.concatenate([_as_bf16(wt_w[j, g]) for g in range(_NG)], axis=1)
        qv = _dot_nt(wt, xs)
        for t in range(n // _C):
            tt = lo // _C + t
            qt = qv[0:_C, t * _C:(t + 1) * _C]
            qs_scr[tt, col(j), :] = (qt * q_scale).astype(_BF16)
            if tt >= _L // _C:
                pq_scr[tt - _L // _C, col(j), :] = _phi(qt).astype(_BF16)
            vt_scr[tt, col(j), :] = qv[_C:2 * _C, t * _C:(t + 1) * _C].astype(_BF16)

    def spectrum(j, a):
        fmat = _as_bf16(f_w[...])
        z_scr[1, a] = _dot_nt(fmat, h_buf[j, :, a * _C:(a + 1) * _C])
        lo = _PAD // 2 + a * _C // 2
        e0, o0 = _row_pairs(ka_w[j, lo:lo + _C // 2, :])
        e1, o1 = _row_pairs(ka_w[j, lo - 1:lo - 1 + _C // 2, :])
        _, o2 = _row_pairs(ka_w[j, lo - 2:lo - 2 + _C // 2, :])
        w0, w1, w2, w3 = (tile(par_scr[j, t]) for t in range(_KS))
        ve, vo = _row_pairs(va_w[j, words(a), :])
        kv = _pack_rows((e0 * w0 + o1 * w1 + e1 * w2 + o2 * w3) * ve,
                        (o0 * w0 + e0 * w1 + o1 * w2 + e1 * w3) * vo)
        kv_scr[words(a), :] = kv
        z_scr[0, a] = _dot(fmat, _as_bf16(kv))

    def cross_chunks():
        z_st, z_ld = zero_smem[0], zero_smem[1]
        nb = 4
        for r in range(_NC):
            re, im = slice(8 * r, 8 * r + 8), slice(_C + 8 * r, _C + 8 * r + 8)

            def triple(which, a):
                x, y = z_scr[z_ld + which, a, re, :], z_scr[z_ld + which, a, im, :]
                return x, y, x + y

            prev = None
            for lo in range(0, _NC, nb):
                u, acc = {}, {}
                for t in range(lo + nb):
                    h = triple(1, t)
                    for a in range(max(lo, t), lo + nb):
                        if a - t not in u:
                            u[a - t] = triple(0, a - t)
                        prod = [x * y for x, y in zip(u[a - t], h)]
                        acc[a] = prod if t == 0 else [x + y for x, y in zip(acc[a], prod)]
                outs = []
                for a in range(lo, lo + nb):
                    k1, k2, k3 = acc[a]
                    yr, yi = cur = (k1 - k2, k3 - k1 - k2)
                    if prev is not None:
                        yr, yi = ((yr - prev[1], yi + prev[0]) if r < _C // 16
                                  else (yr + prev[1], yi - prev[0]))
                    prev = cur
                    outs.append((a, yr, yi))
                for a, yr, yi in outs:
                    z_scr[z_st + 2, a, re, :] = yr
                    z_scr[z_st + 2, a, im, :] = yi

    def finish(j, a):
        y = z_scr[zero_smem[1] + 2, a]
        lo_re, hi_re, lo_im, hi_im = (y[q * _C // 2:(q + 1) * _C // 2] for q in range(4))
        spec_e = jnp.concatenate([lo_re + hi_re, lo_im - hi_im], axis=0).astype(_BF16)
        spec_o = jnp.concatenate([lo_re - hi_re, lo_im + hi_im], axis=0).astype(_BF16)
        ye = _dot(_as_bf16(ft_w[0:_C // 4, :]), spec_e)
        yo = _dot(_as_bf16(ft_w[_C // 4:_C // 2, :]), spec_o)
        skip = tile(par_scr[j, _KS])
        kve, kvo = _row_pairs(kv_scr[words(a), :])
        qe, qo = _row_pairs(qa_w[j, words(a), :])
        outa_w[j, words(a), :] = _pack_rows(qe * (ye + kve * skip), qo * (yo + kvo * skip))

    def convolve(j, fillers, lead):
        for n, job in enumerate(fillers):
            if n == lead:
                for a in range(_NC):
                    spectrum(j, a)
            job()
        cross_chunks()
        for a in range(_NC):
            finish(j, a)
        outa_copy(j).start()

    qs_w = qs_scr.bitcast(_U32)
    pq_w = pq_scr.bitcast(_U32)
    vt_w = vt_scr.bitcast(_U32)
    kn_w = kn_scr.bitcast(_U32)
    pk_w = pk_scr.bitcast(_U32)
    tiles = _L // _C

    row16 = lax.broadcasted_iota(jnp.int32, (16, _C), 0)
    row8 = lax.broadcasted_iota(jnp.int32, (8, _C), 0)

    def in_head(hh):
        return (row16 >= 2 * hh) & (row16 < 2 * hh + 10)

    def spread(f):
        return jnp.concatenate(
            [f[0], f[0], jnp.where(row8 < 4, f[0], f[1]), f[1], f[1],
             f[2], f[2], jnp.where(row8 < 4, f[2], f[3]), f[3], f[3]], axis=0)

    class Quad:
        def __init__(self, m, slot):
            self.m, self.slot = m, slot
            self.wrow = pl.ds(m * 40, 40)
            self.mem = None
            self.a_mem = {}
            first = m * (4 * _DH)
            off, g0 = first % _C, first // _C
            g1 = min(g0 + 1, _NG - 1)
            self.off, self.g0, self.g1 = off, g0, g1
            self.keys = {}

        def window(self, src, lo, n):
            rows = slice(lo // 2, (lo + n) // 2)
            if self.off == 0:
                return _as_bf16(src[self.g0, rows, :])
            lane = lax.broadcasted_iota(jnp.int32, (n // 2, _C), 1)
            w = jnp.where(lane >= self.off, src[self.g0, rows, :], src[self.g1, rows, :])
            return _as_bf16(pltpu.roll(w, _C - self.off, 1))

        def gate(self, hh):
            return gate_scr[self.m * 4 + hh]

        def v_words(self, s, t):
            return vt_w[tiles * s + t, self.wrow, :]

        def memory_update(self, s):
            ones = jnp.full((8, _C), _ONES_BF16_PAIR, _U32)
            v_ext = jnp.concatenate(
                [_as_bf16(jnp.concatenate([self.v_words(s, t), ones], axis=0))
                 for t in range(tiles)], axis=1)
            pk = self.window(pk_w, s * _L, _L)
            row = lax.broadcasted_iota(jnp.int32, (96, _C), 0)
            lane = lax.broadcasted_iota(jnp.int32, (96, _C), 1)
            keep = jnp.zeros((96, _C), jnp.bool_)
            for hh in range(4):
                rows = ((row >= _DH * hh) & (row < _DH * (hh + 1))) | (row == 80 + hh)
                keep = keep | (rows & (lane >= _DH * hh) & (lane < _DH * (hh + 1)))
            upd = jnp.where(keep, _dot(v_ext, pk), 0.0)
            self.mem = upd if self.mem is None else self.mem + upd

        def memory_read(self, s):
            pq = jnp.concatenate(
                [_as_bf16(jnp.concatenate(
                    [pq_w[tiles * (s - 1) + i, self.wrow, :], jnp.zeros((24, _C), _U32)],
                    axis=0)) for i in range(tiles)], axis=1)
            got = _dot(self.mem.astype(_BF16), pq)
            for i in range(tiles):
                gi = got[:, i * _C:(i + 1) * _C]
                fac = [self.gate(hh) / (jnp.broadcast_to(gi[80 + hh:81 + hh], (8, _C)) + 1e-6)
                       for hh in range(4)]
                self.a_mem[s, i] = gi[0:80] * spread(fac)

        def logits(self, s, i, t):
            qq = qs_w[tiles * s + i, self.wrow, :]
            cols = []
            for hh in range(4):
                qh = jnp.where(in_head(hh), qq[8 * hh:8 * hh + 16], jnp.uint32(0))
                parts = [jnp.zeros((8 * hh, _C), _U32)] if hh > 0 else []
                parts += [qh, jnp.zeros((48 - 8 * hh, _C), _U32)]
                cols.append(_as_bf16(jnp.concatenate(parts, axis=0)))
            if (s, t) not in self.keys:
                self.keys[s, t] = self.window(kn_w, s * _L + t * _C, _C)
            keys = self.keys[s, t]
            return _dot(keys, jnp.concatenate(cols, axis=1))

        def store(self, s, i, accs):
            norm = [(1.0 - self.gate(hh)) / (accs[hh][24:32] if hh < 2 else accs[hh][0:8])
                    for hh in range(4)]
            o = jnp.concatenate(
                [accs[0][0:16], jnp.where(row8 < 4, accs[0][16:24], accs[1][0:8]),
                 accs[1][8:24], accs[2][8:24],
                 jnp.where(row8 < 4, accs[2][24:32], accs[3][8:16]), accs[3][16:32]],
                axis=0) * spread(norm)
            if s > 0:
                o = o + self.a_mem.pop((s, i))
            rows = pl.ds(self.m * (4 * _DH), 4 * _DH)
            ot_scr[tiles * s + i, rows, :] = o.astype(_BF16)

    def attention(which):
        quads = [Quad(m, m) for m in which]
        units = [(quad, s, i, t) for quad in quads for s in range(_NSEG)
                 for i in range(tiles) for t in range(i + 1)]
        causal = (lax.broadcasted_iota(jnp.int32, (_C, _C), 0)
                  <= lax.broadcasted_iota(jnp.int32, (_C, _C), 1))
        scores, run_max, accs = {}, {}, None
        for n in range(len(units) + _LAG):
            if n < len(units):
                quad, s, i, t = units[n]
                if s > 0 and (i, t) == (0, 0):
                    quad.memory_update(s - 1)
                if s > 0 and (i, t) == (1, 1):
                    quad.memory_read(s)
                sc = quad.logits(s, i, t)
                cur = []
                for hh in range(4):
                    sh = sc[:, hh * _C:(hh + 1) * _C]
                    if t == i:
                        sh = jnp.where(causal, sh, -jnp.inf)
                    scores[n, hh] = sh
                    part = jnp.max(sh, axis=0, keepdims=True)
                    cur.append(part if t == 0 else jnp.maximum(run_max[n - 1][hh], part))
                run_max[n] = cur
            if n >= _LAG:
                u = n - _LAG
                quad, s, i, t = units[u]
                vq = quad.v_words(s, t)
                cur = []
                for hh in range(4):
                    mx = run_max[u][hh]
                    p = jnp.exp2(scores.pop((u, hh)) - mx).astype(_BF16)
                    vh = _as_bf16(jnp.where(in_head(hh), vq[8 * hh:8 * hh + 16],
                                            jnp.uint32(_ONES_BF16_PAIR)))
                    pv = _dot(vh, p)
                    if t > 0:
                        pv = pv + accs[hh] * jnp.exp2(run_max[u - 1][hh] - mx)
                    cur.append(pv)
                accs = cur
                if t == i:
                    quad.store(s, i, accs)

    start(small + weight_copies(0) + x_copies(0))
    wait(small)
    start(x_copies(1) + x_copies(2))
    wait(weight_copies(0))
    for p in range(len(_X_SPLIT) - 1):
        if p == 1:
            start(x_copies(3))
        if p == 3:
            start(dft_copies + weight_copies(1))
        wait(x_copies(p))
        if p == 0:
            transpose_weights(0)
        if p == 1:
            shift = shift_buf[...].astype(_F32)
            dvec = d_buf[...].astype(_F32).reshape(1, _D)
            for g in range(_NG):
                sl = slice(g * _C, (g + 1) * _C)
                for t in range(_KS):
                    par_scr[g, t] = jnp.broadcast_to(shift[t:t + 1, sl], (8, _C))
                par_scr[g, _KS] = jnp.broadcast_to(dvec[:, sl], (8, _C))
            beta = beta_buf[...].astype(_F32).reshape(1, _H)
            gate = 1.0 / (1.0 + jnp.exp(-beta))
            for hd in range(_H):
                gate_scr[hd] = jnp.broadcast_to(gate[:, hd:hd + 1], (8, _C))
            for g in range(_NG):
                ka_w[g, 0:_PAD // 2, :] = jnp.zeros((_PAD // 2, _C), _U32)
            zero_smem[0] = 0
            zero_smem[1] = 0
        for lo in range(_X_SPLIT[p], _X_SPLIT[p + 1], _PIECE):
            project(0, lo, _PIECE)
    start(conv_copies(0) + [gate_copy(0)])
    wait(weight_copies(1))
    attention(range(1))
    wait(dft_copies)

    def phase1(j, carry):
        @pl.when(j > 0)
        def _():
            wait(weight_copies(j + 1))

        wait(conv_copies(j)[:2] + [gate_copy(j)])
        start(conv_copies(j + 1) + [gate_copy(j + 1)])

        @pl.when(j + 2 < _NG)
        def _():
            start(weight_copies(j + 2))

        @pl.when(j == _NG - 2)
        def _():
            wo_copy.start()

        wait(conv_copies(j)[2:])
        transpose_weights(j + 1)
        jobs = [functools.partial(project, j + 1, lo, _PIECE) for lo in range(0, _S, _PIECE)]
        convolve(j, jobs, 1)
        return carry

    lax.fori_loop(0, _NG - 1, phase1, 0)

    wait([wo_copy])
    attention(range(1, _NQ))

    def output_projection(p):
        lo, hi = _OUT_SPLIT[p] // _C, _OUT_SPLIT[p + 1] // _C
        ot = jnp.concatenate([ot_scr[t] for t in range(lo, hi)], axis=1)
        outb_buf[lo * _C:hi * _C, :] = _dot_tn(ot, wo_buf[...]).astype(_BF16)
        outb_copy(p).start()

    n_out = len(_OUT_SPLIT) - 1
    wait(conv_copies(_NG - 1) + [gate_copy(_NG - 1)])
    convolve(_NG - 1, [functools.partial(output_projection, p) for p in range(_OUT_OVERLAP)], 0)
    for p in range(_OUT_OVERLAP, n_out):
        output_projection(p)
    wait([outa_copy(j) for j in range(_NG)] + [outb_copy(p) for p in range(n_out)])


@jax.jit
def pallas_concat_heads__ssm_conv_h3__memory_aug_infini_attn__prompt_kernel(
    A_q: jax.Array,
    A_k: jax.Array,
    A_v: jax.Array,
    A_shift_k: jax.Array,
    A_ssm_k: jax.Array,
    A_ssm_D: jax.Array,
    B_x: jax.Array,
    B_wq: jax.Array,
    B_wk: jax.Array,
    B_wv: jax.Array,
    B_wo: jax.Array,
    B_beta: jax.Array,
):
    assert A_q.shape == (1, _S, _D) and B_x.shape == (1, _S, _D)
    assert A_shift_k.shape == (_D, _KS) and B_beta.shape == (_H,)
    f_fwd, f_inv = (m.astype(_BF16) for m in _dft_matrices())

    vmem = pltpu.VMEM
    dma = pltpu.SemaphoreType.DMA
    scratch = [
        vmem((_NG, _S, _C), _BF16),
        vmem((_NG, _PAD + _S, _C), _BF16),
        vmem((_NG, _S, _C), _BF16),
        vmem((_NG, _C, _S), _BF16),
        vmem((_NG, _S, _C), _BF16),
        vmem((_NG, _D, _C), _BF16),
        vmem((_NG, _D, _C), _BF16),
        vmem((_NG, _D, _C), _BF16),
        vmem((_D, _D), _BF16),
        vmem((_KS, _D), _BF16),
        vmem((_D,), _BF16),
        vmem((_H,), _BF16),
        vmem((2 * _C, _C), _BF16),
        vmem((_C, _C), _BF16),
        vmem((_NG, _KS + 1, 8, _C), _F32),
        vmem((_H, 8, _C), _F32),
        vmem((_S // 2, _C), _U32),
        vmem((_NG, _S, _C), _BF16),
        vmem((_NG, _NG, 2 * _C, _C), _BF16),
        vmem((3, _NC, 2 * _C, _C), _F32),
        pltpu.SMEM((2,), jnp.int32),
        vmem((_NC, _D, _C), _BF16),
        vmem((_NC - _L // _C, _D, _C), _BF16),
        vmem((_NC, _D, _C), _BF16),
        vmem((_NG, _S, _C), _BF16),
        vmem((_NG, _S - _L, _C), _BF16),
        vmem((_NC, _D, _C), _BF16),
        vmem((_S, _D), _BF16),
        dma((4, _NG)), dma((3, _NG)), dma((len(_X_SPLIT) - 1,)), dma((6,)), dma((_NG,)),
        dma((len(_OUT_SPLIT) - 1,)),
    ]
    out = pl.pallas_call(
        _kernel,
        out_shape=jax.ShapeDtypeStruct((_S, 2 * _D), _BF16),
        in_specs=[pl.BlockSpec(memory_space=pl.ANY)] * 14,
        out_specs=pl.BlockSpec(memory_space=pl.ANY),
        scratch_shapes=scratch,
        compiler_params=pltpu.CompilerParams(vmem_limit_bytes=100 * 1024 * 1024),
        name="h3_infini",
    )(A_q.reshape(_S, _D), A_k.reshape(_S, _D), A_v.reshape(_S, _D), A_shift_k.T,
      A_ssm_k, A_ssm_D, B_x.reshape(_S, _D), B_wq, B_wk, B_wv, B_wo, B_beta,
      f_fwd, f_inv)
    return out.reshape(1, _S, 2 * _D)
```

```python
import functools
import math

import numpy as np
import jax
import jax.numpy as jnp
from jax import lax
import jax.experimental.pallas as pl
import jax.experimental.pallas.tpu as pltpu

_S = 2048
_D = 640
_H = 32
_DH = 20
_NSEG = 4
_L = _S // _NSEG
_C = 128
_NC = _S // _C
_NG = _D // _C
_NQ = _H // 4
_KS = 4
_PIECE = 256
_X_SPLIT = (0, 256, 512, 1024, 2048)
_OUT_SPLIT = (0, 512, 1024, 1536, 1792, 2048)
_OUT_OVERLAP = 2
_PAD = 16
_LAG = 2

_F32 = jnp.float32
_BF16 = jnp.bfloat16
_U32 = jnp.uint32
_LOG2E = math.log2(math.e)
_WINDOW = (0, 16, 40, 56)


def _dft_matrices():
    even = np.arange(0, _C, 2)
    k = np.concatenate([even, _C - 1 - even])
    ang = np.pi * np.outer(2 * k + 1, np.arange(_C)) / (2 * _C)
    fwd = np.concatenate([np.cos(ang), -np.sin(ang)], axis=0)
    half = np.concatenate([np.cos(ang[:_C // 2]), -np.sin(ang[:_C // 2])], axis=0).T / _C
    inv = np.concatenate([half[0::2], half[1::2]], axis=0)
    return fwd.astype(np.float32), inv.astype(np.float32)


def _dot(a, b):
    return jnp.dot(a, b, preferred_element_type=_F32)


def _dot_nt(a, b):
    return lax.dot_general(a, b, (((1,), (1,)), ((), ())), preferred_element_type=_F32)


def _dot_tn(a, b):
    return lax.dot_general(a, b, (((0,), (0,)), ((), ())), preferred_element_type=_F32)


def _as_bf16(words):
    return pltpu.bitcast(words, _BF16)


def _row_pairs(words):
    return tuple(pltpu.unpack_elementwise(words, index=i, packed_dtype=_BF16, unpacked_dtype=_F32)
                 for i in range(2))


def _pack_rows(even, odd):
    return pltpu.pack_elementwise([even, odd], packed_dtype=_BF16)


def _round_bf16(x):
    return x.astype(_BF16).astype(_F32)


def _dot_mixed(a, b):
    return lax.dot_general(a, b, (((1,), (0,)), ((), ())), preferred_element_type=_F32)


def _phi(t):
    return jnp.where(t > 0, t + 1.0, jnp.exp(t))


def _kernel(q_hbm, k_hbm, v_hbm, shift_hbm, h_hbm, d_hbm, x_hbm,
            wq_hbm, wk_hbm, wv_hbm, wo_hbm, beta_hbm, f_hbm, ft_hbm, out_hbm,
            qa_buf, ka_buf, va_buf, h_buf, x_buf, wq_buf, wk_buf, wv_buf, wo_buf,
            shift_buf, d_buf, beta_buf, f_buf, ft_buf,
            par_scr, gate_scr, kv_scr, outa_buf,
            wt_scr, z_scr, zero_smem, qs_scr, pq_scr, vt_scr, kn_scr, pk_scr,
            ot_scr, outb_buf,
            sem_a, sem_w, sem_x, sem_c, sem_oa, sem_ob):

    cp = pltpu.make_async_copy

    def col(j):
        return pl.ds(j * _C if isinstance(j, int) else pl.multiple_of(j * _C, _C), _C)

    def conv_copies(j):
        return [cp(k_hbm.at[:, col(j)], ka_buf.at[j, pl.ds(_PAD, _S)], sem_a.at[0, j]),
                cp(v_hbm.at[:, col(j)], va_buf.at[j], sem_a.at[1, j]),
                cp(h_hbm.at[col(j), :], h_buf.at[j], sem_a.at[2, j])]

    def gate_copy(j):
        return cp(q_hbm.at[:, col(j)], qa_buf.at[j], sem_a.at[3, j])

    def weight_copies(j):
        return [cp(wk_hbm.at[:, col(j)], wk_buf.at[j], sem_w.at[0, j]),
                cp(wq_hbm.at[:, col(j)], wq_buf.at[j], sem_w.at[1, j]),
                cp(wv_hbm.at[:, col(j)], wv_buf.at[j], sem_w.at[2, j])]

    def x_copies(p):
        rows = pl.ds(_X_SPLIT[p], _X_SPLIT[p + 1] - _X_SPLIT[p])
        return [cp(x_hbm.at[rows, col(g)], x_buf.at[g, rows], sem_x.at[p]) for g in range(_NG)]

    def outa_copy(j):
        return cp(outa_buf.at[j], out_hbm.at[:, col(j)], sem_oa.at[j])

    def outb_copy(p):
        rows = pl.ds(_OUT_SPLIT[p], _OUT_SPLIT[p + 1] - _OUT_SPLIT[p])
        return cp(outb_buf.at[rows], out_hbm.at[rows, pl.ds(_D, _D)], sem_ob.at[p])

    small = [cp(shift_hbm, shift_buf, sem_c.at[0]), cp(d_hbm, d_buf, sem_c.at[1]),
             cp(beta_hbm, beta_buf, sem_c.at[2])]
    dft_copies = [cp(f_hbm, f_buf, sem_c.at[3]), cp(ft_hbm, ft_buf, sem_c.at[4])]
    wo_copy = cp(wo_hbm, wo_buf, sem_c.at[5])

    def start(copies):
        for c in copies:
            c.start()

    def wait(copies):
        for c in copies:
            c.wait()

    x_w = x_buf.bitcast(_U32)
    f_w = f_buf.bitcast(_U32)
    ka_w = ka_buf.bitcast(_U32)
    va_w = va_buf.bitcast(_U32)
    qa_w = qa_buf.bitcast(_U32)
    wk_w = wk_buf.bitcast(_U32)
    q_scale = _DH ** -0.5 * _LOG2E
    wt_w = wt_scr.bitcast(_U32)
    ft_w = ft_buf.bitcast(_U32)
    outa_w = outa_buf.bitcast(_U32)

    def tile(v):
        return jnp.tile(v, (_C // 16, 1))

    def words(a):
        return slice(a * _C // 2, (a + 1) * _C // 2)

    def transpose_weights(j):
        for w_buf, base in ((wq_buf, 0), (wv_buf, _C)):
            wt = w_buf[j].T
            for g in range(_NG):
                wt_scr[j, g, base:base + _C, :] = wt[:, g * _C:(g + 1) * _C]

    def project(j, lo, n):
        xs = jnp.concatenate(
            [_as_bf16(x_w[g, lo // 2:(lo + n) // 2, :]) for g in range(_NG)], axis=1)
        wk = jnp.concatenate([_as_bf16(wk_w[j, words(g), :]) for g in range(_NG)], axis=0)
        kn = _dot(xs, wk)
        kn_scr[j, lo:lo + n, :] = kn.astype(_BF16)
        if lo < _S - _L:
            pk_scr[j, lo:lo + n, :] = _phi(kn).astype(_BF16)
        wt = jnp.concatenate([_as_bf16(wt_w[j, g]) for g in range(_NG)], axis=1)
        qv = _dot_nt(wt, xs)
        for t in range(n // _C):
            tt = lo // _C + t
            qt = qv[0:_C, t * _C:(t + 1) * _C]
            qs_scr[tt, col(j), :] = (qt * q_scale).astype(_BF16)
            if tt >= _L // _C:
                pq_scr[tt - _L // _C, col(j), :] = _phi(qt).astype(_BF16)
            vt_scr[tt, col(j), :] = _round_bf16(qv[_C:2 * _C, t * _C:(t + 1) * _C])

    def spectrum(j, a):
        fmat = _as_bf16(f_w[...])
        z_scr[1, a] = _dot_nt(fmat, h_buf[j, :, a * _C:(a + 1) * _C])
        lo = _PAD // 2 + a * _C // 2
        e0, o0 = _row_pairs(ka_w[j, lo:lo + _C // 2, :])
        e1, o1 = _row_pairs(ka_w[j, lo - 1:lo - 1 + _C // 2, :])
        _, o2 = _row_pairs(ka_w[j, lo - 2:lo - 2 + _C // 2, :])
        w0, w1, w2, w3 = (tile(par_scr[j, t]) for t in range(_KS))
        ve, vo = _row_pairs(va_w[j, words(a), :])
        kv = _pack_rows((e0 * w0 + o1 * w1 + e1 * w2 + o2 * w3) * ve,
                        (o0 * w0 + e0 * w1 + o1 * w2 + e1 * w3) * vo)
        kv_scr[words(a), :] = kv
        z_scr[0, a] = _dot(fmat, _as_bf16(kv))

    def cross_chunks():
        z_st, z_ld = zero_smem[0], zero_smem[1]
        nb = 4
        for r in range(_NC):
            re, im = slice(8 * r, 8 * r + 8), slice(_C + 8 * r, _C + 8 * r + 8)

            def triple(which, a):
                x, y = z_scr[z_ld + which, a, re, :], z_scr[z_ld + which, a, im, :]
                return x, y, x + y

            prev = None
            for lo in range(0, _NC, nb):
                u, acc = {}, {}
                for t in range(lo + nb):
                    h = triple(1, t)
                    for a in range(max(lo, t), lo + nb):
                        if a - t not in u:
                            u[a - t] = triple(0, a - t)
                        prod = [x * y for x, y in zip(u[a - t], h)]
                        acc[a] = prod if t == 0 else [x + y for x, y in zip(acc[a], prod)]
                outs = []
                for a in range(lo, lo + nb):
                    k1, k2, k3 = acc[a]
                    yr, yi = cur = (k1 - k2, k3 - k1 - k2)
                    if prev is not None:
                        yr, yi = ((yr - prev[1], yi + prev[0]) if r < _C // 16
                                  else (yr + prev[1], yi - prev[0]))
                    prev = cur
                    outs.append((a, yr, yi))
                for a, yr, yi in outs:
                    z_scr[z_st + 2, a, re, :] = yr
                    z_scr[z_st + 2, a, im, :] = yi

    def finish(j, a):
        y = z_scr[zero_smem[1] + 2, a]
        lo_re, hi_re, lo_im, hi_im = (y[q * _C // 2:(q + 1) * _C // 2] for q in range(4))
        spec_e = jnp.concatenate([lo_re + hi_re, lo_im - hi_im], axis=0).astype(_BF16)
        spec_o = jnp.concatenate([lo_re - hi_re, lo_im + hi_im], axis=0).astype(_BF16)
        ye = _dot(_as_bf16(ft_w[0:_C // 4, :]), spec_e)
        yo = _dot(_as_bf16(ft_w[_C // 4:_C // 2, :]), spec_o)
        skip = tile(par_scr[j, _KS])
        kve, kvo = _row_pairs(kv_scr[words(a), :])
        qe, qo = _row_pairs(qa_w[j, words(a), :])
        outa_w[j, words(a), :] = _pack_rows(qe * (ye + kve * skip), qo * (yo + kvo * skip))

    def convolve(j, fillers, lead):
        for n, job in enumerate(fillers):
            if n == lead:
                for a in range(_NC):
                    spectrum(j, a)
            job()
        cross_chunks()
        for a in range(_NC):
            finish(j, a)
        outa_copy(j).start()

    qs_w = qs_scr.bitcast(_U32)
    pq_w = pq_scr.bitcast(_U32)
    kn_w = kn_scr.bitcast(_U32)
    pk_w = pk_scr.bitcast(_U32)
    tiles = _L // _C

    row16 = lax.broadcasted_iota(jnp.int32, (16, _C), 0)
    row8 = lax.broadcasted_iota(jnp.int32, (8, _C), 0)

    def in_head(hh):
        return (row16 >= 2 * hh) & (row16 < 2 * hh + 10)

    def spread(f):
        return jnp.concatenate(
            [f[0], f[0], jnp.where(row8 < 4, f[0], f[1]), f[1], f[1],
             f[2], f[2], jnp.where(row8 < 4, f[2], f[3]), f[3], f[3]], axis=0)

    class Quad:
        def __init__(self, m, slot):
            self.m, self.slot = m, slot
            self.wrow = pl.ds(m * 40, 40)
            self.mem = None
            self.a_mem = {}
            first = m * (4 * _DH)
            off, g0 = first % _C, first // _C
            g1 = min(g0 + 1, _NG - 1)
            self.off, self.g0, self.g1 = off, g0, g1
            self.keys = {}
            self.q = {}

        def window(self, src, lo, n):
            rows = slice(lo // 2, (lo + n) // 2)
            if self.off == 0:
                return _as_bf16(src[self.g0, rows, :])
            lane = lax.broadcasted_iota(jnp.int32, (n // 2, _C), 1)
            w = jnp.where(lane >= self.off, src[self.g0, rows, :], src[self.g1, rows, :])
            return _as_bf16(pltpu.roll(w, _C - self.off, 1))

        def gate(self, hh):
            return gate_scr[self.m * 4 + hh]

        def values(self, s, t, lo, n):
            first = self.m * (4 * _DH) + lo
            return vt_scr[tiles * s + t, first:first + n, :]

        def values_and_ones(self, s, t, hh):
            v = self.values(s, t, _WINDOW[hh], 24)
            if hh % 2:
                return jnp.concatenate([jnp.where(row8 < 4, 1.0, v[:8]), v[8:]], axis=0)
            return jnp.concatenate([v[:16], jnp.where(row8 < 4, v[16:], 1.0)], axis=0)

        def memory_update(self, s):
            v_ext = jnp.concatenate(
                [jnp.concatenate([self.values(s, t, 0, 80), jnp.ones((8, _C), _F32)], axis=0)
                 for t in range(tiles)], axis=1)
            row = lax.broadcasted_iota(jnp.int32, (88, _C), 0)
            lane = lax.broadcasted_iota(jnp.int32, (88, _C), 1)
            keep = jnp.zeros((88, _C), jnp.bool_)
            for hh in range(4):
                rows = ((row >= _DH * hh) & (row < _DH * (hh + 1))) | (row == 80 + hh)
                keep = keep | (rows & (lane >= _DH * hh) & (lane < _DH * (hh + 1)))
            upd = jnp.where(keep, _dot_mixed(v_ext, self.window(pk_w, s * _L, _L)), 0.0)
            self.mem = upd if self.mem is None else self.mem + upd

        def memory_read(self, s):
            pq = jnp.concatenate(
                [_as_bf16(jnp.concatenate(
                    [pq_w[tiles * (s - 1) + i, self.wrow, :], jnp.zeros((24, _C), _U32)],
                    axis=0)) for i in range(tiles)], axis=1)
            got = _dot_mixed(_round_bf16(self.mem), pq)
            for i in range(tiles):
                gi = got[:, i * _C:(i + 1) * _C]
                fac = [self.gate(hh) / (jnp.broadcast_to(gi[80 + hh:81 + hh], (8, _C)) + 1e-6)
                       for hh in range(4)]
                self.a_mem[s, i] = gi[0:80] * spread(fac)

        def queries(self, s, i):
            if (s, i) not in self.q:
                qq = qs_w[tiles * s + i, self.wrow, :]
                tiles_ = []
                for hh in range(4):
                    qh = jnp.where(in_head(hh), qq[8 * hh:8 * hh + 16], jnp.uint32(0))
                    if hh % 2:
                        qh = pltpu.roll(qh, _C // 2, 1)
                    parts = [jnp.zeros((8 * hh, _C), _U32)] if hh > 0 else []
                    parts += [qh, jnp.zeros((48 - 8 * hh, _C), _U32)]
                    tiles_.append(jnp.concatenate(parts, axis=0))
                self.q = {(s, i): tiles_}
            return self.q[s, i]

        def logits(self, s, i, t):
            if (s, t) not in self.keys:
                self.keys[s, t] = self.window(kn_w, s * _L + t * _C, _C)
            keys, qs = self.keys[s, t], self.queries(s, i)
            all_q = jnp.concatenate([_as_bf16(q) for q in qs], axis=1)
            if t < i:
                sc = _dot(keys, all_q)
                return [sc[:, hh * _C:(hh + 1) * _C] for hh in range(4)]
            half = _C // 2
            key = lax.broadcasted_iota(jnp.int32, (half, _C), 0)
            lane = lax.broadcasted_iota(jnp.int32, (half, _C), 1)
            sc = _dot(keys[:half], all_q)
            top = [jnp.where(key <= (lane ^ (half * (hh % 2))), sc[:, hh * _C:(hh + 1) * _C],
                             -jnp.inf) for hh in range(4)]
            pair = jnp.concatenate(
                [_as_bf16(jnp.where(lane < half, qs[hh + 1], qs[hh])) for hh in (0, 2)], axis=1)
            sc = jnp.concatenate(
                [_dot(keys[lo:lo + half // 2], pair) for lo in (half, half + half // 2)], axis=0)
            low = [jnp.where(key <= (lane & (half - 1)), sc[:, c * _C:(c + 1) * _C], -jnp.inf)
                   for c in range(2)]
            return top, low

        def store(self, s, i, accs):
            part = []
            for hh in range(4):
                r = 0 if hh % 2 else 23
                norm = (1.0 - self.gate(hh)) / jnp.broadcast_to(accs[hh][r:r + 1], (8, _C))
                x = accs[hh] * jnp.tile(norm, (3, 1))
                part.append(pltpu.roll(x, _C // 2, 1) if hh % 2 else x)
            o = jnp.concatenate(
                [part[0][0:16], jnp.where(row8 < 4, part[0][16:24], part[1][0:8]), part[1][8:24],
                 part[2][0:16], jnp.where(row8 < 4, part[2][16:24], part[3][0:8]), part[3][8:24]],
                axis=0)
            if s > 0:
                o = o + self.a_mem.pop((s, i))
            rows = pl.ds(self.m * (4 * _DH), 4 * _DH)
            ot_scr[tiles * s + i, rows, :] = o.astype(_BF16)

    def attention(which):
        quads = [Quad(m, m) for m in which]
        units = [(quad, s, i, t) for quad in quads for s in range(_NSEG)
                 for i in range(tiles) for t in range(i + 1)]
        left = lax.broadcasted_iota(jnp.int32, (8, _C), 1) < _C // 2
        left_w = lax.broadcasted_iota(jnp.int32, (_C // 4, _C), 1) < _C // 2

        def col_max(x):
            return jnp.broadcast_to(jnp.max(x, axis=0, keepdims=True), (8, _C))

        def weights(x, mx):
            return jnp.exp2(x - jnp.tile(mx, (x.shape[0] // 8, 1))).astype(_BF16)

        scores, run_max, accs = {}, {}, None
        for n in range(len(units) + _LAG):
            if n < len(units):
                quad, s, i, t = units[n]
                if s > 0 and (i, t) == (0, 0):
                    quad.memory_update(s - 1)
                if s > 0 and (i, t) == (1, 1):
                    quad.memory_read(s)
                scores[n] = sc = quad.logits(s, i, t)
                if t < i:
                    cur = [col_max(x) for x in sc]
                else:
                    low = [col_max(x) for x in sc[1]]
                    cur = [jnp.maximum(col_max(x), jnp.where((left if hh % 2 else ~left), low[hh // 2],
                                                             -jnp.inf))
                           for hh, x in enumerate(sc[0])]
                if t > 0:
                    cur = [jnp.maximum(x, y) for x, y in zip(cur, run_max[n - 1])]
                run_max[n] = cur
            if n >= _LAG:
                u = n - _LAG
                quad, s, i, t = units[u]
                sc, mx = scores.pop(u), run_max[u]
                if t < i:
                    ps = [weights(sc[hh], mx[hh]) for hh in range(4)]
                else:
                    low = [pltpu.bitcast(weights(sc[1][c], jnp.where(left, mx[2 * c + 1],
                                                                     mx[2 * c])), _U32)
                           for c in range(2)]
                    ps = [jnp.concatenate(
                        [weights(sc[0][hh], mx[hh]),
                         _as_bf16(jnp.where((left_w if hh % 2 else ~left_w), low[hh // 2], jnp.uint32(0)))],
                        axis=0) for hh in range(4)]
                cur = []
                for hh in range(4):
                    pv = _dot_mixed(quad.values_and_ones(s, t, hh), ps[hh])
                    if t > 0:
                        pv = pv + accs[hh] * jnp.tile(
                            jnp.exp2(run_max[u - 1][hh] - mx[hh]), (3, 1))
                    cur.append(pv)
                accs = cur
                if t == i:
                    quad.store(s, i, accs)

    start(small + weight_copies(0) + x_copies(0))
    wait(small)
    start(x_copies(1) + x_copies(2))
    wait(weight_copies(0))
    for p in range(len(_X_SPLIT) - 1):
        if p == 1:
            start(x_copies(3))
        if p == 3:
            start(dft_copies + weight_copies(1))
        wait(x_copies(p))
        if p == 0:
            transpose_weights(0)
        if p == 1:
            shift = shift_buf[...].astype(_F32)
            dvec = d_buf[...].astype(_F32).reshape(1, _D)
            for g in range(_NG):
                sl = slice(g * _C, (g + 1) * _C)
                for t in range(_KS):
                    par_scr[g, t] = jnp.broadcast_to(shift[t:t + 1, sl], (8, _C))
                par_scr[g, _KS] = jnp.broadcast_to(dvec[:, sl], (8, _C))
            beta = beta_buf[...].astype(_F32).reshape(1, _H)
            gate = 1.0 / (1.0 + jnp.exp(-beta))
            for hd in range(_H):
                gate_scr[hd] = jnp.broadcast_to(gate[:, hd:hd + 1], (8, _C))
            for g in range(_NG):
                ka_w[g, 0:_PAD // 2, :] = jnp.zeros((_PAD // 2, _C), _U32)
            zero_smem[0] = 0
            zero_smem[1] = 0
        for lo in range(_X_SPLIT[p], _X_SPLIT[p + 1], _PIECE):
            project(0, lo, _PIECE)
    start(conv_copies(0) + [gate_copy(0)])
    wait(weight_copies(1))
    attention(range(1))
    wait(dft_copies)

    def phase1(j, carry):
        @pl.when(j > 0)
        def _():
            wait(weight_copies(j + 1))

        wait(conv_copies(j)[:2] + [gate_copy(j)])
        start(conv_copies(j + 1) + [gate_copy(j + 1)])

        @pl.when(j + 2 < _NG)
        def _():
            start(weight_copies(j + 2))

        @pl.when(j == _NG - 2)
        def _():
            wo_copy.start()

        wait(conv_copies(j)[2:])
        transpose_weights(j + 1)
        jobs = [functools.partial(project, j + 1, lo, _PIECE) for lo in range(0, _S, _PIECE)]
        convolve(j, jobs, 1)
        return carry

    lax.fori_loop(0, _NG - 1, phase1, 0)

    wait([wo_copy])
    attention(range(1, _NQ))

    def output_projection(p):
        lo, hi = _OUT_SPLIT[p] // _C, _OUT_SPLIT[p + 1] // _C
        ot = jnp.concatenate([ot_scr[t] for t in range(lo, hi)], axis=1)
        outb_buf[lo * _C:hi * _C, :] = _dot_tn(ot, wo_buf[...]).astype(_BF16)
        outb_copy(p).start()

    n_out = len(_OUT_SPLIT) - 1
    wait(conv_copies(_NG - 1) + [gate_copy(_NG - 1)])
    convolve(_NG - 1, [functools.partial(output_projection, p) for p in range(_OUT_OVERLAP)], 0)
    for p in range(_OUT_OVERLAP, n_out):
        output_projection(p)
    wait([outa_copy(j) for j in range(_NG)] + [outb_copy(p) for p in range(n_out)])


@jax.jit
def pallas_concat_heads__ssm_conv_h3__memory_aug_infini_attn__prompt_kernel(
    A_q: jax.Array,
    A_k: jax.Array,
    A_v: jax.Array,
    A_shift_k: jax.Array,
    A_ssm_k: jax.Array,
    A_ssm_D: jax.Array,
    B_x: jax.Array,
    B_wq: jax.Array,
    B_wk: jax.Array,
    B_wv: jax.Array,
    B_wo: jax.Array,
    B_beta: jax.Array,
):
    assert A_q.shape == (1, _S, _D) and B_x.shape == (1, _S, _D)
    assert A_shift_k.shape == (_D, _KS) and B_beta.shape == (_H,)
    f_fwd, f_inv = (m.astype(_BF16) for m in _dft_matrices())

    vmem = pltpu.VMEM
    dma = pltpu.SemaphoreType.DMA
    scratch = [
        vmem((_NG, _S, _C), _BF16),
        vmem((_NG, _PAD + _S, _C), _BF16),
        vmem((_NG, _S, _C), _BF16),
        vmem((_NG, _C, _S), _BF16),
        vmem((_NG, _S, _C), _BF16),
        vmem((_NG, _D, _C), _BF16),
        vmem((_NG, _D, _C), _BF16),
        vmem((_NG, _D, _C), _BF16),
        vmem((_D, _D), _BF16),
        vmem((_KS, _D), _BF16),
        vmem((_D,), _BF16),
        vmem((_H,), _BF16),
        vmem((2 * _C, _C), _BF16),
        vmem((_C, _C), _BF16),
        vmem((_NG, _KS + 1, 8, _C), _F32),
        vmem((_H, 8, _C), _F32),
        vmem((_S // 2, _C), _U32),
        vmem((_NG, _S, _C), _BF16),
        vmem((_NG, _NG, 2 * _C, _C), _BF16),
        vmem((3, _NC, 2 * _C, _C), _F32),
        pltpu.SMEM((2,), jnp.int32),
        vmem((_NC, _D, _C), _BF16),
        vmem((_NC - _L // _C, _D, _C), _BF16),
        vmem((_NC, _D, _C), _F32),
        vmem((_NG, _S, _C), _BF16),
        vmem((_NG, _S - _L, _C), _BF16),
        vmem((_NC, _D, _C), _BF16),
        vmem((_S, _D), _BF16),
        dma((4, _NG)), dma((3, _NG)), dma((len(_X_SPLIT) - 1,)), dma((6,)), dma((_NG,)),
        dma((len(_OUT_SPLIT) - 1,)),
    ]
    out = pl.pallas_call(
        _kernel,
        out_shape=jax.ShapeDtypeStruct((_S, 2 * _D), _BF16),
        in_specs=[pl.BlockSpec(memory_space=pl.ANY)] * 14,
        out_specs=pl.BlockSpec(memory_space=pl.ANY),
        scratch_shapes=scratch,
        compiler_params=pltpu.CompilerParams(vmem_limit_bytes=100 * 1024 * 1024),
        name="h3_infini",
    )(A_q.reshape(_S, _D), A_k.reshape(_S, _D), A_v.reshape(_S, _D), A_shift_k.T,
      A_ssm_k, A_ssm_D, B_x.reshape(_S, _D), B_wq, B_wk, B_wv, B_wo, B_beta,
      f_fwd, f_inv)
    return out.reshape(1, _S, 2 * _D)
```

```python
import functools
import math

import numpy as np
import jax
import jax.numpy as jnp
from jax import lax
import jax.experimental.pallas as pl
import jax.experimental.pallas.tpu as pltpu

_S = 2048
_D = 640
_H = 32
_DH = 20
_NSEG = 4
_L = _S // _NSEG
_C = 128
_NC = _S // _C
_NG = _D // _C
_NQ = _H // 4
_KS = 4
_PIECE = 256
_X_SPLIT = (0, 256, 512, 1024, 2048)
_OUT_SPLIT = (0, 512, 1024, 1536, 1792, 2048)
_OUT_OVERLAP = 2
_PAD = 16
_LAG = 2

_F32 = jnp.float32
_BF16 = jnp.bfloat16
_U32 = jnp.uint32
_LOG2E = math.log2(math.e)
_WINDOW = (0, 16, 40, 56)


def _dft_matrices():
    even = np.arange(0, _C, 2)
    k = np.concatenate([even, _C - 1 - even])
    ang = np.pi * np.outer(2 * k + 1, np.arange(_C)) / (2 * _C)
    fwd = np.concatenate([np.cos(ang), -np.sin(ang)], axis=0)
    half = np.concatenate([np.cos(ang[:_C // 2]), -np.sin(ang[:_C // 2])], axis=0).T / _C
    inv = np.concatenate([half[0::2], half[1::2]], axis=0)
    return fwd.astype(np.float32), inv.astype(np.float32)


def _dot(a, b):
    return jnp.dot(a, b, preferred_element_type=_F32)


def _dot_nt(a, b):
    return lax.dot_general(a, b, (((1,), (1,)), ((), ())), preferred_element_type=_F32)


def _dot_tn(a, b):
    return lax.dot_general(a, b, (((0,), (0,)), ((), ())), preferred_element_type=_F32)


def _as_bf16(words):
    return pltpu.bitcast(words, _BF16)


def _row_pairs(words):
    return tuple(pltpu.unpack_elementwise(words, index=i, packed_dtype=_BF16, unpacked_dtype=_F32)
                 for i in range(2))


def _pack_rows(even, odd):
    return pltpu.pack_elementwise([even, odd], packed_dtype=_BF16)


def _round_bf16(x):
    return x.astype(_BF16).astype(_F32)


def _dot_mixed(a, b):
    return lax.dot_general(a, b, (((1,), (0,)), ((), ())), preferred_element_type=_F32)


def _phi(t):
    return jnp.where(t > 0, t + 1.0, jnp.exp(t))


def _kernel(q_hbm, k_hbm, v_hbm, shift_hbm, h_hbm, d_hbm, x_hbm,
            wq_hbm, wk_hbm, wv_hbm, wo_hbm, beta_hbm, f_hbm, ft_hbm, out_hbm,
            qa_buf, ka_buf, va_buf, h_buf, x_raw, x_buf, wq_buf, wk_buf, wv_buf, wo_buf,
            shift_buf, d_buf, beta_buf, f_buf, ft_buf,
            par_scr, gate_scr, kv_scr, outa_buf,
            wt_scr, z_scr, zero_smem, qs_scr, pq_scr, vt_scr, kn_scr, pk_scr,
            ot_scr, outb_buf,
            sem):

    cp = pltpu.make_async_copy

    def col(j):
        return pl.ds(j * _C if isinstance(j, int) else pl.multiple_of(j * _C, _C), _C)

    def weight_copies(j, s):
        return [cp(wk_hbm.at[:, col(j)], wk_buf.at[j], s),
                cp(wq_hbm.at[:, col(j)], wq_buf.at[j], s),
                cp(wv_hbm.at[:, col(j)], wv_buf.at[j], s)]

    def conv_copies(j):
        s = sem.at[4 + j % 2]
        return [cp(k_hbm.at[:, col(j)], ka_buf.at[j, pl.ds(_PAD, _S)], s),
                cp(v_hbm.at[:, col(j)], va_buf.at[j], s),
                cp(q_hbm.at[:, col(j)], qa_buf.at[j], s),
                cp(h_hbm.at[col(j), :], h_buf.at[j], s)]

    def next_weights(j):
        return weight_copies(j + 1, sem.at[4 + j % 2])

    def x_copies(p):
        rows = pl.ds(_X_SPLIT[p], _X_SPLIT[p + 1] - _X_SPLIT[p])
        return [cp(x_hbm.at[rows], x_raw.at[rows], sem.at[p % 3])]

    def outa_copy(j, s=2):
        return cp(outa_buf.at[j], out_hbm.at[:, col(j)], sem.at[s])

    def outb_copy(p):
        rows = pl.ds(_OUT_SPLIT[p], _OUT_SPLIT[p + 1] - _OUT_SPLIT[p])
        return cp(outb_buf.at[rows], out_hbm.at[rows, pl.ds(_D, _D)], sem.at[2])

    small = [cp(shift_hbm, shift_buf, sem.at[3]), cp(d_hbm, d_buf, sem.at[3]),
             cp(beta_hbm, beta_buf, sem.at[3])]
    first_weights = weight_copies(0, sem.at[0])
    second_batch = [cp(f_hbm, f_buf, sem.at[3]), cp(ft_hbm, ft_buf, sem.at[3])] + weight_copies(
        1, sem.at[3])
    wo_copy = cp(wo_hbm, wo_buf, sem.at[4 + (_NG - 1) % 2])

    def start(copies):
        for c in copies:
            c.start()

    def wait(copies):
        for c in copies:
            c.wait()

    x_w = x_buf.bitcast(_U32)
    f_w = f_buf.bitcast(_U32)
    ka_w = ka_buf.bitcast(_U32)
    va_w = va_buf.bitcast(_U32)
    qa_w = qa_buf.bitcast(_U32)
    wk_w = wk_buf.bitcast(_U32)
    q_scale = _DH ** -0.5 * _LOG2E
    wt_w = wt_scr.bitcast(_U32)
    ft_w = ft_buf.bitcast(_U32)
    outa_w = outa_buf.bitcast(_U32)

    def tile(v):
        return jnp.tile(v, (_C // 16, 1))

    def words(a):
        return slice(a * _C // 2, (a + 1) * _C // 2)

    def transpose_weights(j):
        for w_buf, base in ((wq_buf, 0), (wv_buf, _C)):
            wt = w_buf[j].T
            for g in range(_NG):
                wt_scr[j, g, base:base + _C, :] = wt[:, g * _C:(g + 1) * _C]

    def project(j, lo, n, first=False):
        if first:
            xs = x_raw[lo:lo + n, :]
            for g in range(_NG):
                x_buf[g, lo:lo + n, :] = xs[:, g * _C:(g + 1) * _C]
        else:
            xs = jnp.concatenate(
                [_as_bf16(x_w[g, lo // 2:(lo + n) // 2, :]) for g in range(_NG)], axis=1)
        wk = jnp.concatenate([_as_bf16(wk_w[j, words(g), :]) for g in range(_NG)], axis=0)
        kn = _dot(xs, wk)
        kn_scr[j, lo:lo + n, :] = kn.astype(_BF16)
        if lo < _S - _L:
            pk_scr[j, lo:lo + n, :] = _phi(kn).astype(_BF16)
        wt = jnp.concatenate([_as_bf16(wt_w[j, g]) for g in range(_NG)], axis=1)
        qv = _dot_nt(wt, xs)
        for t in range(n // _C):
            tt = lo // _C + t
            qt = qv[0:_C, t * _C:(t + 1) * _C]
            qs_scr[tt, col(j), :] = (qt * q_scale).astype(_BF16)
            if tt >= _L // _C:
                pq_scr[tt - _L // _C, col(j), :] = _phi(qt).astype(_BF16)
            vt_scr[tt, col(j), :] = _round_bf16(qv[_C:2 * _C, t * _C:(t + 1) * _C])

    def filter_spectrum(j, a):
        z_scr[1, a] = _dot_nt(_as_bf16(f_w[...]), h_buf[j, :, a * _C:(a + 1) * _C])

    def signal_spectrum(j, a):
        lo = _PAD // 2 + a * _C // 2
        e0, o0 = _row_pairs(ka_w[j, lo:lo + _C // 2, :])
        e1, o1 = _row_pairs(ka_w[j, lo - 1:lo - 1 + _C // 2, :])
        _, o2 = _row_pairs(ka_w[j, lo - 2:lo - 2 + _C // 2, :])
        w0, w1, w2, w3 = (tile(par_scr[j, t]) for t in range(_KS))
        ve, vo = _row_pairs(va_w[j, words(a), :])
        kv = _pack_rows((e0 * w0 + o1 * w1 + e1 * w2 + o2 * w3) * ve,
                        (o0 * w0 + e0 * w1 + o1 * w2 + e1 * w3) * vo)
        kv_scr[words(a), :] = kv
        z_scr[0, a] = _dot(_as_bf16(f_w[...]), _as_bf16(kv))

    def cross_chunks():
        z_st, z_ld = zero_smem[0], zero_smem[1]
        nb = 4
        for r in range(_NC):
            re, im = slice(8 * r, 8 * r + 8), slice(_C + 8 * r, _C + 8 * r + 8)

            def triple(which, a):
                x, y = z_scr[z_ld + which, a, re, :], z_scr[z_ld + which, a, im, :]
                return x, y, x + y

            prev = None
            for lo in range(0, _NC, nb):
                u, acc = {}, {}
                for t in range(lo + nb):
                    h = triple(1, t)
                    for a in range(max(lo, t), lo + nb):
                        if a - t not in u:
                            u[a - t] = triple(0, a - t)
                        prod = [x * y for x, y in zip(u[a - t], h)]
                        acc[a] = prod if t == 0 else [x + y for x, y in zip(acc[a], prod)]
                outs = []
                for a in range(lo, lo + nb):
                    k1, k2, k3 = acc[a]
                    yr, yi = cur = (k1 - k2, k3 - k1 - k2)
                    if prev is not None:
                        yr, yi = ((yr - prev[1], yi + prev[0]) if r < _C // 16
                                  else (yr + prev[1], yi - prev[0]))
                    prev = cur
                    outs.append((a, yr, yi))
                for a, yr, yi in outs:
                    z_scr[z_st + 2, a, re, :] = yr
                    z_scr[z_st + 2, a, im, :] = yi

    def finish(j, a):
        y = z_scr[zero_smem[1] + 2, a]
        lo_re, hi_re, lo_im, hi_im = (y[q * _C // 2:(q + 1) * _C // 2] for q in range(4))
        spec_e = jnp.concatenate([lo_re + hi_re, lo_im - hi_im], axis=0).astype(_BF16)
        spec_o = jnp.concatenate([lo_re - hi_re, lo_im + hi_im], axis=0).astype(_BF16)
        ye = _dot(_as_bf16(ft_w[0:_C // 4, :]), spec_e)
        yo = _dot(_as_bf16(ft_w[_C // 4:_C // 2, :]), spec_o)
        skip = tile(par_scr[j, _KS])
        kve, kvo = _row_pairs(kv_scr[words(a), :])
        qe, qo = _row_pairs(qa_w[j, words(a), :])
        outa_w[j, words(a), :] = _pack_rows(qe * (ye + kve * skip), qo * (yo + kvo * skip))

    def convolve(j, before, during):
        for job in before:
            job()
        for a in range(_NC + 4):
            if a < _NC:
                filter_spectrum(j, a)
            if a >= 4:
                signal_spectrum(j, a - 4)
        for job in during:
            job()
        cross_chunks()
        for a in range(_NC):
            finish(j, a)

    qs_w = qs_scr.bitcast(_U32)
    pq_w = pq_scr.bitcast(_U32)
    kn_w = kn_scr.bitcast(_U32)
    pk_w = pk_scr.bitcast(_U32)
    tiles = _L // _C

    row16 = lax.broadcasted_iota(jnp.int32, (16, _C), 0)
    row8 = lax.broadcasted_iota(jnp.int32, (8, _C), 0)

    def in_head(hh):
        return (row16 >= 2 * hh) & (row16 < 2 * hh + 10)

    def spread(f):
        return jnp.concatenate(
            [f[0], f[0], jnp.where(row8 < 4, f[0], f[1]), f[1], f[1],
             f[2], f[2], jnp.where(row8 < 4, f[2], f[3]), f[3], f[3]], axis=0)

    class Quad:
        def __init__(self, m, slot):
            self.m, self.slot = m, slot
            self.wrow = pl.ds(m * 40, 40)
            self.mem = None
            self.a_mem = {}
            first = m * (4 * _DH)
            off, g0 = first % _C, first // _C
            g1 = min(g0 + 1, _NG - 1)
            self.off, self.g0, self.g1 = off, g0, g1
            self.keys = {}
            self.q = {}

        def window(self, src, lo, n):
            rows = slice(lo // 2, (lo + n) // 2)
            if self.off == 0:
                return _as_bf16(src[self.g0, rows, :])
            lane = lax.broadcasted_iota(jnp.int32, (n // 2, _C), 1)
            w = jnp.where(lane >= self.off, src[self.g0, rows, :], src[self.g1, rows, :])
            return _as_bf16(pltpu.roll(w, _C - self.off, 1))

        def gate(self, hh):
            return gate_scr[self.m * 4 + hh]

        def values(self, s, t, lo, n):
            first = self.m * (4 * _DH) + lo
            return vt_scr[tiles * s + t, first:first + n, :]

        def values_and_ones(self, s, t, hh):
            v = self.values(s, t, _WINDOW[hh], 24)
            if hh % 2:
                return jnp.concatenate([jnp.where(row8 < 4, 1.0, v[:8]), v[8:]], axis=0)
            return jnp.concatenate([v[:16], jnp.where(row8 < 4, v[16:], 1.0)], axis=0)

        def memory_update(self, s):
            v_ext = jnp.concatenate(
                [jnp.concatenate([self.values(s, t, 0, 80), jnp.ones((8, _C), _F32)], axis=0)
                 for t in range(tiles)], axis=1)
            row = lax.broadcasted_iota(jnp.int32, (88, _C), 0)
            lane = lax.broadcasted_iota(jnp.int32, (88, _C), 1)
            keep = jnp.zeros((88, _C), jnp.bool_)
            for hh in range(4):
                rows = ((row >= _DH * hh) & (row < _DH * (hh + 1))) | (row == 80 + hh)
                keep = keep | (rows & (lane >= _DH * hh) & (lane < _DH * (hh + 1)))
            upd = jnp.where(keep, _dot_mixed(v_ext, self.window(pk_w, s * _L, _L)), 0.0)
            self.mem = upd if self.mem is None else self.mem + upd

        def memory_read(self, s):
            pq = jnp.concatenate(
                [_as_bf16(jnp.concatenate(
                    [pq_w[tiles * (s - 1) + i, self.wrow, :], jnp.zeros((24, _C), _U32)],
                    axis=0)) for i in range(tiles)], axis=1)
            got = _dot_mixed(_round_bf16(self.mem), pq)
            for i in range(tiles):
                gi = got[:, i * _C:(i + 1) * _C]
                fac = [self.gate(hh) / (jnp.broadcast_to(gi[80 + hh:81 + hh], (8, _C)) + 1e-6)
                       for hh in range(4)]
                self.a_mem[s, i] = gi[0:80] * spread(fac)

        def queries(self, s, i):
            if (s, i) not in self.q:
                qq = qs_w[tiles * s + i, self.wrow, :]
                tiles_ = []
                for hh in range(4):
                    qh = jnp.where(in_head(hh), qq[8 * hh:8 * hh + 16], jnp.uint32(0))
                    if hh % 2:
                        qh = pltpu.roll(qh, _C // 2, 1)
                    parts = [jnp.zeros((8 * hh, _C), _U32)] if hh > 0 else []
                    parts += [qh, jnp.zeros((48 - 8 * hh, _C), _U32)]
                    tiles_.append(jnp.concatenate(parts, axis=0))
                self.q = {(s, i): tiles_}
            return self.q[s, i]

        def logits(self, s, i, t):
            if (s, t) not in self.keys:
                self.keys[s, t] = self.window(kn_w, s * _L + t * _C, _C)
            keys, qs = self.keys[s, t], self.queries(s, i)
            all_q = jnp.concatenate([_as_bf16(q) for q in qs], axis=1)
            if t < i:
                sc = _dot(keys, all_q)
                return [sc[:, hh * _C:(hh + 1) * _C] for hh in range(4)]
            half = _C // 2
            key = lax.broadcasted_iota(jnp.int32, (half, _C), 0)
            lane = lax.broadcasted_iota(jnp.int32, (half, _C), 1)
            sc = _dot(keys[:half], all_q)
            top = [jnp.where(key <= (lane ^ (half * (hh % 2))), sc[:, hh * _C:(hh + 1) * _C],
                             -jnp.inf) for hh in range(4)]
            pair = jnp.concatenate(
                [_as_bf16(jnp.where(lane < half, qs[hh + 1], qs[hh])) for hh in (0, 2)], axis=1)
            sc = jnp.concatenate(
                [_dot(keys[lo:lo + half // 2], pair) for lo in (half, half + half // 2)], axis=0)
            low = [jnp.where(key <= (lane & (half - 1)), sc[:, c * _C:(c + 1) * _C], -jnp.inf)
                   for c in range(2)]
            return top, low

        def store(self, s, i, accs):
            part = []
            for hh in range(4):
                r = 0 if hh % 2 else 23
                norm = (1.0 - self.gate(hh)) / jnp.broadcast_to(accs[hh][r:r + 1], (8, _C))
                x = accs[hh] * jnp.tile(norm, (3, 1))
                part.append(pltpu.roll(x, _C // 2, 1) if hh % 2 else x)
            o = jnp.concatenate(
                [part[0][0:16], jnp.where(row8 < 4, part[0][16:24], part[1][0:8]), part[1][8:24],
                 part[2][0:16], jnp.where(row8 < 4, part[2][16:24], part[3][0:8]), part[3][8:24]],
                axis=0)
            if s > 0:
                o = o + self.a_mem.pop((s, i))
            rows = pl.ds(self.m * (4 * _DH), 4 * _DH)
            ot_scr[tiles * s + i, rows, :] = o.astype(_BF16)

    def attention(which):
        quads = [Quad(m, m) for m in which]
        units = [(quad, s, i, t) for quad in quads for s in range(_NSEG)
                 for i in range(tiles) for t in range(i + 1)]
        left = lax.broadcasted_iota(jnp.int32, (8, _C), 1) < _C // 2
        left_w = lax.broadcasted_iota(jnp.int32, (_C // 4, _C), 1) < _C // 2

        def col_max(x):
            return jnp.broadcast_to(jnp.max(x, axis=0, keepdims=True), (8, _C))

        def weights(x, mx):
            return jnp.exp2(x - jnp.tile(mx, (x.shape[0] // 8, 1))).astype(_BF16)

        scores, run_max, accs = {}, {}, None
        for n in range(len(units) + _LAG):
            if n < len(units):
                quad, s, i, t = units[n]
                if s > 0 and (i, t) == (0, 0):
                    quad.memory_update(s - 1)
                if s > 0 and (i, t) == (1, 1):
                    quad.memory_read(s)
                scores[n] = sc = quad.logits(s, i, t)
                if t < i:
                    cur = [col_max(x) for x in sc]
                else:
                    low = [col_max(x) for x in sc[1]]
                    cur = [jnp.maximum(col_max(x), jnp.where((left if hh % 2 else ~left), low[hh // 2],
                                                             -jnp.inf))
                           for hh, x in enumerate(sc[0])]
                if t > 0:
                    cur = [jnp.maximum(x, y) for x, y in zip(cur, run_max[n - 1])]
                run_max[n] = cur
            if n >= _LAG:
                u = n - _LAG
                quad, s, i, t = units[u]
                sc, mx = scores.pop(u), run_max[u]
                if t < i:
                    ps = [weights(sc[hh], mx[hh]) for hh in range(4)]
                else:
                    low = [pltpu.bitcast(weights(sc[1][c], jnp.where(left, mx[2 * c + 1],
                                                                     mx[2 * c])), _U32)
                           for c in range(2)]
                    ps = [jnp.concatenate(
                        [weights(sc[0][hh], mx[hh]),
                         _as_bf16(jnp.where((left_w if hh % 2 else ~left_w), low[hh // 2], jnp.uint32(0)))],
                        axis=0) for hh in range(4)]
                cur = []
                for hh in range(4):
                    pv = _dot_mixed(quad.values_and_ones(s, t, hh), ps[hh])
                    if t > 0:
                        pv = pv + accs[hh] * jnp.tile(
                            jnp.exp2(run_max[u - 1][hh] - mx[hh]), (3, 1))
                    cur.append(pv)
                accs = cur
                if t == i:
                    quad.store(s, i, accs)

    def first_rows(p):
        for lo in range(_X_SPLIT[p], _X_SPLIT[p + 1], _PIECE):
            project(0, lo, _PIECE, first=True)

    start(small + first_weights + x_copies(0))
    wait(small)
    start(x_copies(1))
    wait(first_weights)
    start(x_copies(2))
    wait(x_copies(0))
    transpose_weights(0)
    first_rows(0)
    start(x_copies(3))
    wait(x_copies(1))
    first_rows(1)
    start(second_batch)
    wait(x_copies(2))
    first_rows(2)
    start(conv_copies(0))
    wait(x_copies(3))
    shift = shift_buf[...].astype(_F32)
    dvec = d_buf[...].astype(_F32).reshape(1, _D)
    for g in range(_NG):
        sl = slice(g * _C, (g + 1) * _C)
        for t in range(_KS):
            par_scr[g, t] = jnp.broadcast_to(shift[t:t + 1, sl], (8, _C))
        par_scr[g, _KS] = jnp.broadcast_to(dvec[:, sl], (8, _C))
        ka_w[g, 0:_PAD // 2, :] = jnp.zeros((_PAD // 2, _C), _U32)
    beta = beta_buf[...].astype(_F32).reshape(1, _H)
    gate = 1.0 / (1.0 + jnp.exp(-beta))
    for hd in range(_H):
        gate_scr[hd] = jnp.broadcast_to(gate[:, hd:hd + 1], (8, _C))
    zero_smem[0] = 0
    zero_smem[1] = 0
    first_rows(3)
    attention(range(1))
    wait(second_batch)

    def phase1(j, carry):
        @pl.when(j > 0)
        def _():
            wait(next_weights(j))

        wait(conv_copies(j)[:3])

        @pl.when(j + 2 < _NG)
        def _():
            start(conv_copies(j + 1) + next_weights(j + 1))

        wait(conv_copies(j)[3:])
        transpose_weights(j + 1)
        jobs = [functools.partial(project, j + 1, lo, _PIECE) for lo in range(0, _S, _PIECE)]
        convolve(j, jobs[:1], jobs[1:])
        outa_copy(j, jnp.where(j == 0, 1, 2)).start()
        return carry

    lax.fori_loop(0, _NG - 1, phase1, 0)

    start(conv_copies(_NG - 1) + [wo_copy])
    wait([outa_copy(0, 1)])
    attention(range(1, _NQ))

    def output_projection(p):
        lo, hi = _OUT_SPLIT[p] // _C, _OUT_SPLIT[p + 1] // _C
        ot = jnp.concatenate([ot_scr[t] for t in range(lo, hi)], axis=1)
        outb_buf[lo * _C:hi * _C, :] = _dot_tn(ot, wo_buf[...]).astype(_BF16)
        outb_copy(p).start()

    n_out = len(_OUT_SPLIT) - 1
    wait(conv_copies(_NG - 1) + [wo_copy])
    convolve(_NG - 1, [], [functools.partial(output_projection, p) for p in range(_OUT_OVERLAP)])
    outa_copy(_NG - 1).start()
    for p in range(_OUT_OVERLAP, n_out):
        output_projection(p)
    wait([outa_copy(j) for j in range(1, _NG)] + [outb_copy(p) for p in range(n_out)])


@jax.jit
def pallas_concat_heads__ssm_conv_h3__memory_aug_infini_attn__prompt_kernel(
    A_q: jax.Array,
    A_k: jax.Array,
    A_v: jax.Array,
    A_shift_k: jax.Array,
    A_ssm_k: jax.Array,
    A_ssm_D: jax.Array,
    B_x: jax.Array,
    B_wq: jax.Array,
    B_wk: jax.Array,
    B_wv: jax.Array,
    B_wo: jax.Array,
    B_beta: jax.Array,
):
    assert A_q.shape == (1, _S, _D) and B_x.shape == (1, _S, _D)
    assert A_shift_k.shape == (_D, _KS) and B_beta.shape == (_H,)
    f_fwd, f_inv = (m.astype(_BF16) for m in _dft_matrices())

    vmem = pltpu.VMEM
    dma = pltpu.SemaphoreType.DMA
    scratch = [
        vmem((_NG, _S, _C), _BF16),
        vmem((_NG, _PAD + _S, _C), _BF16),
        vmem((_NG, _S, _C), _BF16),
        vmem((_NG, _C, _S), _BF16),
        vmem((_S, _D), _BF16),
        vmem((_NG, _S, _C), _BF16),
        vmem((_NG, _D, _C), _BF16),
        vmem((_NG, _D, _C), _BF16),
        vmem((_NG, _D, _C), _BF16),
        vmem((_D, _D), _BF16),
        vmem((_KS, _D), _BF16),
        vmem((_D,), _BF16),
        vmem((_H,), _BF16),
        vmem((2 * _C, _C), _BF16),
        vmem((_C, _C), _BF16),
        vmem((_NG, _KS + 1, 8, _C), _F32),
        vmem((_H, 8, _C), _F32),
        vmem((_S // 2, _C), _U32),
        vmem((_NG, _S, _C), _BF16),
        vmem((_NG, _NG, 2 * _C, _C), _BF16),
        vmem((3, _NC, 2 * _C, _C), _F32),
        pltpu.SMEM((2,), jnp.int32),
        vmem((_NC, _D, _C), _BF16),
        vmem((_NC - _L // _C, _D, _C), _BF16),
        vmem((_NC, _D, _C), _F32),
        vmem((_NG, _S, _C), _BF16),
        vmem((_NG, _S - _L, _C), _BF16),
        vmem((_NC, _D, _C), _BF16),
        vmem((_S, _D), _BF16),
        dma((6,)),
    ]
    out = pl.pallas_call(
        _kernel,
        out_shape=jax.ShapeDtypeStruct((_S, 2 * _D), _BF16),
        in_specs=[pl.BlockSpec(memory_space=pl.ANY)] * 14,
        out_specs=pl.BlockSpec(memory_space=pl.ANY),
        scratch_shapes=scratch,
        compiler_params=pltpu.CompilerParams(vmem_limit_bytes=100 * 1024 * 1024),
        name="h3_infini",
    )(A_q.reshape(_S, _D), A_k.reshape(_S, _D), A_v.reshape(_S, _D), A_shift_k.T,
      A_ssm_k, A_ssm_D, B_x.reshape(_S, _D), B_wq, B_wk, B_wv, B_wo, B_beta,
      f_fwd, f_inv)
    return out.reshape(1, _S, 2 * _D)
```

```python
import functools
import math

import numpy as np
import jax
import jax.numpy as jnp
from jax import lax
import jax.experimental.pallas as pl
import jax.experimental.pallas.tpu as pltpu

_S = 2048
_D = 640
_H = 32
_DH = 20
_NSEG = 4
_L = _S // _NSEG
_KS = 4
_C = 128
_HALF = _C // 2
_NC = _S // _C
_NT = _L // _C
_NG = _D // _C
_QW = 4 * _DH
_NQ = _H // 4

_PIECE = 256
_X_SPLIT = (0, 256, 512, 1024, 2048)
_OUT_SPLIT = (0, 512, 1024, 1536, 1792, 2048)
_OUT_OVERLAP = 2
_PAD = 16
_LAG = 2
_WINDOW = (0, 16, 40, 56)

_F32 = jnp.float32
_BF16 = jnp.bfloat16
_U32 = jnp.uint32
_Q_SCALE = _DH ** -0.5 * math.log2(math.e)


def _dft_matrices():
    even = np.arange(0, _C, 2)
    k = np.concatenate([even, _C - 1 - even])
    ang = np.pi * np.outer(2 * k + 1, np.arange(_C)) / (2 * _C)
    fwd = np.concatenate([np.cos(ang), -np.sin(ang)], axis=0)
    half = np.concatenate([np.cos(ang[:_HALF]), -np.sin(ang[:_HALF])], axis=0).T / _C
    inv = np.concatenate([half[0::2], half[1::2]], axis=0)
    return fwd.astype(np.float32), inv.astype(np.float32)


def _dot(a, b, dims=((1,), (0,))):
    return lax.dot_general(a, b, (dims, ((), ())), preferred_element_type=_F32)


def _as_bf16(words):
    return pltpu.bitcast(words, _BF16)


def _row_pairs(words):
    return tuple(pltpu.unpack_elementwise(words, index=i, packed_dtype=_BF16, unpacked_dtype=_F32)
                 for i in range(2))


def _pack_rows(even, odd):
    return pltpu.pack_elementwise([even, odd], packed_dtype=_BF16)


def _round_bf16(x):
    return x.astype(_BF16).astype(_F32)


def _rows(vreg, like):
    return jnp.tile(vreg, (like.shape[0] // 8, 1))


def _iota(shape, axis):
    return lax.broadcasted_iota(jnp.int32, shape, axis)


def _phi(t):
    return jnp.where(t > 0, t + 1.0, jnp.exp(t))


def _kernel(q_hbm, k_hbm, v_hbm, shift_hbm, h_hbm, d_hbm, x_hbm,
            wq_hbm, wk_hbm, wv_hbm, wo_hbm, beta_hbm, f_hbm, g_hbm, out_hbm,
            qa_buf, ka_buf, va_buf, h_buf, x_raw, wq_buf, wk_buf, wv_buf, wo_buf,
            shift_buf, d_buf, beta_buf, f_buf, g_buf, outa_buf, outb_buf,
            par_scr, gate_scr, kv_scr, z_scr, zero_smem,
            x_scr, wt_scr, qs_scr, pq_scr, vt_scr, kn_scr, pk_scr, ot_scr, sem):
    qa_w, ka_w, va_w, outa_w, f_w, g_w, wk_w, x_w, wt_w, qs_w, pq_w, kn_w, pk_w = (
        ref.bitcast(_U32) for ref in (qa_buf, ka_buf, va_buf, outa_buf, f_buf, g_buf, wk_buf,
                                      x_scr, wt_scr, qs_scr, pq_scr, kn_scr, pk_scr))

    def block(j):
        return pl.ds(j * _C if isinstance(j, int) else pl.multiple_of(j * _C, _C), _C)

    def words(a):
        return slice(a * _HALF, (a + 1) * _HALF)

    cp = pltpu.make_async_copy

    def start(copies):
        for c in copies:
            c.start()

    def wait(copies):
        for c in copies:
            c.wait()

    def weight_copies(j, s):
        return [cp(w.at[:, block(j)], buf.at[j], s)
                for w, buf in ((wk_hbm, wk_buf), (wq_hbm, wq_buf), (wv_hbm, wv_buf))]

    def conv_copies(j):
        s = sem.at[4 + (j & 1)]
        return [cp(k_hbm.at[:, block(j)], ka_buf.at[j, pl.ds(_PAD, _S)], s),
                cp(v_hbm.at[:, block(j)], va_buf.at[j], s),
                cp(q_hbm.at[:, block(j)], qa_buf.at[j], s),
                cp(h_hbm.at[block(j), :], h_buf.at[j], s)]

    def next_weights(j):
        return weight_copies(j + 1, sem.at[4 + (j & 1)])

    def x_copies(p):
        rows = pl.ds(_X_SPLIT[p], _X_SPLIT[p + 1] - _X_SPLIT[p])
        return [cp(x_hbm.at[rows], x_raw.at[rows], sem.at[p % 3])]

    def outa_copy(j, s=2):
        return cp(outa_buf.at[j], out_hbm.at[:, block(j)], sem.at[s])

    def outb_copy(p):
        rows = pl.ds(_OUT_SPLIT[p], _OUT_SPLIT[p + 1] - _OUT_SPLIT[p])
        return cp(outb_buf.at[rows], out_hbm.at[rows, pl.ds(_D, _D)], sem.at[2])

    def transpose_weights(j):
        for w_buf, base in ((wq_buf, 0), (wv_buf, _C)):
            wt = w_buf[j].T
            for g in range(_NG):
                wt_scr[j, g, base:base + _C, :] = wt[:, g * _C:(g + 1) * _C]

    def project(j, lo, first=False):
        n = _PIECE
        if first:
            xs = x_raw[lo:lo + n, :]
            for g in range(_NG):
                x_scr[g, lo:lo + n, :] = xs[:, g * _C:(g + 1) * _C]
        else:
            xs = jnp.concatenate(
                [_as_bf16(x_w[g, lo // 2:(lo + n) // 2, :]) for g in range(_NG)], axis=1)
        wk = jnp.concatenate([_as_bf16(wk_w[j, words(g), :]) for g in range(_NG)], axis=0)
        kn = _dot(xs, wk)
        kn_scr[j, lo:lo + n, :] = kn.astype(_BF16)
        if lo < _S - _L:
            pk_scr[j, lo:lo + n, :] = _phi(kn).astype(_BF16)
        wt = jnp.concatenate([_as_bf16(wt_w[j, g]) for g in range(_NG)], axis=1)
        qv = _dot(wt, xs, ((1,), (1,)))
        for t in range(n // _C):
            tt = lo // _C + t
            qt = qv[0:_C, t * _C:(t + 1) * _C]
            qs_scr[tt, block(j), :] = (qt * _Q_SCALE).astype(_BF16)
            if tt >= _NT:
                pq_scr[tt - _NT, block(j), :] = _phi(qt).astype(_BF16)
            vt_scr[tt, block(j), :] = _round_bf16(qv[_C:2 * _C, t * _C:(t + 1) * _C])

    def filter_spectrum(j, a):
        z_scr[1, a] = _dot(_as_bf16(f_w[...]), h_buf[j, :, a * _C:(a + 1) * _C], ((1,), (1,)))

    def signal_spectrum(j, a):
        lo = _PAD // 2 + a * _HALF
        e0, o0 = _row_pairs(ka_w[j, lo:lo + _HALF, :])
        e1, o1 = _row_pairs(ka_w[j, lo - 1:lo - 1 + _HALF, :])
        _, o2 = _row_pairs(ka_w[j, lo - 2:lo - 2 + _HALF, :])
        w0, w1, w2, w3 = (_rows(par_scr[j, t], e0) for t in range(_KS))
        ve, vo = _row_pairs(va_w[j, words(a), :])
        kv = _pack_rows((e0 * w0 + o1 * w1 + e1 * w2 + o2 * w3) * ve,
                        (o0 * w0 + e0 * w1 + o1 * w2 + e1 * w3) * vo)
        kv_scr[words(a), :] = kv
        z_scr[0, a] = _dot(_as_bf16(f_w[...]), _as_bf16(kv))

    def cross_chunks():
        z_st, z_ld = zero_smem[0], zero_smem[1]
        nb = 4
        for r in range(_NC):
            re, im = slice(8 * r, 8 * r + 8), slice(_C + 8 * r, _C + 8 * r + 8)

            def triple(which, a):
                x, y = z_scr[z_ld + which, a, re, :], z_scr[z_ld + which, a, im, :]
                return x, y, x + y

            prev = None
            for lo in range(0, _NC, nb):
                u, acc = {}, {}
                for t in range(lo + nb):
                    h = triple(1, t)
                    for a in range(max(lo, t), lo + nb):
                        if a - t not in u:
                            u[a - t] = triple(0, a - t)
                        prod = [x * y for x, y in zip(u[a - t], h)]
                        acc[a] = prod if t == 0 else [x + y for x, y in zip(acc[a], prod)]
                outs = []
                for a in range(lo, lo + nb):
                    k1, k2, k3 = acc[a]
                    yr, yi = cur = (k1 - k2, k3 - k1 - k2)
                    if prev is not None:
                        yr, yi = ((yr - prev[1], yi + prev[0]) if r < _NC // 2
                                  else (yr + prev[1], yi - prev[0]))
                    prev = cur
                    outs.append((a, yr, yi))
                for a, yr, yi in outs:
                    z_scr[z_st + 2, a, re, :] = yr
                    z_scr[z_st + 2, a, im, :] = yi

    def finish(j, a):
        y = z_scr[zero_smem[1] + 2, a]
        lo_re, hi_re, lo_im, hi_im = (y[q * _HALF:(q + 1) * _HALF] for q in range(4))
        spec_e = jnp.concatenate([lo_re + hi_re, lo_im - hi_im], axis=0).astype(_BF16)
        spec_o = jnp.concatenate([lo_re - hi_re, lo_im + hi_im], axis=0).astype(_BF16)
        ye = _dot(_as_bf16(g_w[0:_HALF // 2, :]), spec_e)
        yo = _dot(_as_bf16(g_w[_HALF // 2:_HALF, :]), spec_o)
        skip = _rows(par_scr[j, _KS], ye)
        kve, kvo = _row_pairs(kv_scr[words(a), :])
        qe, qo = _row_pairs(qa_w[j, words(a), :])
        outa_w[j, words(a), :] = _pack_rows(qe * (ye + kve * skip), qo * (yo + kvo * skip))

    def convolve(j, before, during):
        for job in before:
            job()
        for a in range(_NC + 4):
            if a < _NC:
                filter_spectrum(j, a)
            if a >= 4:
                signal_spectrum(j, a - 4)
        for job in during:
            job()
        cross_chunks()
        for a in range(_NC):
            finish(j, a)

    row8 = _iota((8, _C), 0)

    class Quad:
        def __init__(self, m):
            self.m = m
            self.wrow = pl.ds(m * _QW // 2, _QW // 2)
            self.mem = None
            self.a_mem, self.keys, self.q = {}, {}, {}

        def gate(self, hh):
            return gate_scr[4 * self.m + hh]

        def window(self, src, lo, n):
            g, off = divmod(self.m * _QW, _C)
            rows = slice(lo // 2, (lo + n) // 2)
            if off == 0:
                return _as_bf16(src[g, rows, :])
            w = jnp.where(_iota((n // 2, _C), 1) >= off, src[g, rows, :],
                          src[min(g + 1, _NG - 1), rows, :])
            return _as_bf16(pltpu.roll(w, _C - off, 1))

        def values(self, s, t, lo, n):
            first = self.m * _QW + lo
            return vt_scr[_NT * s + t, first:first + n, :]

        def values_and_ones(self, s, t, hh):
            v = self.values(s, t, _WINDOW[hh], 24)
            if hh % 2:
                return jnp.concatenate([jnp.where(row8 < 4, 1.0, v[:8]), v[8:]], axis=0)
            return jnp.concatenate([v[:16], jnp.where(row8 < 4, v[16:], 1.0)], axis=0)

        def memory_update(self, s):
            v_ext = jnp.concatenate(
                [jnp.concatenate([self.values(s, t, 0, _QW), jnp.ones((8, _C), _F32)], axis=0)
                 for t in range(_NT)], axis=1)
            row, lane = _iota((_QW + 8, _C), 0), _iota((_QW + 8, _C), 1)
            keep = jnp.zeros((_QW + 8, _C), jnp.bool_)
            for hh in range(4):
                rows = ((row >= _DH * hh) & (row < _DH * (hh + 1))) | (row == _QW + hh)
                keep = keep | (rows & (lane >= _DH * hh) & (lane < _DH * (hh + 1)))
            upd = jnp.where(keep, _dot(v_ext, self.window(pk_w, s * _L, _L)), 0.0)
            self.mem = upd if self.mem is None else self.mem + upd

        def memory_read(self, s):
            pq = jnp.concatenate(
                [_as_bf16(jnp.concatenate(
                    [pq_w[_NT * (s - 1) + i, self.wrow, :],
                     jnp.zeros((_HALF - _QW // 2, _C), _U32)], axis=0))
                 for i in range(_NT)], axis=1)
            got = _dot(_round_bf16(self.mem), pq)
            for i in range(_NT):
                gi = got[:, i * _C:(i + 1) * _C]
                f = [self.gate(hh)
                     / (jnp.broadcast_to(gi[_QW + hh:_QW + hh + 1], (8, _C)) + 1e-6)
                     for hh in range(4)]
                self.a_mem[s, i] = gi[0:_QW] * jnp.concatenate(
                    [f[0], f[0], jnp.where(row8 < 4, f[0], f[1]), f[1], f[1],
                     f[2], f[2], jnp.where(row8 < 4, f[2], f[3]), f[3], f[3]], axis=0)

        def queries(self, s, i):
            if (s, i) not in self.q:
                qq = qs_w[_NT * s + i, self.wrow, :]
                row = _iota((16, _C), 0)
                tiles = []
                for hh in range(4):
                    qh = jnp.where((row >= 2 * hh) & (row < 2 * hh + _DH // 2),
                                   qq[8 * hh:8 * hh + 16], jnp.uint32(0))
                    if hh % 2:
                        qh = pltpu.roll(qh, _HALF, 1)
                    parts = [jnp.zeros((8 * hh, _C), _U32)] if hh > 0 else []
                    parts += [qh, jnp.zeros((_HALF - 16 - 8 * hh, _C), _U32)]
                    tiles.append(jnp.concatenate(parts, axis=0))
                self.q = {(s, i): tiles}
            return self.q[s, i]

        def logits(self, s, i, t):
            if (s, t) not in self.keys:
                self.keys[s, t] = self.window(kn_w, s * _L + t * _C, _C)
            keys, qs = self.keys[s, t], self.queries(s, i)
            all_q = jnp.concatenate([_as_bf16(q) for q in qs], axis=1)
            if t < i:
                sc = _dot(keys, all_q)
                return [sc[:, hh * _C:(hh + 1) * _C] for hh in range(4)]
            key, lane = _iota((_HALF, _C), 0), _iota((_HALF, _C), 1)
            sc = _dot(keys[:_HALF], all_q)
            top = [jnp.where(key <= (lane ^ (_HALF * (hh % 2))), sc[:, hh * _C:(hh + 1) * _C],
                             -jnp.inf) for hh in range(4)]
            pair = jnp.concatenate(
                [_as_bf16(jnp.where(lane < _HALF, qs[hh + 1], qs[hh])) for hh in (0, 2)], axis=1)
            sc = jnp.concatenate(
                [_dot(keys[lo:lo + _HALF // 2], pair) for lo in (_HALF, _HALF + _HALF // 2)],
                axis=0)
            low = [jnp.where(key <= (lane & (_HALF - 1)), sc[:, c * _C:(c + 1) * _C], -jnp.inf)
                   for c in range(2)]
            return top, low

        def store(self, s, i, accs):
            part = []
            for hh in range(4):
                r = 0 if hh % 2 else 23
                norm = (1.0 - self.gate(hh)) / jnp.broadcast_to(accs[hh][r:r + 1], (8, _C))
                x = accs[hh] * _rows(norm, accs[hh])
                part.append(pltpu.roll(x, _HALF, 1) if hh % 2 else x)
            o = jnp.concatenate(
                [part[0][0:16], jnp.where(row8 < 4, part[0][16:24], part[1][0:8]), part[1][8:24],
                 part[2][0:16], jnp.where(row8 < 4, part[2][16:24], part[3][0:8]), part[3][8:24]],
                axis=0)
            if s > 0:
                o = o + self.a_mem.pop((s, i))
            ot_scr[_NT * s + i, self.m * _QW:(self.m + 1) * _QW, :] = o.astype(_BF16)

    def attention(which):
        units = [(quad, s, i, t) for quad in map(Quad, which) for s in range(_NSEG)
                 for i in range(_NT) for t in range(i + 1)]
        left, left_w = _iota((8, _C), 1) < _HALF, _iota((_HALF // 2, _C), 1) < _HALF

        def col_max(x):
            return jnp.broadcast_to(jnp.max(x, axis=0, keepdims=True), (8, _C))

        def weights(x, mx):
            return jnp.exp2(x - _rows(mx, x)).astype(_BF16)

        scores, run_max, accs = {}, {}, None
        for n in range(len(units) + _LAG):
            if n < len(units):
                quad, s, i, t = units[n]
                if s > 0 and (i, t) == (0, 0):
                    quad.memory_update(s - 1)
                if s > 0 and (i, t) == (1, 1):
                    quad.memory_read(s)
                scores[n] = sc = quad.logits(s, i, t)
                if t < i:
                    cur = [col_max(x) for x in sc]
                else:
                    low = [col_max(x) for x in sc[1]]
                    cur = [jnp.maximum(col_max(x),
                                       jnp.where(left if hh % 2 else ~left, low[hh // 2], -jnp.inf))
                           for hh, x in enumerate(sc[0])]
                if t > 0:
                    cur = [jnp.maximum(x, y) for x, y in zip(cur, run_max[n - 1])]
                run_max[n] = cur
            if n >= _LAG:
                u = n - _LAG
                quad, s, i, t = units[u]
                sc, mx = scores.pop(u), run_max[u]
                if t < i:
                    ps = [weights(sc[hh], mx[hh]) for hh in range(4)]
                else:
                    low = [pltpu.bitcast(
                        weights(sc[1][c], jnp.where(left, mx[2 * c + 1], mx[2 * c])), _U32)
                        for c in range(2)]
                    ps = [jnp.concatenate(
                        [weights(sc[0][hh], mx[hh]),
                         _as_bf16(jnp.where(left_w if hh % 2 else ~left_w, low[hh // 2],
                                            jnp.uint32(0)))], axis=0) for hh in range(4)]
                cur = []
                for hh in range(4):
                    pv = _dot(quad.values_and_ones(s, t, hh), ps[hh])
                    if t > 0:
                        pv = pv + accs[hh] * _rows(jnp.exp2(run_max[u - 1][hh] - mx[hh]), pv)
                    cur.append(pv)
                accs = cur
                if t == i:
                    quad.store(s, i, accs)

    def output_projection(p):
        lo, hi = _OUT_SPLIT[p] // _C, _OUT_SPLIT[p + 1] // _C
        ot = jnp.concatenate([ot_scr[t] for t in range(lo, hi)], axis=1)
        outb_buf[lo * _C:hi * _C, :] = _dot(ot, wo_buf[...], ((0,), (0,))).astype(_BF16)
        outb_copy(p).start()

    def first_rows(p):
        for lo in range(_X_SPLIT[p], _X_SPLIT[p + 1], _PIECE):
            project(0, lo, first=True)

    small = [cp(shift_hbm, shift_buf, sem.at[3]), cp(d_hbm, d_buf, sem.at[3]),
             cp(beta_hbm, beta_buf, sem.at[3])]
    first_weights = weight_copies(0, sem.at[0])
    second_batch = [cp(f_hbm, f_buf, sem.at[3]), cp(g_hbm, g_buf, sem.at[3])]
    second_batch += weight_copies(1, sem.at[3])
    wo_copy = cp(wo_hbm, wo_buf, sem.at[4 + ((_NG - 1) & 1)])

    start(small + first_weights + x_copies(0))
    for g in range(_NG):
        ka_w[g, 0:_PAD // 2, :] = jnp.zeros((_PAD // 2, _C), _U32)
    zero_smem[0] = 0
    zero_smem[1] = 0
    wait(first_weights)
    start(x_copies(1) + x_copies(2))
    wait(x_copies(0) + small)
    transpose_weights(0)
    first_rows(0)
    start(x_copies(3))
    wait(x_copies(1))
    first_rows(1)
    start(second_batch)
    wait(x_copies(2))
    first_rows(2)
    start(conv_copies(0))
    wait(x_copies(3))
    shift = shift_buf[...].astype(_F32)
    skip = d_buf[...].astype(_F32).reshape(1, _D)
    for g in range(_NG):
        lanes = slice(g * _C, (g + 1) * _C)
        for t in range(_KS):
            par_scr[g, t] = jnp.broadcast_to(shift[t:t + 1, lanes], (8, _C))
        par_scr[g, _KS] = jnp.broadcast_to(skip[:, lanes], (8, _C))
    gate = 1.0 / (1.0 + jnp.exp(-beta_buf[...].astype(_F32).reshape(1, _H)))
    for hd in range(_H):
        gate_scr[hd] = jnp.broadcast_to(gate[:, hd:hd + 1], (8, _C))
    first_rows(3)
    attention(range(1))
    wait(second_batch)

    def fused(j, carry):
        @pl.when(j > 0)
        def _():
            wait(next_weights(j))

        wait(conv_copies(j)[:3])

        @pl.when(j + 2 < _NG)
        def _():
            start(conv_copies(j + 1) + next_weights(j + 1))

        wait(conv_copies(j)[3:])
        transpose_weights(j + 1)
        jobs = [functools.partial(project, j + 1, lo) for lo in range(0, _S, _PIECE)]
        convolve(j, jobs[:1], jobs[1:])
        outa_copy(j, jnp.where(j == 0, 1, 2)).start()
        return carry

    lax.fori_loop(0, _NG - 1, fused, 0)

    start(conv_copies(_NG - 1) + [wo_copy])
    wait([outa_copy(0, 1)])
    attention(range(1, _NQ))

    n_out = len(_OUT_SPLIT) - 1
    wait(conv_copies(_NG - 1) + [wo_copy])
    convolve(_NG - 1, [], [functools.partial(output_projection, p) for p in range(_OUT_OVERLAP)])
    outa_copy(_NG - 1).start()
    for p in range(_OUT_OVERLAP, n_out):
        output_projection(p)
    wait([outa_copy(j) for j in range(1, _NG)] + [outb_copy(p) for p in range(n_out)])


@jax.jit
def pallas_concat_heads__ssm_conv_h3__memory_aug_infini_attn__prompt_kernel(
    A_q: jax.Array,
    A_k: jax.Array,
    A_v: jax.Array,
    A_shift_k: jax.Array,
    A_ssm_k: jax.Array,
    A_ssm_D: jax.Array,
    B_x: jax.Array,
    B_wq: jax.Array,
    B_wk: jax.Array,
    B_wv: jax.Array,
    B_wo: jax.Array,
    B_beta: jax.Array,
):
    assert A_q.shape == (1, _S, _D) and B_x.shape == (1, _S, _D)
    assert A_shift_k.shape == (_D, _KS) and B_beta.shape == (_H,)
    f_fwd, f_inv = (m.astype(_BF16) for m in _dft_matrices())

    vmem = pltpu.VMEM
    scratch = [
        vmem((_NG, _S, _C), _BF16),
        vmem((_NG, _PAD + _S, _C), _BF16),
        vmem((_NG, _S, _C), _BF16),
        vmem((_NG, _C, _S), _BF16),
        vmem((_S, _D), _BF16),
        vmem((_NG, _D, _C), _BF16),
        vmem((_NG, _D, _C), _BF16),
        vmem((_NG, _D, _C), _BF16),
        vmem((_D, _D), _BF16),
        vmem((_KS, _D), _BF16),
        vmem((_D,), _BF16),
        vmem((_H,), _BF16),
        vmem((2 * _C, _C), _BF16),
        vmem((_C, _C), _BF16),
        vmem((_NG, _S, _C), _BF16),
        vmem((_S, _D), _BF16),
        vmem((_NG, _KS + 1, 8, _C), _F32),
        vmem((_H, 8, _C), _F32),
        vmem((_S // 2, _C), _U32),
        vmem((3, _NC, 2 * _C, _C), _F32),
        pltpu.SMEM((2,), jnp.int32),
        vmem((_NG, _S, _C), _BF16),
        vmem((_NG, _NG, 2 * _C, _C), _BF16),
        vmem((_NC, _D, _C), _BF16),
        vmem((_NC - _NT, _D, _C), _BF16),
        vmem((_NC, _D, _C), _F32),
        vmem((_NG, _S, _C), _BF16),
        vmem((_NG, _S - _L, _C), _BF16),
        vmem((_NC, _D, _C), _BF16),
        pltpu.SemaphoreType.DMA((6,)),
    ]
    out = pl.pallas_call(
        _kernel,
        out_shape=jax.ShapeDtypeStruct((_S, 2 * _D), _BF16),
        in_specs=[pl.BlockSpec(memory_space=pl.ANY)] * 14,
        out_specs=pl.BlockSpec(memory_space=pl.ANY),
        scratch_shapes=scratch,
        compiler_params=pltpu.CompilerParams(
            vmem_limit_bytes=100 * 1024 * 1024, disable_bounds_checks=True),
        name="h3_infini",
    )(A_q.reshape(_S, _D), A_k.reshape(_S, _D), A_v.reshape(_S, _D), A_shift_k.T,
      A_ssm_k, A_ssm_D, B_x.reshape(_S, _D), B_wq, B_wk, B_wv, B_wo, B_beta, f_fwd, f_inv)
    return out.reshape(1, _S, 2 * _D)
```

```python
import functools
import math

import numpy as np
import jax
import jax.numpy as jnp
from jax import lax
import jax.experimental.pallas as pl
import jax.experimental.pallas.tpu as pltpu

_S = 2048
_D = 640
_H = 32
_DH = 20
_NSEG = 4
_L = _S // _NSEG
_KS = 4
_C = 128
_HALF = _C // 2
_NC = _S // _C
_NT = _L // _C
_NG = _D // _C
_QW = 4 * _DH
_NQ = _H // 4

_PIECE = 256
_X_SPLIT = (0, 256, 512, 1024, 2048)
_OUT_SPLIT = (0, 512, 1024, 1536, 1792, 2048)
_OUT_OVERLAP = 2
_PAD = 16
_LAG = 2
_WINDOW = (0, 16, 40, 56)

_F32 = jnp.float32
_BF16 = jnp.bfloat16
_U32 = jnp.uint32
_Q_SCALE = _DH ** -0.5 * math.log2(math.e)


def _dft_matrices():
    even = np.arange(0, _C, 2)
    k = np.concatenate([even, _C - 1 - even])
    ang = np.pi * np.outer(2 * k + 1, np.arange(_C)) / (2 * _C)
    fwd = np.concatenate([np.cos(ang), -np.sin(ang)], axis=0)
    half = np.concatenate([np.cos(ang[:_HALF]), -np.sin(ang[:_HALF])], axis=0).T / _C
    inv = np.concatenate([half[0::2], half[1::2]], axis=0)
    fwd = np.concatenate([fwd, np.concatenate([fwd[:, 0::2], fwd[:, 1::2]], axis=1)], axis=0)
    return fwd.astype(np.float32), inv.astype(np.float32)


def _dot(a, b, dims=((1,), (0,))):
    return lax.dot_general(a, b, (dims, ((), ())), preferred_element_type=_F32)


def _as_bf16(words):
    return pltpu.bitcast(words, _BF16)


def _row_pairs(words):
    return (lax.bitcast_convert_type(words << 16, _F32),
            lax.bitcast_convert_type(words & jnp.uint32(0xFFFF0000), _F32))


def _pack_rows(even, odd):
    n = even.shape[0]
    bits = lax.bitcast_convert_type(_round_bf16(jnp.concatenate([even, odd], axis=0)), _U32)
    return (bits[:n] >> 16) | bits[n:]


def _round_bf16(x):
    return x.astype(_BF16).astype(_F32)


def _rows(vreg, like):
    return jnp.tile(vreg, (like.shape[0] // 8, 1))


def _iota(shape, axis):
    return lax.broadcasted_iota(jnp.int32, shape, axis)


def _phi(t):
    return jnp.where(t > 0, t + 1.0, jnp.exp(t))


def _kernel(q_hbm, k_hbm, v_hbm, shift_hbm, h_hbm, d_hbm, x_hbm,
            wq_hbm, wk_hbm, wv_hbm, wo_hbm, beta_hbm, f_hbm, g_hbm, out_hbm,
            qa_buf, ka_buf, va_buf, h_buf, x_raw, wq_buf, wk_buf, wv_buf, wo_buf,
            shift_buf, d_buf, beta_buf, f_buf, g_buf, outa_buf, outb_buf,
            par_scr, gate_scr, skip_scr, z_scr, zero_smem,
            x_scr, wt_scr, qs_scr, pq_scr, vt_scr, kn_scr, pk_scr, ot_scr, sem):
    qa_w, ka_w, va_w, outa_w, f_w, g_w, wk_w, x_w, wt_w, qs_w, pq_w, kn_w, pk_w = (
        ref.bitcast(_U32) for ref in (qa_buf, ka_buf, va_buf, outa_buf, f_buf, g_buf, wk_buf,
                                      x_scr, wt_scr, qs_scr, pq_scr, kn_scr, pk_scr))

    def block(j):
        return pl.ds(j * _C if isinstance(j, int) else pl.multiple_of(j * _C, _C), _C)

    def words(a):
        return slice(a * _HALF, (a + 1) * _HALF)

    cp = pltpu.make_async_copy

    def start(copies):
        for c in copies:
            c.start()

    def wait(copies):
        for c in copies:
            c.wait()

    def weight_copies(j, s):
        return [cp(w.at[:, block(j)], buf.at[j], s)
                for w, buf in ((wk_hbm, wk_buf), (wq_hbm, wq_buf), (wv_hbm, wv_buf))]

    def signal_copies(j):
        s = sem.at[4 + (j & 1)]
        return [cp(k_hbm.at[:, block(j)], ka_buf.at[j, pl.ds(_PAD, _S)], s),
                cp(v_hbm.at[:, block(j)], va_buf.at[j], s),
                cp(q_hbm.at[:, block(j)], qa_buf.at[j], s)]

    def filter_copy(j):
        return [cp(h_hbm.at[block(j), :], h_buf.at[j], sem.at[4 + (j & 1)])]

    def conv_copies(j):
        return signal_copies(j) + filter_copy(j)

    def next_weights(j):
        return weight_copies(j + 1, sem.at[4 + (j & 1)])

    def x_copies(p):
        rows = pl.ds(_X_SPLIT[p], _X_SPLIT[p + 1] - _X_SPLIT[p])
        return [cp(x_hbm.at[rows], x_raw.at[rows], sem.at[p % 3])]

    def outa_copy(j, s=2):
        return cp(outa_buf.at[j], out_hbm.at[:, block(j)], sem.at[s])

    def outb_copy(p):
        rows = pl.ds(_OUT_SPLIT[p], _OUT_SPLIT[p + 1] - _OUT_SPLIT[p])
        return cp(outb_buf.at[rows], out_hbm.at[rows, pl.ds(_D, _D)], sem.at[2])

    def transpose_weights(j):
        for w_buf, base in ((wq_buf, 0), (wv_buf, _C)):
            wt = w_buf[j].T
            for g in range(_NG):
                wt_scr[j, g, base:base + _C, :] = wt[:, g * _C:(g + 1) * _C]

    def project(j, lo, first=False):
        n = _PIECE
        if first:
            xs = x_raw[lo:lo + n, :]
            for g in range(_NG):
                x_scr[g, lo:lo + n, :] = xs[:, g * _C:(g + 1) * _C]
        else:
            xs = jnp.concatenate(
                [_as_bf16(x_w[g, lo // 2:(lo + n) // 2, :]) for g in range(_NG)], axis=1)
        wk = jnp.concatenate([_as_bf16(wk_w[j, words(g), :]) for g in range(_NG)], axis=0)
        kn = _dot(xs, wk)
        kn_scr[j, lo:lo + n, :] = kn.astype(_BF16)
        if lo < _S - _L:
            pk_scr[j, lo:lo + n, :] = _phi(kn).astype(_BF16)
        wt = jnp.concatenate([_as_bf16(wt_w[j, g]) for g in range(_NG)], axis=1)
        qv = _dot(wt, xs, ((1,), (1,)))
        for t in range(n // _C):
            tt = lo // _C + t
            qt = qv[0:_C, t * _C:(t + 1) * _C]
            qs_scr[tt, block(j), :] = (qt * _Q_SCALE).astype(_BF16)
            if tt >= _NT:
                pq_scr[tt - _NT, block(j), :] = _phi(qt).astype(_BF16)
            vt_scr[tt, block(j), :] = _round_bf16(qv[_C:2 * _C, t * _C:(t + 1) * _C])

    def filter_spectrum(j, a):
        z_scr[1, a] = _dot(_as_bf16(f_w[0:_C, :]), h_buf[j, :, a * _C:(a + 1) * _C],
                           ((1,), (1,)))

    def signal_spectrum(j, a):
        lo = _PAD // 2 + a * _HALF
        e0, o0 = _row_pairs(ka_w[j, lo:lo + _HALF, :])
        e1, o1 = _row_pairs(ka_w[j, lo - 1:lo - 1 + _HALF, :])
        _, o2 = _row_pairs(ka_w[j, lo - 2:lo - 2 + _HALF, :])
        w0, w1, w2, w3 = (_rows(par_scr[j, t], e0) for t in range(_KS))
        ve, vo = _row_pairs(va_w[j, words(a), :])
        kv = jnp.concatenate([(e0 * w0 + o1 * w1 + e1 * w2 + o2 * w3) * ve,
                              (o0 * w0 + e0 * w1 + o1 * w2 + e1 * w3) * vo], axis=0)
        skip_scr[a] = kv * _rows(par_scr[j, _KS], kv)
        z_scr[0, a] = _dot(_as_bf16(f_w[_C:2 * _C, :]), kv.astype(_BF16))

    def cross_chunks():
        z_st, z_ld = zero_smem[0], zero_smem[1]
        nb = 4
        for r in range(_NC):
            re, im = slice(8 * r, 8 * r + 8), slice(_C + 8 * r, _C + 8 * r + 8)

            def triple(which, a):
                x, y = z_scr[z_ld + which, a, re, :], z_scr[z_ld + which, a, im, :]
                return x, y, x + y

            prev = None
            for lo in range(0, _NC, nb):
                u, acc = {}, {}
                for t in range(lo + nb):
                    h = triple(1, t)
                    for a in range(max(lo, t), lo + nb):
                        if a - t not in u:
                            u[a - t] = triple(0, a - t)
                        prod = [x * y for x, y in zip(u[a - t], h)]
                        acc[a] = prod if t == 0 else [x + y for x, y in zip(acc[a], prod)]
                outs = []
                for a in range(lo, lo + nb):
                    k1, k2, k3 = acc[a]
                    yr, yi = cur = (k1 - k2, k3 - k1 - k2)
                    if prev is not None:
                        yr, yi = ((yr - prev[1], yi + prev[0]) if r < _NC // 2
                                  else (yr + prev[1], yi - prev[0]))
                    prev = cur
                    outs.append((a, yr, yi))
                for a, yr, yi in outs:
                    z_scr[z_st + 2, a, re, :] = yr
                    z_scr[z_st + 2, a, im, :] = yi

    def finish(j, a):
        y = z_scr[zero_smem[1] + 2, a]
        lo_re, hi_re, lo_im, hi_im = (y[q * _HALF:(q + 1) * _HALF] for q in range(4))
        spec_e = jnp.concatenate([lo_re + hi_re, lo_im - hi_im], axis=0).astype(_BF16)
        spec_o = jnp.concatenate([lo_re - hi_re, lo_im + hi_im], axis=0).astype(_BF16)
        ye = _dot(_as_bf16(g_w[0:_HALF // 2, :]), spec_e)
        yo = _dot(_as_bf16(g_w[_HALF // 2:_HALF, :]), spec_o)
        qe, qo = _row_pairs(qa_w[j, words(a), :])
        outa_w[j, words(a), :] = _pack_rows(qe * (ye + skip_scr[a, 0:_HALF, :]),
                                            qo * (yo + skip_scr[a, _HALF:_C, :]))

    def convolve(j, before, during):
        for job in before:
            job()
        for a in range(_NC + 4):
            if a < _NC:
                filter_spectrum(j, a)
            if a >= 4:
                signal_spectrum(j, a - 4)
        for job in during:
            job()
        cross_chunks()
        for a in range(_NC):
            finish(j, a)

    row8 = _iota((8, _C), 0)

    class Quad:
        def __init__(self, m):
            self.m = m
            self.wrow = pl.ds(m * _QW // 2, _QW // 2)
            self.mem = None
            self.a_mem, self.keys, self.q = {}, {}, {}

        def gate(self, hh):
            return gate_scr[4 * self.m + hh]

        def window(self, src, lo, n):
            g, off = divmod(self.m * _QW, _C)
            rows = slice(lo // 2, (lo + n) // 2)
            if off == 0:
                return _as_bf16(src[g, rows, :])
            w = jnp.where(_iota((n // 2, _C), 1) >= off, src[g, rows, :],
                          src[min(g + 1, _NG - 1), rows, :])
            return _as_bf16(pltpu.roll(w, _C - off, 1))

        def values(self, s, t, lo, n):
            first = self.m * _QW + lo
            return vt_scr[_NT * s + t, first:first + n, :]

        def values_and_ones(self, s, t, hh):
            v = self.values(s, t, _WINDOW[hh], 24)
            if hh % 2:
                return jnp.concatenate([jnp.where(row8 < 4, 1.0, v[:8]), v[8:]], axis=0)
            return jnp.concatenate([v[:16], jnp.where(row8 < 4, v[16:], 1.0)], axis=0)

        def memory_update(self, s):
            v_ext = jnp.concatenate(
                [jnp.concatenate([self.values(s, t, 0, _QW), jnp.ones((8, _C), _F32)], axis=0)
                 for t in range(_NT)], axis=1)
            row, lane = _iota((_QW + 8, _C), 0), _iota((_QW + 8, _C), 1)
            keep = jnp.zeros((_QW + 8, _C), jnp.bool_)
            for hh in range(4):
                rows = ((row >= _DH * hh) & (row < _DH * (hh + 1))) | (row == _QW + hh)
                keep = keep | (rows & (lane >= _DH * hh) & (lane < _DH * (hh + 1)))
            upd = jnp.where(keep, _dot(v_ext, self.window(pk_w, s * _L, _L)), 0.0)
            self.mem = upd if self.mem is None else self.mem + upd

        def memory_read(self, s):
            pq = jnp.concatenate(
                [_as_bf16(jnp.concatenate(
                    [pq_w[_NT * (s - 1) + i, self.wrow, :],
                     jnp.zeros((_HALF - _QW // 2, _C), _U32)], axis=0))
                 for i in range(_NT)], axis=1)
            got = _dot(_round_bf16(self.mem), pq)
            for i in range(_NT):
                gi = got[:, i * _C:(i + 1) * _C]
                f = [self.gate(hh)
                     / (jnp.broadcast_to(gi[_QW + hh:_QW + hh + 1], (8, _C)) + 1e-6)
                     for hh in range(4)]
                self.a_mem[s, i] = gi[0:_QW] * jnp.concatenate(
                    [f[0], f[0], jnp.where(row8 < 4, f[0], f[1]), f[1], f[1],
                     f[2], f[2], jnp.where(row8 < 4, f[2], f[3]), f[3], f[3]], axis=0)

        def queries(self, s, i):
            if (s, i) not in self.q:
                qq = qs_w[_NT * s + i, self.wrow, :]
                row = _iota((16, _C), 0)
                tiles = []
                for hh in range(4):
                    qh = jnp.where((row >= 2 * hh) & (row < 2 * hh + _DH // 2),
                                   qq[8 * hh:8 * hh + 16], jnp.uint32(0))
                    if hh % 2:
                        qh = pltpu.roll(qh, _HALF, 1)
                    parts = [jnp.zeros((8 * hh, _C), _U32)] if hh > 0 else []
                    parts += [qh, jnp.zeros((_HALF - 16 - 8 * hh, _C), _U32)]
                    tiles.append(jnp.concatenate(parts, axis=0))
                self.q = {(s, i): tiles}
            return self.q[s, i]

        def logits(self, s, i, t):
            if (s, t) not in self.keys:
                self.keys[s, t] = self.window(kn_w, s * _L + t * _C, _C)
            keys, qs = self.keys[s, t], self.queries(s, i)
            all_q = jnp.concatenate([_as_bf16(q) for q in qs], axis=1)
            if t < i:
                sc = _dot(keys, all_q)
                return [sc[:, hh * _C:(hh + 1) * _C] for hh in range(4)]
            key, lane = _iota((_HALF, _C), 0), _iota((_HALF, _C), 1)
            sc = _dot(keys[:_HALF], all_q)
            top = [jnp.where(key <= (lane ^ (_HALF * (hh % 2))), sc[:, hh * _C:(hh + 1) * _C],
                             -jnp.inf) for hh in range(4)]
            pair = jnp.concatenate(
                [_as_bf16(jnp.where(lane < _HALF, qs[hh + 1], qs[hh])) for hh in (0, 2)], axis=1)
            sc = jnp.concatenate(
                [_dot(keys[lo:lo + _HALF // 2], pair) for lo in (_HALF, _HALF + _HALF // 2)],
                axis=0)
            low = [jnp.where(key <= (lane & (_HALF - 1)), sc[:, c * _C:(c + 1) * _C], -jnp.inf)
                   for c in range(2)]
            return top, low

        def store(self, s, i, accs):
            part = []
            for hh in range(4):
                r = 0 if hh % 2 else 23
                norm = (1.0 - self.gate(hh)) / jnp.broadcast_to(accs[hh][r:r + 1], (8, _C))
                x = accs[hh] * _rows(norm, accs[hh])
                part.append(pltpu.roll(x, _HALF, 1) if hh % 2 else x)
            o = jnp.concatenate(
                [part[0][0:16], jnp.where(row8 < 4, part[0][16:24], part[1][0:8]), part[1][8:24],
                 part[2][0:16], jnp.where(row8 < 4, part[2][16:24], part[3][0:8]), part[3][8:24]],
                axis=0)
            if s > 0:
                o = o + self.a_mem.pop((s, i))
            ot_scr[_NT * s + i, self.m * _QW:(self.m + 1) * _QW, :] = o.astype(_BF16)

    def attention(which):
        units = [(quad, s, i, t) for quad in map(Quad, which) for s in range(_NSEG)
                 for i in range(_NT) for t in range(i + 1)]
        left, left_w = _iota((8, _C), 1) < _HALF, _iota((_HALF // 2, _C), 1) < _HALF

        def col_max(x):
            return jnp.broadcast_to(jnp.max(x, axis=0, keepdims=True), (8, _C))

        def weights(x, mx):
            return jnp.exp2(x - _rows(mx, x)).astype(_BF16)

        scores, run_max, accs = {}, {}, None
        for n in range(len(units) + _LAG):
            if n < len(units):
                quad, s, i, t = units[n]
                if s > 0 and (i, t) == (0, 0):
                    quad.memory_update(s - 1)
                if s > 0 and (i, t) == (1, 1):
                    quad.memory_read(s)
                scores[n] = sc = quad.logits(s, i, t)
                if t < i:
                    cur = [col_max(x) for x in sc]
                else:
                    low = [col_max(x) for x in sc[1]]
                    cur = [jnp.maximum(col_max(x),
                                       jnp.where(left if hh % 2 else ~left, low[hh // 2], -jnp.inf))
                           for hh, x in enumerate(sc[0])]
                if t > 0:
                    cur = [jnp.maximum(x, y) for x, y in zip(cur, run_max[n - 1])]
                run_max[n] = cur
            if n >= _LAG:
                u = n - _LAG
                quad, s, i, t = units[u]
                sc, mx = scores.pop(u), run_max[u]
                if t < i:
                    ps = [weights(sc[hh], mx[hh]) for hh in range(4)]
                else:
                    low = [pltpu.bitcast(
                        weights(sc[1][c], jnp.where(left, mx[2 * c + 1], mx[2 * c])), _U32)
                        for c in range(2)]
                    ps = [jnp.concatenate(
                        [weights(sc[0][hh], mx[hh]),
                         _as_bf16(jnp.where(left_w if hh % 2 else ~left_w, low[hh // 2],
                                            jnp.uint32(0)))], axis=0) for hh in range(4)]
                cur = []
                for hh in range(4):
                    pv = _dot(quad.values_and_ones(s, t, hh), ps[hh])
                    if t > 0:
                        pv = pv + accs[hh] * _rows(jnp.exp2(run_max[u - 1][hh] - mx[hh]), pv)
                    cur.append(pv)
                accs = cur
                if t == i:
                    quad.store(s, i, accs)

    def output_projection(p):
        lo, hi = _OUT_SPLIT[p] // _C, _OUT_SPLIT[p + 1] // _C
        ot = jnp.concatenate([ot_scr[t] for t in range(lo, hi)], axis=1)
        outb_buf[lo * _C:hi * _C, :] = _dot(ot, wo_buf[...], ((0,), (0,))).astype(_BF16)
        outb_copy(p).start()

    def first_rows(p):
        for lo in range(_X_SPLIT[p], _X_SPLIT[p + 1], _PIECE):
            project(0, lo, first=True)

    small = [cp(shift_hbm, shift_buf, sem.at[3]), cp(d_hbm, d_buf, sem.at[3]),
             cp(beta_hbm, beta_buf, sem.at[3])]
    first_weights = weight_copies(0, sem.at[0])
    second_batch = [cp(f_hbm, f_buf, sem.at[3]), cp(g_hbm, g_buf, sem.at[3])]
    second_batch += weight_copies(1, sem.at[3])
    wo_copy = cp(wo_hbm, wo_buf, sem.at[4 + ((_NG - 1) & 1)])

    start(small + first_weights + x_copies(0))
    for g in range(_NG):
        ka_w[g, 0:_PAD // 2, :] = jnp.zeros((_PAD // 2, _C), _U32)
    zero_smem[0] = 0
    zero_smem[1] = 0
    wait(first_weights)
    start(x_copies(1) + x_copies(2))
    wait(x_copies(0) + small)
    transpose_weights(0)
    first_rows(0)
    start(x_copies(3))
    wait(x_copies(1))
    first_rows(1)
    start(second_batch)
    wait(x_copies(2))
    first_rows(2)
    start(conv_copies(0))
    wait(x_copies(3))
    shift = shift_buf[...].astype(_F32)
    skip = d_buf[...].astype(_F32).reshape(1, _D)
    for g in range(_NG):
        lanes = slice(g * _C, (g + 1) * _C)
        for t in range(_KS):
            par_scr[g, t] = jnp.broadcast_to(shift[t:t + 1, lanes], (8, _C))
        par_scr[g, _KS] = jnp.broadcast_to(skip[:, lanes], (8, _C))
    gate = 1.0 / (1.0 + jnp.exp(-beta_buf[...].astype(_F32).reshape(1, _H)))
    for hd in range(_H):
        gate_scr[hd] = jnp.broadcast_to(gate[:, hd:hd + 1], (8, _C))
    first_rows(3)
    attention(range(1))
    wait(second_batch)

    def fused(j, carry):
        @pl.when(j > 0)
        def _():
            wait(next_weights(j))

        wait(signal_copies(j))

        @pl.when(j + 2 < _NG)
        def _():
            start(conv_copies(j + 1) + next_weights(j + 1))

        wait(filter_copy(j))
        transpose_weights(j + 1)
        jobs = [functools.partial(project, j + 1, lo) for lo in range(0, _S, _PIECE)]
        convolve(j, jobs[:1], jobs[1:])
        outa_copy(j, jnp.where(j == 0, 1, 2)).start()
        return carry

    lax.fori_loop(0, _NG - 1, fused, 0)

    start(conv_copies(_NG - 1) + [wo_copy])
    wait([outa_copy(0, 1)])
    attention(range(1, _NQ))

    n_out = len(_OUT_SPLIT) - 1
    wait(conv_copies(_NG - 1) + [wo_copy])
    convolve(_NG - 1, [], [functools.partial(output_projection, p) for p in range(_OUT_OVERLAP)])
    outa_copy(_NG - 1).start()
    for p in range(_OUT_OVERLAP, n_out):
        output_projection(p)
    wait([outa_copy(j) for j in range(1, _NG)] + [outb_copy(p) for p in range(n_out)])


@jax.jit
def pallas_concat_heads__ssm_conv_h3__memory_aug_infini_attn__prompt_kernel(
    A_q: jax.Array,
    A_k: jax.Array,
    A_v: jax.Array,
    A_shift_k: jax.Array,
    A_ssm_k: jax.Array,
    A_ssm_D: jax.Array,
    B_x: jax.Array,
    B_wq: jax.Array,
    B_wk: jax.Array,
    B_wv: jax.Array,
    B_wo: jax.Array,
    B_beta: jax.Array,
):
    assert A_q.shape == (1, _S, _D) and B_x.shape == (1, _S, _D)
    assert A_shift_k.shape == (_D, _KS) and B_beta.shape == (_H,)
    f_fwd, f_inv = (m.astype(_BF16) for m in _dft_matrices())

    vmem = pltpu.VMEM
    scratch = [
        vmem((_NG, _S, _C), _BF16),
        vmem((_NG, _PAD + _S, _C), _BF16),
        vmem((_NG, _S, _C), _BF16),
        vmem((_NG, _C, _S), _BF16),
        vmem((_S, _D), _BF16),
        vmem((_NG, _D, _C), _BF16),
        vmem((_NG, _D, _C), _BF16),
        vmem((_NG, _D, _C), _BF16),
        vmem((_D, _D), _BF16),
        vmem((_KS, _D), _BF16),
        vmem((_D,), _BF16),
        vmem((_H,), _BF16),
        vmem((4 * _C, _C), _BF16),
        vmem((_C, _C), _BF16),
        vmem((_NG, _S, _C), _BF16),
        vmem((_S, _D), _BF16),
        vmem((_NG, _KS + 1, 8, _C), _F32),
        vmem((_H, 8, _C), _F32),
        vmem((_NC, _C, _C), _F32),
        vmem((3, _NC, 2 * _C, _C), _F32),
        pltpu.SMEM((2,), jnp.int32),
        vmem((_NG, _S, _C), _BF16),
        vmem((_NG, _NG, 2 * _C, _C), _BF16),
        vmem((_NC, _D, _C), _BF16),
        vmem((_NC - _NT, _D, _C), _BF16),
        vmem((_NC, _D, _C), _F32),
        vmem((_NG, _S, _C), _BF16),
        vmem((_NG, _S - _L, _C), _BF16),
        vmem((_NC, _D, _C), _BF16),
        pltpu.SemaphoreType.DMA((6,)),
    ]
    out = pl.pallas_call(
        _kernel,
        out_shape=jax.ShapeDtypeStruct((_S, 2 * _D), _BF16),
        in_specs=[pl.BlockSpec(memory_space=pl.ANY)] * 14,
        out_specs=pl.BlockSpec(memory_space=pl.ANY),
        scratch_shapes=scratch,
        compiler_params=pltpu.CompilerParams(
            vmem_limit_bytes=100 * 1024 * 1024, disable_bounds_checks=True),
        name="h3_infini",
    )(A_q.reshape(_S, _D), A_k.reshape(_S, _D), A_v.reshape(_S, _D), A_shift_k.T,
      A_ssm_k, A_ssm_D, B_x.reshape(_S, _D), B_wq, B_wk, B_wv, B_wo, B_beta, f_fwd, f_inv)
    return out.reshape(1, _S, 2 * _D)
```

```python
import functools
import math

import numpy as np
import jax
import jax.numpy as jnp
from jax import lax
import jax.experimental.pallas as pl
import jax.experimental.pallas.tpu as pltpu

_S = 2048
_D = 640
_H = 32
_DH = 20
_NSEG = 4
_L = _S // _NSEG
_KS = 4
_C = 128
_HALF = _C // 2
_NC = _S // _C
_NT = _L // _C
_NG = _D // _C
_QW = 4 * _DH
_NQ = _H // 4

_PIECE = 256
_X_SPLIT = (0, 256, 512, 1024, 2048)
_OUT_SPLIT = tuple(range(0, _S + 1, 256))
_OUT_OVERLAP = 4
_PAD = 16
_LAG = 2
_WINDOW = (0, 16, 40, 56)

_F32 = jnp.float32
_BF16 = jnp.bfloat16
_U32 = jnp.uint32
_Q_SCALE = _DH ** -0.5 * math.log2(math.e)


def _dft_matrices():
    even = np.arange(0, _C, 2)
    k = np.concatenate([even, _C - 1 - even])
    ang = np.pi * np.outer(2 * k + 1, np.arange(_C)) / (2 * _C)
    fwd = np.concatenate([np.cos(ang), -np.sin(ang)], axis=0)
    half = np.concatenate([np.cos(ang[:_HALF]), -np.sin(ang[:_HALF])], axis=0).T / _C
    inv = np.concatenate([half[0::2], half[1::2]], axis=0)
    fwd = np.concatenate([fwd, np.concatenate([fwd[:, 0::2], fwd[:, 1::2]], axis=1)], axis=0)
    return fwd.astype(np.float32), inv.astype(np.float32)


def _dot(a, b, dims=((1,), (0,))):
    return lax.dot_general(a, b, (dims, ((), ())), preferred_element_type=_F32)


def _as_bf16(words):
    return pltpu.bitcast(words, _BF16)


def _row_pairs(words):
    return (lax.bitcast_convert_type(words << 16, _F32),
            lax.bitcast_convert_type(words & jnp.uint32(0xFFFF0000), _F32))


def _pack_rows(even, odd):
    n = even.shape[0]
    bits = lax.bitcast_convert_type(_round_bf16(jnp.concatenate([even, odd], axis=0)), _U32)
    return (bits[:n] >> 16) | bits[n:]


def _round_bf16(x):
    return x.astype(_BF16).astype(_F32)


def _rows(vreg, like):
    return jnp.tile(vreg, (like.shape[0] // 8, 1))


def _iota(shape, axis):
    return lax.broadcasted_iota(jnp.int32, shape, axis)


def _phi(t):
    return jnp.where(t > 0, t + 1.0, jnp.exp(t))


def _kernel(q_hbm, k_hbm, v_hbm, shift_hbm, h_hbm, d_hbm, x_hbm,
            wq_hbm, wk_hbm, wv_hbm, wo_hbm, beta_hbm, f_hbm, g_hbm, out_hbm,
            qa_buf, ka_buf, va_buf, h_buf, x_buf, wq_buf, wk_buf, wv_buf, wo_buf,
            shift_buf, d_buf, beta_buf, f_buf, g_buf, outa_buf, outb_buf,
            par_scr, gate_scr, skip_scr, z_scr, zero_smem,
            wt_scr, qs_scr, pq_scr, vt_scr, kn_scr, pk_scr, ot_scr, sem):
    qa_w, ka_w, va_w, outa_w, f_w, g_w, wk_w, wt_w, qs_w, pq_w, kn_w, pk_w = (
        ref.bitcast(_U32) for ref in (qa_buf, ka_buf, va_buf, outa_buf, f_buf, g_buf, wk_buf,
                                      wt_scr, qs_scr, pq_scr, kn_scr, pk_scr))

    def block(j):
        return pl.ds(j * _C if isinstance(j, int) else pl.multiple_of(j * _C, _C), _C)

    def words(a):
        return slice(a * _HALF, (a + 1) * _HALF)

    cp = pltpu.make_async_copy

    def start(copies):
        for c in copies:
            c.start()

    def wait(copies):
        for c in copies:
            c.wait()

    def weight_copies(j, s):
        return [cp(w.at[:, block(j)], buf.at[j], s)
                for w, buf in ((wk_hbm, wk_buf), (wq_hbm, wq_buf), (wv_hbm, wv_buf))]

    def signal_copies(j):
        s = sem.at[4 + (j & 1)]
        return [cp(k_hbm.at[:, block(j)], ka_buf.at[j, pl.ds(_PAD, _S)], s),
                cp(v_hbm.at[:, block(j)], va_buf.at[j], s),
                cp(q_hbm.at[:, block(j)], qa_buf.at[j], s)]

    def filter_copy(j):
        return [cp(h_hbm.at[block(j), :], h_buf.at[j], sem.at[4 + (j & 1)])]

    def conv_copies(j):
        return signal_copies(j) + filter_copy(j)

    def next_weights(j):
        return weight_copies(j + 1, sem.at[4 + (j & 1)])

    def x_copies(p):
        rows = pl.ds(_X_SPLIT[p], _X_SPLIT[p + 1] - _X_SPLIT[p])
        return [cp(x_hbm.at[rows], x_buf.at[rows], sem.at[p % 3])]

    def outa_copy(j, s=2):
        return cp(outa_buf.at[j], out_hbm.at[:, block(j)], sem.at[s])

    def outb_copy(p):
        rows = pl.ds(_OUT_SPLIT[p], _OUT_SPLIT[p + 1] - _OUT_SPLIT[p])
        return cp(outb_buf.at[rows], out_hbm.at[rows, pl.ds(_D, _D)], sem.at[2])

    def transpose_weights(j):
        for w_buf, base in ((wq_buf, 0), (wv_buf, _C)):
            wt = w_buf[j].T
            for g in range(_NG):
                wt_scr[j, g, base:base + _C, :] = wt[:, g * _C:(g + 1) * _C]

    def project(j, lo):
        n = _PIECE
        xs = x_buf[lo:lo + n, :]
        wk = jnp.concatenate([_as_bf16(wk_w[j, words(g), :]) for g in range(_NG)], axis=0)
        kn = _dot(xs, wk)
        kn_scr[j, lo:lo + n, :] = kn.astype(_BF16)
        if lo < _S - _L:
            pk_scr[j, lo:lo + n, :] = _phi(kn).astype(_BF16)
        wt = jnp.concatenate([_as_bf16(wt_w[j, g]) for g in range(_NG)], axis=1)
        qv = _dot(wt, xs, ((1,), (1,)))
        for t in range(n // _C):
            tt = lo // _C + t
            qt = qv[0:_C, t * _C:(t + 1) * _C]
            qs_scr[tt, block(j), :] = (qt * _Q_SCALE).astype(_BF16)
            if tt >= _NT:
                pq_scr[tt - _NT, block(j), :] = _phi(qt).astype(_BF16)
            vt_scr[tt, block(j), :] = _round_bf16(qv[_C:2 * _C, t * _C:(t + 1) * _C])

    def filter_spectrum(j, a):
        z_scr[1, a] = _dot(_as_bf16(f_w[0:_C, :]), h_buf[j, :, a * _C:(a + 1) * _C],
                           ((1,), (1,)))

    def signal_spectrum(j, a):
        lo = _PAD // 2 + a * _HALF
        e0, o0 = _row_pairs(ka_w[j, lo:lo + _HALF, :])
        e1, o1 = _row_pairs(ka_w[j, lo - 1:lo - 1 + _HALF, :])
        _, o2 = _row_pairs(ka_w[j, lo - 2:lo - 2 + _HALF, :])
        w0, w1, w2, w3 = (_rows(par_scr[j, t], e0) for t in range(_KS))
        ve, vo = _row_pairs(va_w[j, words(a), :])
        kv = jnp.concatenate([(e0 * w0 + o1 * w1 + e1 * w2 + o2 * w3) * ve,
                              (o0 * w0 + e0 * w1 + o1 * w2 + e1 * w3) * vo], axis=0)
        skip_scr[a] = kv * _rows(par_scr[j, _KS], kv)
        z_scr[0, a] = _dot(_as_bf16(f_w[_C:2 * _C, :]), kv.astype(_BF16))

    def cross_chunks():
        z_st, z_ld = zero_smem[0], zero_smem[1]
        nb = 4
        for r in range(_NC):
            re, im = slice(8 * r, 8 * r + 8), slice(_C + 8 * r, _C + 8 * r + 8)

            def triple(which, a):
                x, y = z_scr[z_ld + which, a, re, :], z_scr[z_ld + which, a, im, :]
                return x, y, x + y

            prev = None
            for lo in range(0, _NC, nb):
                u, acc = {}, {}
                for t in range(lo + nb):
                    h = triple(1, t)
                    for a in range(max(lo, t), lo + nb):
                        if a - t not in u:
                            u[a - t] = triple(0, a - t)
                        prod = [x * y for x, y in zip(u[a - t], h)]
                        acc[a] = prod if t == 0 else [x + y for x, y in zip(acc[a], prod)]
                outs = []
                for a in range(lo, lo + nb):
                    k1, k2, k3 = acc[a]
                    yr, yi = cur = (k1 - k2, k3 - k1 - k2)
                    if prev is not None:
                        yr, yi = ((yr - prev[1], yi + prev[0]) if r < _NC // 2
                                  else (yr + prev[1], yi - prev[0]))
                    prev = cur
                    outs.append((a, yr, yi))
                for a, yr, yi in outs:
                    z_scr[z_st + 2, a, re, :] = yr
                    z_scr[z_st + 2, a, im, :] = yi

    def finish(j, a):
        y = z_scr[zero_smem[1] + 2, a]
        lo_re, hi_re, lo_im, hi_im = (y[q * _HALF:(q + 1) * _HALF] for q in range(4))
        spec_e = jnp.concatenate([lo_re + hi_re, lo_im - hi_im], axis=0).astype(_BF16)
        spec_o = jnp.concatenate([lo_re - hi_re, lo_im + hi_im], axis=0).astype(_BF16)
        ye = _dot(_as_bf16(g_w[0:_HALF // 2, :]), spec_e)
        yo = _dot(_as_bf16(g_w[_HALF // 2:_HALF, :]), spec_o)
        qe, qo = _row_pairs(qa_w[j, words(a), :])
        outa_w[j, words(a), :] = _pack_rows(qe * (ye + skip_scr[a, 0:_HALF, :]),
                                            qo * (yo + skip_scr[a, _HALF:_C, :]))

    def convolve(j, before, during):
        for job in before:
            job()
        for a in range(_NC + 4):
            if a < _NC:
                filter_spectrum(j, a)
            if a >= 4:
                signal_spectrum(j, a - 4)
        for job in during:
            job()
        cross_chunks()
        for a in range(_NC):
            finish(j, a)

    row8 = _iota((8, _C), 0)

    class Quad:
        def __init__(self, m):
            self.m = m
            self.wrow = pl.ds(m * _QW // 2, _QW // 2)
            self.mem = None
            self.a_mem, self.keys, self.q = {}, {}, {}

        def gate(self, hh):
            return gate_scr[4 * self.m + hh]

        def window(self, src, lo, n):
            g, off = divmod(self.m * _QW, _C)
            rows = slice(lo // 2, (lo + n) // 2)
            if off == 0:
                return _as_bf16(src[g, rows, :])
            w = jnp.where(_iota((n // 2, _C), 1) >= off, src[g, rows, :],
                          src[min(g + 1, _NG - 1), rows, :])
            return _as_bf16(pltpu.roll(w, _C - off, 1))

        def natural_window(self, src, lo, n):
            g, off = divmod(self.m * _QW, _C)
            rows = slice(lo // 2, (lo + n) // 2)
            if off + _QW <= _C:
                return _as_bf16(src[g, rows, :])
            return _as_bf16(jnp.where(_iota((n // 2, _C), 1) >= off, src[g, rows, :],
                                      src[g + 1, rows, :]))

        def values(self, s, t, lo, n):
            first = self.m * _QW + lo
            return vt_scr[_NT * s + t, first:first + n, :]

        def values_and_ones(self, s, t, hh):
            v = self.values(s, t, _WINDOW[hh], 24)
            if hh % 2:
                return jnp.concatenate([jnp.where(row8 < 4, 1.0, v[:8]), v[8:]], axis=0)
            return jnp.concatenate([v[:16], jnp.where(row8 < 4, v[16:], 1.0)], axis=0)

        def memory_update(self, s):
            v_ext = jnp.concatenate(
                [jnp.concatenate([self.values(s, t, 0, _QW), jnp.ones((8, _C), _F32)], axis=0)
                 for t in range(_NT)], axis=1)
            row = _iota((_QW + 8, _C), 0)
            lane = (_iota((_QW + 8, _C), 1) - self.m * _QW % _C) & (_C - 1)
            keep = jnp.zeros((_QW + 8, _C), jnp.bool_)
            for hh in range(4):
                rows = ((row >= _DH * hh) & (row < _DH * (hh + 1))) | (row == _QW + hh)
                keep = keep | (rows & (lane >= _DH * hh) & (lane < _DH * (hh + 1)))
            upd = jnp.where(keep, _dot(v_ext, self.natural_window(pk_w, s * _L, _L)), 0.0)
            self.mem = upd if self.mem is None else self.mem + upd

        def memory_read(self, s):
            tiles = []
            for i in range(_NT):
                w = pq_w[_NT * (s - 1) + i, self.wrow, :]
                slots = [jnp.zeros((8, _C), _U32)] * 8
                for t in range(_QW // 16):
                    slots[(self.m * _QW // 16 + t) % 8] = w[8 * t:8 * t + 8]
                tiles.append(_as_bf16(jnp.concatenate(slots, axis=0)))
            pq = jnp.concatenate(tiles, axis=1)
            got = _dot(_round_bf16(self.mem), pq)
            for i in range(_NT):
                gi = got[:, i * _C:(i + 1) * _C]
                f = [self.gate(hh)
                     / (jnp.broadcast_to(gi[_QW + hh:_QW + hh + 1], (8, _C)) + 1e-6)
                     for hh in range(4)]
                self.a_mem[s, i] = gi[0:_QW] * jnp.concatenate(
                    [f[0], f[0], jnp.where(row8 < 4, f[0], f[1]), f[1], f[1],
                     f[2], f[2], jnp.where(row8 < 4, f[2], f[3]), f[3], f[3]], axis=0)

        def queries(self, s, i):
            if (s, i) not in self.q:
                qq = qs_w[_NT * s + i, self.wrow, :]
                row = _iota((16, _C), 0)
                tiles = []
                for hh in range(4):
                    qh = jnp.where((row >= 2 * hh) & (row < 2 * hh + _DH // 2),
                                   qq[8 * hh:8 * hh + 16], jnp.uint32(0))
                    if hh % 2:
                        qh = pltpu.roll(qh, _HALF, 1)
                    parts = [jnp.zeros((8 * hh, _C), _U32)] if hh > 0 else []
                    parts += [qh, jnp.zeros((_HALF - 16 - 8 * hh, _C), _U32)]
                    tiles.append(jnp.concatenate(parts, axis=0))
                self.q = {(s, i): tiles}
            return self.q[s, i]

        def logits(self, s, i, t):
            if (s, t) not in self.keys:
                self.keys[s, t] = self.window(kn_w, s * _L + t * _C, _C)
            keys, qs = self.keys[s, t], self.queries(s, i)
            all_q = jnp.concatenate([_as_bf16(q) for q in qs], axis=1)
            if t < i:
                sc = _dot(keys, all_q)
                return [sc[:, hh * _C:(hh + 1) * _C] for hh in range(4)]
            key, lane = _iota((_HALF, _C), 0), _iota((_HALF, _C), 1)
            sc = _dot(keys[:_HALF], all_q)
            top = [jnp.where(key <= (lane ^ (_HALF * (hh % 2))), sc[:, hh * _C:(hh + 1) * _C],
                             -jnp.inf) for hh in range(4)]
            pair = jnp.concatenate(
                [_as_bf16(jnp.where(lane < _HALF, qs[hh + 1], qs[hh])) for hh in (0, 2)], axis=1)
            sc = jnp.concatenate(
                [_dot(keys[lo:lo + _HALF // 2], pair) for lo in (_HALF, _HALF + _HALF // 2)],
                axis=0)
            low = [jnp.where(key <= (lane & (_HALF - 1)), sc[:, c * _C:(c + 1) * _C], -jnp.inf)
                   for c in range(2)]
            return top, low

        def store(self, s, i, accs):
            part = []
            for hh in range(4):
                r = 0 if hh % 2 else 23
                norm = (1.0 - self.gate(hh)) / jnp.broadcast_to(accs[hh][r:r + 1], (8, _C))
                x = accs[hh] * _rows(norm, accs[hh])
                part.append(pltpu.roll(x, _HALF, 1) if hh % 2 else x)
            o = jnp.concatenate(
                [part[0][0:16], jnp.where(row8 < 4, part[0][16:24], part[1][0:8]), part[1][8:24],
                 part[2][0:16], jnp.where(row8 < 4, part[2][16:24], part[3][0:8]), part[3][8:24]],
                axis=0)
            if s > 0:
                o = o + self.a_mem.pop((s, i))
            ot_scr[_NT * s + i, self.m * _QW:(self.m + 1) * _QW, :] = o.astype(_BF16)

    def attention(which):
        units = [(quad, s, i, t) for quad in map(Quad, which) for s in range(_NSEG)
                 for i in range(_NT) for t in range(i + 1)]
        left, left_w = _iota((8, _C), 1) < _HALF, _iota((_HALF // 2, _C), 1) < _HALF

        def col_max(x):
            return jnp.broadcast_to(jnp.max(x, axis=0, keepdims=True), (8, _C))

        def weights(x, mx):
            return jnp.exp2(x - _rows(mx, x)).astype(_BF16)

        scores, run_max, accs = {}, {}, None
        for n in range(len(units) + _LAG):
            if n < len(units):
                quad, s, i, t = units[n]
                if s > 0 and (i, t) == (0, 0):
                    quad.memory_update(s - 1)
                if s > 0 and (i, t) == (1, 1):
                    quad.memory_read(s)
                scores[n] = sc = quad.logits(s, i, t)
                if t < i:
                    cur = [col_max(x) for x in sc]
                else:
                    low = [col_max(x) for x in sc[1]]
                    cur = [jnp.maximum(col_max(x),
                                       jnp.where(left if hh % 2 else ~left, low[hh // 2], -jnp.inf))
                           for hh, x in enumerate(sc[0])]
                if t > 0:
                    cur = [jnp.maximum(x, y) for x, y in zip(cur, run_max[n - 1])]
                run_max[n] = cur
            if n >= _LAG:
                u = n - _LAG
                quad, s, i, t = units[u]
                sc, mx = scores.pop(u), run_max[u]
                if t < i:
                    ps = [weights(sc[hh], mx[hh]) for hh in range(4)]
                else:
                    low = [pltpu.bitcast(
                        weights(sc[1][c], jnp.where(left, mx[2 * c + 1], mx[2 * c])), _U32)
                        for c in range(2)]
                    ps = [jnp.concatenate(
                        [weights(sc[0][hh], mx[hh]),
                         _as_bf16(jnp.where(left_w if hh % 2 else ~left_w, low[hh // 2],
                                            jnp.uint32(0)))], axis=0) for hh in range(4)]
                cur = []
                for hh in range(4):
                    pv = _dot(quad.values_and_ones(s, t, hh), ps[hh])
                    if t > 0:
                        pv = pv + accs[hh] * _rows(jnp.exp2(run_max[u - 1][hh] - mx[hh]), pv)
                    cur.append(pv)
                accs = cur
                if t == i:
                    quad.store(s, i, accs)

    def output_projection(p):
        lo, hi = _OUT_SPLIT[p] // _C, _OUT_SPLIT[p + 1] // _C
        ot = jnp.concatenate([ot_scr[t] for t in range(lo, hi)], axis=1)
        outb_buf[lo * _C:hi * _C, :] = _dot(ot, wo_buf[...], ((0,), (0,))).astype(_BF16)
        outb_copy(p).start()

    def first_rows(p):
        for lo in range(_X_SPLIT[p], _X_SPLIT[p + 1], _PIECE):
            project(0, lo)

    small = [cp(shift_hbm, shift_buf, sem.at[3]), cp(d_hbm, d_buf, sem.at[3]),
             cp(beta_hbm, beta_buf, sem.at[3])]
    first_weights = weight_copies(0, sem.at[0])
    second_batch = [cp(f_hbm, f_buf, sem.at[3]), cp(g_hbm, g_buf, sem.at[3])]
    second_batch += weight_copies(1, sem.at[3])
    wo_copy = cp(wo_hbm, wo_buf, sem.at[4 + ((_NG - 1) & 1)])

    start(small + first_weights + x_copies(0))
    for g in range(_NG):
        ka_w[g, 0:_PAD // 2, :] = jnp.zeros((_PAD // 2, _C), _U32)
    zero_smem[0] = 0
    zero_smem[1] = 0
    wait(first_weights)
    start(x_copies(1) + x_copies(2))
    wait(x_copies(0) + small)
    transpose_weights(0)
    first_rows(0)
    start(x_copies(3))
    wait(x_copies(1))
    first_rows(1)
    wait(x_copies(2))
    first_rows(2)
    start(second_batch + conv_copies(0))
    wait(x_copies(3))
    shift = shift_buf[...].astype(_F32)
    skip = d_buf[...].astype(_F32).reshape(1, _D)
    for g in range(_NG):
        lanes = slice(g * _C, (g + 1) * _C)
        for t in range(_KS):
            par_scr[g, t] = jnp.broadcast_to(shift[t:t + 1, lanes], (8, _C))
        par_scr[g, _KS] = jnp.broadcast_to(skip[:, lanes], (8, _C))
    gate = 1.0 / (1.0 + jnp.exp(-beta_buf[...].astype(_F32).reshape(1, _H)))
    for hd in range(_H):
        gate_scr[hd] = jnp.broadcast_to(gate[:, hd:hd + 1], (8, _C))
    first_rows(3)
    attention(range(1))
    wait(second_batch)

    def fused(j, carry):
        @pl.when(j > 0)
        def _():
            wait(next_weights(j))

        wait(signal_copies(j))

        @pl.when(j + 2 < _NG)
        def _():
            start(conv_copies(j + 1) + next_weights(j + 1))

        wait(filter_copy(j))
        transpose_weights(j + 1)
        jobs = [functools.partial(project, j + 1, lo) for lo in range(0, _S, _PIECE)]
        convolve(j, jobs[:1], jobs[1:])
        outa_copy(j, jnp.where(j == 0, 1, 2)).start()
        return carry

    lax.fori_loop(0, _NG - 1, fused, 0)

    start(conv_copies(_NG - 1) + [wo_copy])
    wait([outa_copy(0, 1)])
    attention(range(1, _NQ))

    n_out = len(_OUT_SPLIT) - 1
    wait(conv_copies(_NG - 1) + [wo_copy])
    convolve(_NG - 1, [], [functools.partial(output_projection, p) for p in range(_OUT_OVERLAP)])
    outa_copy(_NG - 1).start()
    for p in range(_OUT_OVERLAP, n_out):
        output_projection(p)
    wait([outa_copy(j) for j in range(1, _NG)] + [outb_copy(p) for p in range(n_out)])


@jax.jit
def pallas_concat_heads__ssm_conv_h3__memory_aug_infini_attn__prompt_kernel(
    A_q: jax.Array,
    A_k: jax.Array,
    A_v: jax.Array,
    A_shift_k: jax.Array,
    A_ssm_k: jax.Array,
    A_ssm_D: jax.Array,
    B_x: jax.Array,
    B_wq: jax.Array,
    B_wk: jax.Array,
    B_wv: jax.Array,
    B_wo: jax.Array,
    B_beta: jax.Array,
):
    assert A_q.shape == (1, _S, _D) and B_x.shape == (1, _S, _D)
    assert A_shift_k.shape == (_D, _KS) and B_beta.shape == (_H,)
    f_fwd, f_inv = (m.astype(_BF16) for m in _dft_matrices())

    vmem = pltpu.VMEM
    scratch = [
        vmem((_NG, _S, _C), _BF16),
        vmem((_NG, _PAD + _S, _C), _BF16),
        vmem((_NG, _S, _C), _BF16),
        vmem((_NG, _C, _S), _BF16),
        vmem((_S, _D), _BF16),
        vmem((_NG, _D, _C), _BF16),
        vmem((_NG, _D, _C), _BF16),
        vmem((_NG, _D, _C), _BF16),
        vmem((_D, _D), _BF16),
        vmem((_KS, _D), _BF16),
        vmem((_D,), _BF16),
        vmem((_H,), _BF16),
        vmem((4 * _C, _C), _BF16),
        vmem((_C, _C), _BF16),
        vmem((_NG, _S, _C), _BF16),
        vmem((_S, _D), _BF16),
        vmem((_NG, _KS + 1, 8, _C), _F32),
        vmem((_H, 8, _C), _F32),
        vmem((_NC, _C, _C), _F32),
        vmem((3, _NC, 2 * _C, _C), _F32),
        pltpu.SMEM((2,), jnp.int32),
        vmem((_NG, _NG, 2 * _C, _C), _BF16),
        vmem((_NC, _D, _C), _BF16),
        vmem((_NC - _NT, _D, _C), _BF16),
        vmem((_NC, _D, _C), _F32),
        vmem((_NG, _S, _C), _BF16),
        vmem((_NG, _S - _L, _C), _BF16),
        vmem((_NC, _D, _C), _BF16),
        pltpu.SemaphoreType.DMA((6,)),
    ]
    out = pl.pallas_call(
        _kernel,
        out_shape=jax.ShapeDtypeStruct((_S, 2 * _D), _BF16),
        in_specs=[pl.BlockSpec(memory_space=pl.ANY)] * 14,
        out_specs=pl.BlockSpec(memory_space=pl.ANY),
        scratch_shapes=scratch,
        compiler_params=pltpu.CompilerParams(
            vmem_limit_bytes=100 * 1024 * 1024, disable_bounds_checks=True),
        name="h3_infini",
    )(A_q.reshape(_S, _D), A_k.reshape(_S, _D), A_v.reshape(_S, _D), A_shift_k.T,
      A_ssm_k, A_ssm_D, B_x.reshape(_S, _D), B_wq, B_wk, B_wv, B_wo, B_beta, f_fwd, f_inv)
    return out.reshape(1, _S, 2 * _D)
```

```python
import functools
import math

import numpy as np
import jax
import jax.numpy as jnp
from jax import lax
import jax.experimental.pallas as pl
import jax.experimental.pallas.tpu as pltpu

_S = 2048
_D = 640
_H = 32
_DH = 20
_NSEG = 4
_L = _S // _NSEG
_KS = 4
_C = 128
_HALF = _C // 2
_NC = _S // _C
_NT = _L // _C
_NG = _D // _C
_QW = 4 * _DH
_NQ = _H // 4

_PIECE = 256
_X_SPLIT = (0, 256, 512, 1024, 1536, 2048)
_OUT_SPLIT = tuple(range(0, _S + 1, 256))
_OUT_OVERLAP = 4
_PAD = 16
_LAG = 2
_WINDOW = (0, 16, 40, 56)

_F32 = jnp.float32
_BF16 = jnp.bfloat16
_U32 = jnp.uint32
_Q_SCALE = _DH ** -0.5 * math.log2(math.e)


def _dft_matrices():
    even = np.arange(0, _C, 2)
    k = np.concatenate([even, _C - 1 - even])
    ang = np.pi * np.outer(2 * k + 1, np.arange(_C)) / (2 * _C)
    fwd = np.concatenate([np.cos(ang), -np.sin(ang)], axis=0)
    half = np.concatenate([np.cos(ang[:_HALF]), -np.sin(ang[:_HALF])], axis=0).T / _C
    inv = np.concatenate([half[0::2], half[1::2]], axis=0)
    fwd = np.concatenate([fwd, np.concatenate([fwd[:, 0::2], fwd[:, 1::2]], axis=1)], axis=0)
    return fwd.astype(np.float32), inv.astype(np.float32)


def _dot(a, b, dims=((1,), (0,))):
    return lax.dot_general(a, b, (dims, ((), ())), preferred_element_type=_F32)


def _as_bf16(words):
    return pltpu.bitcast(words, _BF16)


def _row_pairs(words):
    return (lax.bitcast_convert_type(words << 16, _F32),
            lax.bitcast_convert_type(words & jnp.uint32(0xFFFF0000), _F32))


def _pack_rows(even, odd):
    n = even.shape[0]
    bits = lax.bitcast_convert_type(_round_bf16(jnp.concatenate([even, odd], axis=0)), _U32)
    return (bits[:n] >> 16) | bits[n:]


def _round_bf16(x):
    return x.astype(_BF16).astype(_F32)


def _rows(vreg, like):
    return jnp.tile(vreg, (like.shape[0] // 8, 1))


def _iota(shape, axis):
    return lax.broadcasted_iota(jnp.int32, shape, axis)


def _phi(t):
    return jnp.where(t > 0, t + 1.0, jnp.exp(t))


def _kernel(q_hbm, k_hbm, v_hbm, shift_hbm, h_hbm, d_hbm, x_hbm,
            wq_hbm, wk_hbm, wv_hbm, wo_hbm, beta_hbm, f_hbm, g_hbm, out_hbm,
            qa_buf, ka_buf, va_buf, h_buf, x_buf, wq_buf, wk_buf, wv_buf, wo_buf,
            shift_buf, d_buf, beta_buf, f_buf, g_buf, outa_buf, outb_buf,
            par_scr, gate_scr, skip_scr, z_scr, zero_smem,
            wt_scr, qs_scr, pq_scr, vt_scr, kn_scr, pk_scr, ot_scr, sem):
    qa_w, ka_w, va_w, outa_w, f_w, g_w, wk_w, wt_w, qs_w, pq_w, kn_w, pk_w = (
        ref.bitcast(_U32) for ref in (qa_buf, ka_buf, va_buf, outa_buf, f_buf, g_buf, wk_buf,
                                      wt_scr, qs_scr, pq_scr, kn_scr, pk_scr))

    def block(j):
        return pl.ds(j * _C if isinstance(j, int) else pl.multiple_of(j * _C, _C), _C)

    def words(a):
        return slice(a * _HALF, (a + 1) * _HALF)

    cp = pltpu.make_async_copy

    def start(copies):
        for c in copies:
            c.start()

    def wait(copies):
        for c in copies:
            c.wait()

    def weight_copies(j, s):
        return [cp(w.at[:, block(j)], buf.at[j], s)
                for w, buf in ((wk_hbm, wk_buf), (wq_hbm, wq_buf), (wv_hbm, wv_buf))]

    def signal_copies(j):
        s = sem.at[4 + (j & 1)]
        return [cp(k_hbm.at[:, block(j)], ka_buf.at[j, pl.ds(_PAD, _S)], s),
                cp(v_hbm.at[:, block(j)], va_buf.at[j], s),
                cp(q_hbm.at[:, block(j)], qa_buf.at[j], s)]

    def filter_copy(j):
        return [cp(h_hbm.at[block(j), :], h_buf.at[j], sem.at[4 + (j & 1)])]

    def conv_copies(j):
        return signal_copies(j) + filter_copy(j)

    def next_weights(j):
        return weight_copies(j + 1, sem.at[4 + (j & 1)])

    def x_copies(p):
        rows = pl.ds(_X_SPLIT[p], _X_SPLIT[p + 1] - _X_SPLIT[p])
        return [cp(x_hbm.at[rows], x_buf.at[rows], sem.at[p % 3])]

    def outa_copy(j, s=2):
        return cp(outa_buf.at[j], out_hbm.at[:, block(j)], sem.at[s])

    def outb_copy(p):
        rows = pl.ds(_OUT_SPLIT[p], _OUT_SPLIT[p + 1] - _OUT_SPLIT[p])
        return cp(outb_buf.at[rows], out_hbm.at[rows, pl.ds(_D, _D)], sem.at[2])

    def transpose_weights(j):
        for w_buf, base in ((wq_buf, 0), (wv_buf, _C)):
            wt = w_buf[j].T
            for g in range(_NG):
                wt_scr[j, g, base:base + _C, :] = wt[:, g * _C:(g + 1) * _C]

    def project(j, lo, fine=False):
        n = _PIECE
        xs = x_buf[lo:lo + n, :]
        wk = jnp.concatenate([_as_bf16(wk_w[j, words(g), :]) for g in range(_NG)], axis=0)
        if fine:
            kn = jnp.concatenate([_dot(xs[r:r + _HALF], wk) for r in range(0, n, _HALF)], axis=0)
        else:
            kn = _dot(xs, wk)
        kn_scr[j, lo:lo + n, :] = kn.astype(_BF16)
        if lo < _S - _L:
            pk_scr[j, lo:lo + n, :] = _phi(kn).astype(_BF16)
        wt = jnp.concatenate([_as_bf16(wt_w[j, g]) for g in range(_NG)], axis=1)
        if fine:
            qv = jnp.concatenate([_dot(wt[r:r + _C], xs, ((1,), (1,))) for r in (0, _C)], axis=0)
        else:
            qv = _dot(wt, xs, ((1,), (1,)))
        for t in range(n // _C):
            tt = lo // _C + t
            qt = qv[0:_C, t * _C:(t + 1) * _C]
            qs_scr[tt, block(j), :] = (qt * _Q_SCALE).astype(_BF16)
            if tt >= _NT:
                pq_scr[tt - _NT, block(j), :] = _phi(qt).astype(_BF16)
            vt_scr[tt, block(j), :] = _round_bf16(qv[_C:2 * _C, t * _C:(t + 1) * _C])

    def filter_spectrum(j, a):
        z_scr[1, a] = _dot(_as_bf16(f_w[0:_C, :]), h_buf[j, :, a * _C:(a + 1) * _C],
                           ((1,), (1,)))

    def signal_spectrum(j, a):
        lo = _PAD // 2 + a * _HALF
        e0, o0 = _row_pairs(ka_w[j, lo:lo + _HALF, :])
        e1, o1 = _row_pairs(ka_w[j, lo - 1:lo - 1 + _HALF, :])
        _, o2 = _row_pairs(ka_w[j, lo - 2:lo - 2 + _HALF, :])
        w0, w1, w2, w3 = (_rows(par_scr[j, t], e0) for t in range(_KS))
        ve, vo = _row_pairs(va_w[j, words(a), :])
        kv = jnp.concatenate([(e0 * w0 + o1 * w1 + e1 * w2 + o2 * w3) * ve,
                              (o0 * w0 + e0 * w1 + o1 * w2 + e1 * w3) * vo], axis=0)
        skip_scr[a] = kv * _rows(par_scr[j, _KS], kv)
        z_scr[0, a] = _dot(_as_bf16(f_w[_C:2 * _C, :]), kv.astype(_BF16))

    def cross_chunks():
        z_st, z_ld = zero_smem[0], zero_smem[1]
        nb = 4
        for r in range(_NC):
            re, im = slice(8 * r, 8 * r + 8), slice(_C + 8 * r, _C + 8 * r + 8)

            def triple(which, a):
                x, y = z_scr[z_ld + which, a, re, :], z_scr[z_ld + which, a, im, :]
                return x, y, x + y

            prev = None
            for lo in range(0, _NC, nb):
                u, acc = {}, {}
                for t in range(lo + nb):
                    h = triple(1, t)
                    for a in range(max(lo, t), lo + nb):
                        if a - t not in u:
                            u[a - t] = triple(0, a - t)
                        prod = [x * y for x, y in zip(u[a - t], h)]
                        acc[a] = prod if t == 0 else [x + y for x, y in zip(acc[a], prod)]
                outs = []
                for a in range(lo, lo + nb):
                    k1, k2, k3 = acc[a]
                    yr, yi = cur = (k1 - k2, k3 - k1 - k2)
                    if prev is not None:
                        yr, yi = ((yr - prev[1], yi + prev[0]) if r < _NC // 2
                                  else (yr + prev[1], yi - prev[0]))
                    prev = cur
                    outs.append((a, yr, yi))
                for a, yr, yi in outs:
                    z_scr[z_st + 2, a, re, :] = yr
                    z_scr[z_st + 2, a, im, :] = yi

    def finish(j, a):
        y = z_scr[zero_smem[1] + 2, a]
        lo_re, hi_re, lo_im, hi_im = (y[q * _HALF:(q + 1) * _HALF] for q in range(4))
        spec_e = jnp.concatenate([lo_re + hi_re, lo_im - hi_im], axis=0).astype(_BF16)
        spec_o = jnp.concatenate([lo_re - hi_re, lo_im + hi_im], axis=0).astype(_BF16)
        ye = _dot(_as_bf16(g_w[0:_HALF // 2, :]), spec_e)
        yo = _dot(_as_bf16(g_w[_HALF // 2:_HALF, :]), spec_o)
        qe, qo = _row_pairs(qa_w[j, words(a), :])
        outa_w[j, words(a), :] = _pack_rows(qe * (ye + skip_scr[a, 0:_HALF, :]),
                                            qo * (yo + skip_scr[a, _HALF:_C, :]))

    def convolve(j, before, during):
        for job in before:
            job()
        for a in range(_NC + 4):
            if a < _NC:
                filter_spectrum(j, a)
            if a >= 4:
                signal_spectrum(j, a - 4)
        for job in during:
            job()
        cross_chunks()
        for a in range(_NC):
            finish(j, a)

    row8 = _iota((8, _C), 0)

    class Quad:
        def __init__(self, m):
            self.m = m
            self.wrow = pl.ds(m * _QW // 2, _QW // 2)
            self.mem = None
            self.a_mem, self.keys, self.q = {}, {}, {}

        def gate(self, hh):
            return gate_scr[4 * self.m + hh]

        def window(self, src, lo, n):
            g, off = divmod(self.m * _QW, _C)
            rows = slice(lo // 2, (lo + n) // 2)
            if off == 0:
                return _as_bf16(src[g, rows, :])
            w = jnp.where(_iota((n // 2, _C), 1) >= off, src[g, rows, :],
                          src[min(g + 1, _NG - 1), rows, :])
            return _as_bf16(pltpu.roll(w, _C - off, 1))

        def natural_window(self, src, lo, n):
            g, off = divmod(self.m * _QW, _C)
            rows = slice(lo // 2, (lo + n) // 2)
            if off + _QW <= _C:
                return _as_bf16(src[g, rows, :])
            return _as_bf16(jnp.where(_iota((n // 2, _C), 1) >= off, src[g, rows, :],
                                      src[g + 1, rows, :]))

        def values(self, s, t, lo, n):
            first = self.m * _QW + lo
            return vt_scr[_NT * s + t, first:first + n, :]

        def values_and_ones(self, s, t, hh):
            v = self.values(s, t, _WINDOW[hh], 24)
            if hh % 2:
                return jnp.concatenate([jnp.where(row8 < 4, 1.0, v[:8]), v[8:]], axis=0)
            return jnp.concatenate([v[:16], jnp.where(row8 < 4, v[16:], 1.0)], axis=0)

        def memory_update(self, s):
            v_ext = jnp.concatenate(
                [jnp.concatenate([self.values(s, t, 0, _QW), jnp.ones((8, _C), _F32)], axis=0)
                 for t in range(_NT)], axis=1)
            row = _iota((_QW + 8, _C), 0)
            lane = (_iota((_QW + 8, _C), 1) - self.m * _QW % _C) & (_C - 1)
            keep = jnp.zeros((_QW + 8, _C), jnp.bool_)
            for hh in range(4):
                rows = ((row >= _DH * hh) & (row < _DH * (hh + 1))) | (row == _QW + hh)
                keep = keep | (rows & (lane >= _DH * hh) & (lane < _DH * (hh + 1)))
            upd = jnp.where(keep, _dot(v_ext, self.natural_window(pk_w, s * _L, _L)), 0.0)
            self.mem = upd if self.mem is None else self.mem + upd

        def memory_read(self, s):
            tiles = []
            for i in range(_NT):
                w = pq_w[_NT * (s - 1) + i, self.wrow, :]
                slots = [jnp.zeros((8, _C), _U32)] * 8
                for t in range(_QW // 16):
                    slots[(self.m * _QW // 16 + t) % 8] = w[8 * t:8 * t + 8]
                tiles.append(_as_bf16(jnp.concatenate(slots, axis=0)))
            pq = jnp.concatenate(tiles, axis=1)
            got = _dot(_round_bf16(self.mem), pq)
            for i in range(_NT):
                gi = got[:, i * _C:(i + 1) * _C]
                f = [self.gate(hh)
                     / (jnp.broadcast_to(gi[_QW + hh:_QW + hh + 1], (8, _C)) + 1e-6)
                     for hh in range(4)]
                self.a_mem[s, i] = gi[0:_QW] * jnp.concatenate(
                    [f[0], f[0], jnp.where(row8 < 4, f[0], f[1]), f[1], f[1],
                     f[2], f[2], jnp.where(row8 < 4, f[2], f[3]), f[3], f[3]], axis=0)

        def queries(self, s, i):
            if (s, i) not in self.q:
                qq = qs_w[_NT * s + i, self.wrow, :]
                row = _iota((16, _C), 0)
                tiles = []
                for hh in range(4):
                    qh = jnp.where((row >= 2 * hh) & (row < 2 * hh + _DH // 2),
                                   qq[8 * hh:8 * hh + 16], jnp.uint32(0))
                    if hh % 2:
                        qh = pltpu.roll(qh, _HALF, 1)
                    parts = [jnp.zeros((8 * hh, _C), _U32)] if hh > 0 else []
                    parts += [qh, jnp.zeros((_HALF - 16 - 8 * hh, _C), _U32)]
                    tiles.append(jnp.concatenate(parts, axis=0))
                self.q = {(s, i): tiles}
            return self.q[s, i]

        def logits(self, s, i, t):
            if (s, t) not in self.keys:
                self.keys[s, t] = self.window(kn_w, s * _L + t * _C, _C)
            keys, qs = self.keys[s, t], self.queries(s, i)
            all_q = jnp.concatenate([_as_bf16(q) for q in qs], axis=1)
            if t < i:
                sc = _dot(keys, all_q)
                return [sc[:, hh * _C:(hh + 1) * _C] for hh in range(4)]
            key, lane = _iota((_HALF, _C), 0), _iota((_HALF, _C), 1)
            sc = _dot(keys[:_HALF], all_q)
            top = [jnp.where(key <= (lane ^ (_HALF * (hh % 2))), sc[:, hh * _C:(hh + 1) * _C],
                             -jnp.inf) for hh in range(4)]
            pair = jnp.concatenate(
                [_as_bf16(jnp.where(lane < _HALF, qs[hh + 1], qs[hh])) for hh in (0, 2)], axis=1)
            sc = jnp.concatenate(
                [_dot(keys[lo:lo + _HALF // 2], pair) for lo in (_HALF, _HALF + _HALF // 2)],
                axis=0)
            low = [jnp.where(key <= (lane & (_HALF - 1)), sc[:, c * _C:(c + 1) * _C], -jnp.inf)
                   for c in range(2)]
            return top, low

        def store(self, s, i, accs):
            part = []
            for hh in range(4):
                r = 0 if hh % 2 else 23
                norm = (1.0 - self.gate(hh)) / jnp.broadcast_to(accs[hh][r:r + 1], (8, _C))
                x = accs[hh] * _rows(norm, accs[hh])
                part.append(pltpu.roll(x, _HALF, 1) if hh % 2 else x)
            o = jnp.concatenate(
                [part[0][0:16], jnp.where(row8 < 4, part[0][16:24], part[1][0:8]), part[1][8:24],
                 part[2][0:16], jnp.where(row8 < 4, part[2][16:24], part[3][0:8]), part[3][8:24]],
                axis=0)
            if s > 0:
                o = o + self.a_mem.pop((s, i))
            ot_scr[_NT * s + i, self.m * _QW:(self.m + 1) * _QW, :] = o.astype(_BF16)

    def attention(which):
        units = [(quad, s, i, t) for quad in map(Quad, which) for s in range(_NSEG)
                 for i in range(_NT) for t in range(i + 1)]
        left, left_w = _iota((8, _C), 1) < _HALF, _iota((_HALF // 2, _C), 1) < _HALF

        def col_max(x):
            return jnp.broadcast_to(jnp.max(x, axis=0, keepdims=True), (8, _C))

        def weights(x, mx):
            return jnp.exp2(x - _rows(mx, x)).astype(_BF16)

        scores, run_max, accs = {}, {}, None
        for n in range(len(units) + _LAG):
            if n < len(units):
                quad, s, i, t = units[n]
                if s > 0 and (i, t) == (0, 0):
                    quad.memory_update(s - 1)
                if s > 0 and (i, t) == (1, 1):
                    quad.memory_read(s)
                scores[n] = sc = quad.logits(s, i, t)
                if t < i:
                    cur = [col_max(x) for x in sc]
                else:
                    low = [col_max(x) for x in sc[1]]
                    cur = [jnp.maximum(col_max(x),
                                       jnp.where(left if hh % 2 else ~left, low[hh // 2], -jnp.inf))
                           for hh, x in enumerate(sc[0])]
                if t > 0:
                    cur = [jnp.maximum(x, y) for x, y in zip(cur, run_max[n - 1])]
                run_max[n] = cur
            if n >= _LAG:
                u = n - _LAG
                quad, s, i, t = units[u]
                sc, mx = scores.pop(u), run_max[u]
                if t < i:
                    ps = [weights(sc[hh], mx[hh]) for hh in range(4)]
                else:
                    low = [pltpu.bitcast(
                        weights(sc[1][c], jnp.where(left, mx[2 * c + 1], mx[2 * c])), _U32)
                        for c in range(2)]
                    ps = [jnp.concatenate(
                        [weights(sc[0][hh], mx[hh]),
                         _as_bf16(jnp.where(left_w if hh % 2 else ~left_w, low[hh // 2],
                                            jnp.uint32(0)))], axis=0) for hh in range(4)]
                cur = []
                for hh in range(4):
                    pv = _dot(quad.values_and_ones(s, t, hh), ps[hh])
                    if t > 0:
                        pv = pv + accs[hh] * _rows(jnp.exp2(run_max[u - 1][hh] - mx[hh]), pv)
                    cur.append(pv)
                accs = cur
                if t == i:
                    quad.store(s, i, accs)

    def output_projection(p):
        lo, hi = _OUT_SPLIT[p] // _C, _OUT_SPLIT[p + 1] // _C
        ot = jnp.concatenate([ot_scr[t] for t in range(lo, hi)], axis=1)
        outb_buf[lo * _C:hi * _C, :] = _dot(ot, wo_buf[...], ((0,), (0,))).astype(_BF16)
        outb_copy(p).start()

    def first_rows(p):
        for lo in range(_X_SPLIT[p], _X_SPLIT[p + 1], _PIECE):
            project(0, lo, fine=p < 4)

    small = [cp(shift_hbm, shift_buf, sem.at[3]), cp(d_hbm, d_buf, sem.at[3]),
             cp(beta_hbm, beta_buf, sem.at[3])]
    first_weights = weight_copies(0, sem.at[0])
    second_batch = [cp(f_hbm, f_buf, sem.at[3]), cp(g_hbm, g_buf, sem.at[3])]
    second_batch += weight_copies(1, sem.at[3])
    wo_copy = cp(wo_hbm, wo_buf, sem.at[4 + ((_NG - 1) & 1)])

    start(small + first_weights + x_copies(0))
    for g in range(_NG):
        ka_w[g, 0:_PAD // 2, :] = jnp.zeros((_PAD // 2, _C), _U32)
    zero_smem[0] = 0
    zero_smem[1] = 0
    wait(first_weights)
    start(x_copies(1) + x_copies(2))
    wait(x_copies(0) + small)
    transpose_weights(0)
    first_rows(0)
    start(x_copies(3))
    wait(x_copies(1))
    first_rows(1)
    start(x_copies(4))
    wait(x_copies(2))
    first_rows(2)
    wait(x_copies(3))
    first_rows(3)
    start(second_batch + conv_copies(0))
    wait(x_copies(4))
    shift = shift_buf[...].astype(_F32)
    skip = d_buf[...].astype(_F32).reshape(1, _D)
    for g in range(_NG):
        lanes = slice(g * _C, (g + 1) * _C)
        for t in range(_KS):
            par_scr[g, t] = jnp.broadcast_to(shift[t:t + 1, lanes], (8, _C))
        par_scr[g, _KS] = jnp.broadcast_to(skip[:, lanes], (8, _C))
    gate = 1.0 / (1.0 + jnp.exp(-beta_buf[...].astype(_F32).reshape(1, _H)))
    for hd in range(_H):
        gate_scr[hd] = jnp.broadcast_to(gate[:, hd:hd + 1], (8, _C))
    first_rows(4)
    attention(range(1))
    wait(second_batch)

    def fused(j, carry):
        @pl.when(j > 0)
        def _():
            wait(next_weights(j))

        wait(signal_copies(j))

        @pl.when(j + 2 < _NG)
        def _():
            start(conv_copies(j + 1) + next_weights(j + 1))

        wait(filter_copy(j))
        transpose_weights(j + 1)
        jobs = [functools.partial(project, j + 1, lo) for lo in range(0, _S, _PIECE)]
        convolve(j, jobs[:1], jobs[1:])
        outa_copy(j, jnp.where(j == 0, 1, 2)).start()
        return carry

    lax.fori_loop(0, _NG - 1, fused, 0)

    start(conv_copies(_NG - 1) + [wo_copy])
    wait([outa_copy(0, 1)])
    attention(range(1, _NQ))

    n_out = len(_OUT_SPLIT) - 1
    wait(conv_copies(_NG - 1) + [wo_copy])
    convolve(_NG - 1, [], [functools.partial(output_projection, p) for p in range(_OUT_OVERLAP)])
    outa_copy(_NG - 1).start()
    for p in range(_OUT_OVERLAP, n_out):
        output_projection(p)
    wait([outa_copy(j) for j in range(1, _NG)] + [outb_copy(p) for p in range(n_out)])


@jax.jit
def pallas_concat_heads__ssm_conv_h3__memory_aug_infini_attn__prompt_kernel(
    A_q: jax.Array,
    A_k: jax.Array,
    A_v: jax.Array,
    A_shift_k: jax.Array,
    A_ssm_k: jax.Array,
    A_ssm_D: jax.Array,
    B_x: jax.Array,
    B_wq: jax.Array,
    B_wk: jax.Array,
    B_wv: jax.Array,
    B_wo: jax.Array,
    B_beta: jax.Array,
):
    assert A_q.shape == (1, _S, _D) and B_x.shape == (1, _S, _D)
    assert A_shift_k.shape == (_D, _KS) and B_beta.shape == (_H,)
    f_fwd, f_inv = (m.astype(_BF16) for m in _dft_matrices())

    vmem = pltpu.VMEM
    scratch = [
        vmem((_NG, _S, _C), _BF16),
        vmem((_NG, _PAD + _S, _C), _BF16),
        vmem((_NG, _S, _C), _BF16),
        vmem((_NG, _C, _S), _BF16),
        vmem((_S, _D), _BF16),
        vmem((_NG, _D, _C), _BF16),
        vmem((_NG, _D, _C), _BF16),
        vmem((_NG, _D, _C), _BF16),
        vmem((_D, _D), _BF16),
        vmem((_KS, _D), _BF16),
        vmem((_D,), _BF16),
        vmem((_H,), _BF16),
        vmem((4 * _C, _C), _BF16),
        vmem((_C, _C), _BF16),
        vmem((_NG, _S, _C), _BF16),
        vmem((_S, _D), _BF16),
        vmem((_NG, _KS + 1, 8, _C), _F32),
        vmem((_H, 8, _C), _F32),
        vmem((_NC, _C, _C), _F32),
        vmem((3, _NC, 2 * _C, _C), _F32),
        pltpu.SMEM((2,), jnp.int32),
        vmem((_NG, _NG, 2 * _C, _C), _BF16),
        vmem((_NC, _D, _C), _BF16),
        vmem((_NC - _NT, _D, _C), _BF16),
        vmem((_NC, _D, _C), _F32),
        vmem((_NG, _S, _C), _BF16),
        vmem((_NG, _S - _L, _C), _BF16),
        vmem((_NC, _D, _C), _BF16),
        pltpu.SemaphoreType.DMA((6,)),
    ]
    out = pl.pallas_call(
        _kernel,
        out_shape=jax.ShapeDtypeStruct((_S, 2 * _D), _BF16),
        in_specs=[pl.BlockSpec(memory_space=pl.ANY)] * 14,
        out_specs=pl.BlockSpec(memory_space=pl.ANY),
        scratch_shapes=scratch,
        compiler_params=pltpu.CompilerParams(
            vmem_limit_bytes=100 * 1024 * 1024, disable_bounds_checks=True),
        name="h3_infini",
    )(A_q.reshape(_S, _D), A_k.reshape(_S, _D), A_v.reshape(_S, _D), A_shift_k.T,
      A_ssm_k, A_ssm_D, B_x.reshape(_S, _D), B_wq, B_wk, B_wv, B_wo, B_beta, f_fwd, f_inv)
    return out.reshape(1, _S, 2 * _D)
```
